```python
import jax
import jax.numpy as jnp

def _softmax(x, axis=-1):
    return jax.nn.softmax(x, axis=axis)
def _gelu(x):
    return jax.nn.gelu(x, approximate=True)
def _silu(x):
    return jax.nn.silu(x)
def _sigmoid(x):
    return jax.nn.sigmoid(x)
def _layernorm(x, axis=-1, eps=1e-5):
    m = jnp.mean(x, axis=axis, keepdims=True)
    v = jnp.var(x, axis=axis, keepdims=True)
    return (x - m) / jnp.sqrt(v + eps)
def _scatter_add(tgt, idx, src, axis=0):
    return tgt.at[idx].add(src)
def _segment_sum(src, seg, n):
    return jax.ops.segment_sum(src, seg, n)
class _Rng:
    def __init__(self, key):
        self._k = key
    def _next(self):
        self._k, sub = jax.random.split(self._k)
        return sub
    def normal(self, shape):
        return jax.random.normal(self._next(), shape, dtype=jnp.bfloat16)
    def randint(self, lo, hi, shape):
        return jax.random.randint(self._next(), shape, lo, hi, dtype=jnp.int32)
    def uniform(self, shape, lo=0.0, hi=1.0):
        return jax.random.uniform(self._next(), shape, jnp.bfloat16, lo, hi)
    def permutation(self, n):
        return jax.random.permutation(self._next(), n)


kernel_name = 'standalone__modern_conv_block_slak__vision'

def setup_inputs():
    _rng = _Rng(jax.random.key(int.from_bytes(__import__("os").urandom(4), "little")))
    _w = (lambda a: (lambda t: t.astype(jnp.bfloat16) if jnp.issubdtype(t.dtype, jnp.floating) else t)(jnp.asarray(a)))
    H = W = 384
    C = 384
    K = 1
    return {
        "x": _w((lambda *s: _rng.normal(s) * 0.05)(1, H, W, C)),
        "dw": _w((lambda *s: _rng.normal(s) * 0.05)(K, K, C)),
        "w1": _w((lambda *s: _rng.normal(s) * 0.05)(C, 4 * C)),
        "w2": _w((lambda *s: _rng.normal(s) * 0.05)(4 * C, C)),
        "grn_g": _w((lambda *s: _rng.normal(s) * 0.05)(4 * C)),
        "grn_b": _w((lambda *s: _rng.normal(s) * 0.05)(4 * C)),
    }

def reference(x, dw, w1, w2, grn_g, grn_b):
    B, H, W, C = x.shape
    K = dw.shape[0]
    pad = K // 2
    xp = jnp.pad(x, ((0,0),(pad,pad),(pad,pad),(0,0)))
    out = jnp.zeros_like(x)
    for i in range(K):
        for j in range(K):
            out = out + xp[:, i:i+H, j:j+W, :] * dw[i, j][None, None, None, :]
    h = _layernorm(out, axis=-1)
    h = _gelu(h @ w1)
    gx = jnp.sqrt((h * h).sum(axis=(1, 2), keepdims=True) + 1e-6)
    nx = gx / (gx.mean(axis=-1, keepdims=True) + 1e-6)
    h = grn_g[None, None, None, :] * (h * nx) + grn_b[None, None, None, :] + h
    return x + h @ w2
```

```python
import functools
import numpy as np
import jax
import jax.numpy as jnp
from jax import lax
import jax.experimental.pallas as pl
import jax.experimental.pallas.tpu as pltpu

C = 384
HID = 1536
L = 128
F32 = jnp.float32
BF16 = jnp.bfloat16
U32 = jnp.uint32
pk = lambda v: pltpu.bitcast(v.astype(BF16), U32)
upk = lambda v: pltpu.bitcast(v, BF16)


def pack16(v):
    t = v.shape[0] // 16
    lo = jnp.concatenate([v[16 * g:16 * g + 8] for g in range(t)], axis=0)
    hi = jnp.concatenate([v[16 * g + 8:16 * g + 16] for g in range(t)], axis=0)
    return pltpu.pack_elementwise([lo, hi], packed_dtype=BF16)


def unpack16(w):
    lo = pltpu.unpack_elementwise(w, index=0, packed_dtype=BF16, unpacked_dtype=F32)
    hi = pltpu.unpack_elementwise(w, index=1, packed_dtype=BF16, unpacked_dtype=F32)
    parts = []
    for g in range(w.shape[0] // 8):
        parts += [lo[8 * g:8 * g + 8], hi[8 * g:8 * g + 8]]
    return jnp.concatenate(parts, axis=0)
K0 = float(np.sqrt(2.0 / np.pi))
ALPHA = float((K0 * 0.044715) ** (1.0 / 3.0))
C0 = K0 / ALPHA
HS = 0.5 / ALPHA

WB = [[1, 0, -1, 1, 0, 0, 0, 0, 0], [-1, -1, 0, 0, 0, 0, -1, 0, 0], [0, 0, 0, 1, 1, 0, 0, -1, 0],
      [0, -1, 0, 0, -1, -1, 0, 0, 0], [0, 0, 1, 0, 0, 0, 0, 1, 1], [0, 0, 0, 0, 0, 1, 1, 0, -1],
      [0, -1, 0, 0, 0, 0, 0, 0, 0], [0, -1, 0, 1, 0, 0, 0, 0, 0], [0, 0, 0, 1, 0, 0, 0, 0, 0],
      [0, 0, 0, 0, 0, -1, 0, 0, 0], [0, 0, 0, 0, 0, -1, 0, -1, 0], [0, 0, 0, 0, 0, 0, 0, -1, 0],
      [0, 0, -1, 0, 0, 0, 0, 0, 0], [0, 0, -1, 0, 0, 0, -1, 0, 0], [0, 0, 0, 0, 0, 0, -1, 0, 0]]
SG = [1, -1, -1, -1, 1, 1, 1, 1, 1, 1, 1, -1, 1, 1, 1]


def hk_operands(get32, raw):
    memo = {}
    def m(name, f):
        if name not in memo:
            memo[name] = f()
        return memo[name]
    f6 = lambda: m("f6", lambda: get32(0, 0) - get32(0, 1))
    f7 = lambda: m("f7", lambda: get32(1, 0) - f6())
    f11 = lambda: m("f11", lambda: get32(1, 1) + get32(1, 2))
    f10 = lambda: m("f10", lambda: get32(0, 2) - f11())
    forms = {
        0: lambda: get32(1, 0) - get32(0, 0),
        5: lambda: get32(1, 2) - get32(0, 2),
        6: f6, 7: f7,
        8: lambda: f7() - get32(1, 1),
        9: lambda: -(get32(0, 1) + f10()),
        10: f10, 11: f11,
        12: lambda: get32(0, 0) - get32(0, 2),
        13: lambda: get32(0, 2) - get32(1, 0),
        14: lambda: get32(1, 2) - get32(1, 0),
    }
    forms[9] = lambda: get32(0, 1) + f10()
    raws = {1: (1, 0), 2: (1, 1), 3: (0, 1), 4: (0, 2)}
    def op(p):
        return raw(*raws[p]) if p in raws else forms[p]().astype(BF16)
    return op
SG[9] = -1


def hk_combine(P, emit):
    p6 = P(6); p10 = P(10); p11 = P(11)
    s2 = p10 - p11
    v2 = P(9) + s2
    emit(0, 1, P(3) - v2 - p6)
    p4 = P(4)
    t2 = s2 + p4
    p12 = P(12)
    emit(0, 2, v2 + p4 - p12)
    s1 = p6 + P(7)
    v1 = P(8) - s1
    emit(1, 1, v1 + p11 - P(2))
    p1 = P(1)
    t1 = s1 + p1 - p12
    p14 = P(14)
    emit(1, 0, p1 - v1 - p14)
    p13 = P(13)
    t3 = t2 + p13 - p14
    emit(0, 0, t1 - p13 - P(0))
    emit(1, 2, t3 - P(5))


def make(CH=512, G=4, S=72, XR=4, MC1=32, MC2=None, vmem_mb=127, flags=None, E1=2, E2=2,
         run1=True, run2=True, dma=True, comp=True):
    TM = CH * G
    MC2 = MC2 or CH

    @jax.jit
    def fn(x, dw, w1, w2, grn_g, grn_b):
        B, H, W, _ = x.shape
        N = B * H * W
        NT = N // TM
        NCH = N // CH
        NHC = NCH - S
        R1 = -(-NHC * 65536 // (NT - E1))
        R2 = -(-NHC * 65536 // (NT - E2))
        assert max(R1, R2) <= G * 65536 and S >= 2 * G

        def kernel(x_hbm, dw_ref, w1_ref, w2_ref, g_ref, b_ref, out_hbm, h_hbm,
                   xbuf, hbuf, ws, ssq, xsem, osem, hsem):
            class _Nop:
                def start(self): pass
                def wait(self): pass
            mk = pltpu.make_async_copy if dma else (lambda *a: _Nop())

            def x_copy(i, slot):
                return mk(x_hbm.at[pl.ds(i * TM, TM)], xbuf.at[slot], xsem.at[slot])

            def o_copy(i, slot):
                return mk(xbuf.at[slot], out_hbm.at[pl.ds(i * TM, TM)], osem.at[slot])

            def h_out(c, slot):
                return mk(hbuf.at[slot], h_hbm.at[c], hsem.at[slot])

            def h_in(c, slot):
                return mk(h_hbm.at[c], hbuf.at[slot], hsem.at[slot])

            def wrap(v, n):
                return jnp.where(v >= n, v - n, v)

            def wrapn(v, n):
                return jnp.where(v < 0, v + n, v)

            def comb(coefs, get):
                acc = None
                for q in sorted(range(9), key=lambda q: -coefs[q]):
                    c = coefs[q]
                    if c == 0:
                        continue
                    v = get(q // 3, q % 3)
                    acc = (v if c > 0 else -v) if acc is None else (acc + v if c > 0 else acc - v)
                return acc

            for i in range(XR - 1):
                x_copy(i, i).start()
            ssq[...] = jnp.zeros_like(ssq)
            dwv = dw_ref[...].astype(F32)
            for p in range(15):
                for c in range(4):
                    ws[p * 4 + c] = pk(comb([SG[p] * v for v in WB[p]], lambda k, j: w1_ref[k * L:(k + 1) * L, j * 512 + c * L:j * 512 + (c + 1) * L].astype(F32)))

            def layernorm(xs, r0):
                y = xbuf[xs, pl.ds(r0, MC1), :].astype(F32) * dwv
                mu = jnp.sum(y, axis=-1, keepdims=True) * (1.0 / C)
                d = y - mu
                ss = jnp.sum(d * d, axis=-1, keepdims=True)
                return d * lax.rsqrt(ss * (1.0 / (C * ALPHA * ALPHA)) + 1e-5 / (ALPHA * ALPHA))

            def act(y, hs, r0, c):
                t = jnp.tanh(y * (y * y + C0))
                h = y * t + y
                ssq[:, c * L:(c + 1) * L] += jnp.sum((h * h).reshape(MC1 // 8, 8, L), axis=0)
                hbuf[hs, pl.ds(r0 // 2, MC1 // 2), c * L:(c + 1) * L] = pack16(h)

            def phase1(i, carry):
                xs, hb, q, qs = carry
                @pl.when(i + XR - 1 < NT)
                def _():
                    x_copy(i + XR - 1, wrapn(xs - 1, XR)).start()
                x_copy(i, xs).wait()
                slots = [wrap(hb + u, S) for u in range(G)]
                for u in range(G):
                    @pl.when(i * G + u >= S)
                    def _():
                        h_out(i * G + u - S, slots[u]).wait()
                for u in range(G if comp else 0):
                    for m in range(CH // (2 * MC1)):
                        r0 = [(2 * m + t) * MC1 for t in range(2)]
                        a = [layernorm(xs, u * CH + r) for r in r0]
                        g32 = lambda t, k: a[t][:, k * L:(k + 1) * L]
                        op0 = hk_operands(g32, lambda t, k: g32(t, k).astype(BF16))
                        ops = {}
                        def op(p):
                            if p not in ops:
                                ops[p] = op0(p)
                            return ops[p]
                        for c in range(4):
                            hk_combine(lambda p: jnp.dot(op(p), upk(ws[p * 4 + c]), preferred_element_type=F32),
                                       lambda t, j, y: act(y, slots[u], r0[t], 4 * j + c))
                qn = jnp.minimum(((i + 1) * R1) >> 16, NHC)
                for u in range(G):
                    @pl.when(q + u < qn)
                    def _():
                        h_out(q + u, wrap(qs + u, S)).start()
                return wrap(xs + 1, XR), wrap(hb + G, S), qn, wrap(qs + (qn - q), S)

            z = jnp.int32(0)
            if run1:
                lax.fori_loop(0, NT, phase1, (z, z, z, z))
            else:
                for i in range(XR - 1):
                    x_copy(i, i).wait()

            gx = jnp.sqrt(jnp.sum(ssq[...], axis=0, keepdims=True) * (HS * HS) + 1e-6)
            nx = gx / (jnp.mean(gx, axis=-1, keepdims=True) + 1e-6)
            sc = (g_ref[...].astype(F32) * nx + 1.0) * HS
            for r in range(4):
                cols = [jnp.broadcast_to(sc[:, (4 * k + r) * L:(4 * k + r + 1) * L], (L, L)).T for k in range(3)]
                tile = lambda k, j: w2_ref[(4 * k + r) * L:(4 * k + r + 1) * L, j * L:(j + 1) * L].astype(F32) * cols[k]
                for p in range(15):
                    ws[p * 4 + r] = pk(comb([SG[p] * v for v in WB[p]], tile))
            bias = jnp.dot(jnp.broadcast_to(b_ref[...], (16, HID)), w2_ref[...], preferred_element_type=F32)[0:1]

            def phase2(j, carry):
                xs, hb, q, qs = carry
                i = NT - 1 - j
                @pl.when(j >= XR)
                def _():
                    x_copy(i, xs).wait()
                slots = [wrap(hb + u, S) for u in range(G)]
                for u in range(G):
                    @pl.when(i * G + u < NHC)
                    def _():
                        h_in(i * G + u, slots[u]).wait()
                for m in range(TM // (2 * MC2) if comp else 0):
                    r0 = [(2 * m + t) * MC2 for t in range(2)]
                    g32 = lambda t, k: unpack16(hbuf[slots[r0[t] // CH], pl.ds(r0[t] % CH // 2, MC2 // 2), k * 512:(k + 1) * 512])
                    op = hk_operands(g32, lambda t, k: g32(t, k).astype(BF16))
                    def emit(t, jj, o):
                        cs = slice(jj * L, (jj + 1) * L)
                        rows = pl.ds(r0[t], MC2)
                        xbuf[xs, rows, cs] = (o + bias[:, cs] + xbuf[xs, rows, cs].astype(F32)).astype(BF16)
                    hk_combine(lambda p: jnp.dot(op(p), upk(jnp.concatenate([ws[p * 4 + c] for c in range(4)], axis=0)), preferred_element_type=F32), emit)
                o_copy(i, xs).start()
                nxt = wrap(xs + 1, XR)
                @pl.when(j >= 1)
                def _():
                    o_copy(i + 1, nxt).wait()
                    @pl.when(i + 1 - XR >= 0)
                    def _():
                        x_copy(i + 1 - XR, nxt).start()
                qn = jnp.minimum(((j + 1) * R2) >> 16, NHC)
                for u in range(G):
                    @pl.when(q + u < qn)
                    def _():
                        h_in(NHC - 1 - q - u, wrapn(qs - u, S)).start()
                return wrapn(xs - 1, XR), wrapn(hb - G, S), qn, wrapn(qs - (qn - q), S)

            if run2:
                lax.fori_loop(0, NT, phase2, (z + (NT - 1) % XR, z + (NCH - G) % S, z, z + (NHC - 1) % S))
                o_copy(0, 0).wait()

        out, _ = pl.pallas_call(
            kernel,
            in_specs=[pl.BlockSpec(memory_space=pl.ANY)] + [pl.BlockSpec(memory_space=pltpu.VMEM)] * 5,
            out_specs=[pl.BlockSpec(memory_space=pl.ANY)] * 2,
            out_shape=[jax.ShapeDtypeStruct((N, C), BF16), jax.ShapeDtypeStruct((NHC, CH // 2, HID), U32)],
            scratch_shapes=[
                pltpu.VMEM((XR, TM, C), BF16),
                pltpu.VMEM((S, CH // 2, HID), U32),
                pltpu.VMEM((60, L // 2, L), U32),
                pltpu.VMEM((8, HID), F32),
                pltpu.SemaphoreType.DMA((XR,)),
                pltpu.SemaphoreType.DMA((XR,)),
                pltpu.SemaphoreType.DMA((S,)),
            ],
            compiler_params=pltpu.CompilerParams(vmem_limit_bytes=vmem_mb * 1024 * 1024, flags=flags),
        )(x.reshape(N, C), dw.reshape(1, C), w1, w2, grn_g.reshape(1, HID), grn_b.reshape(1, HID))
        return out.reshape(x.shape)
    return fn


pallas_standalone__modern_conv_block_slak__vision_kernel = make(CH=384,G=4,S=100,MC1=48)
```

```python
import functools
import numpy as np
import jax
import jax.numpy as jnp
from jax import lax
import jax.experimental.pallas as pl
import jax.experimental.pallas.tpu as pltpu

C = 384
HID = 1536
L = 128
F32 = jnp.float32
BF16 = jnp.bfloat16
U32 = jnp.uint32
pk = lambda v: pltpu.bitcast(v.astype(BF16), U32)
upk = lambda v: pltpu.bitcast(v, BF16)


def pack16(v):
    t = v.shape[0] // 16
    lo = jnp.concatenate([v[16 * g:16 * g + 8] for g in range(t)], axis=0)
    hi = jnp.concatenate([v[16 * g + 8:16 * g + 16] for g in range(t)], axis=0)
    return pltpu.pack_elementwise([lo, hi], packed_dtype=BF16)


def unpack16(w):
    lo = pltpu.unpack_elementwise(w, index=0, packed_dtype=BF16, unpacked_dtype=F32)
    hi = pltpu.unpack_elementwise(w, index=1, packed_dtype=BF16, unpacked_dtype=F32)
    parts = []
    for g in range(w.shape[0] // 8):
        parts += [lo[8 * g:8 * g + 8], hi[8 * g:8 * g + 8]]
    return jnp.concatenate(parts, axis=0)
K0 = float(np.sqrt(2.0 / np.pi))
ALPHA = float((K0 * 0.044715) ** (1.0 / 3.0))
C0 = K0 / ALPHA
HS = 0.5 / ALPHA

S433 = dict(m=4, k=3, n=3,
    a_prog=[(3, -1, 1, 1), (10, -1, 3, 1), (2, 1, 6, 1), (5, 1, 7, 1), (3, 1, 9, 1), (0, 1, 16, 1), (17, 1, 2, -1), (9, -1, 18, 1), (4, 1, 1, 1), (20, 1, 10, 1), (20, 1, 5, 1), (21, 1, 7, -1), (10, 1, 22, 1), (5, 1, 8, -1), (25, 1, 11, 1), (6, 1, 25, 1), (6, 1, 26, 1), (13, 1, 28, 1), (16, -1, 29, 1), (22, 1, 12, -1), (31, 1, 15, -1), (18, 1, 24, -1), (11, -1, 33, 1), (12, 1, 14, 1), (19, 1, 35, 1), (14, 1, 15, 1), (37, 1, 27, -1)],
    a_use=[13, 1, 16, 17, 18, 34, 2, 10, 11, 24, 21, 3, 5, 22, 19, 12, 1, 32, 15, 7, 27, 6, 36, 14, 38, 28, 30, 23, 26],
    c_prog=[(7, 1, 4, 1), (7, 1, 9, -1), (11, -1, 5, 1), (2, 1, 5, -1), (3, 1, 6, 1), (10, -1, 4, 1), (1, 1, 4, -1), (0, 1, 8, -1), (11, 1, 1, 1), (9, -1, 17, 1), (16, 1, 8, -1), (0, 1, 15, -1), (12, 1, 11, 1), (14, -1, 23, 1), (24, 1, 17, -1), (18, 1, 21, 1), (8, 1, 9, -1), (28, -1, 6, 1), (7, -1, 0, 1), (6, -1, 30, 1), (8, -1, 2, 1), (1, 1, 32, 1), (12, -1, 22, 1), (34, 1, 5, -1), (3, -1, 23, 1), (21, -1, 36, 1)],
    c_use=[(21, -1), (18, 1), (27, -1), (1, -1), (20, -1), (11, 1), (33, 1), (17, -1), (26, 1), (24, -1), (12, -1), (37, 1), (35, -1), (14, 1), (25, -1), (23, 1), (15, -1), (3, -1), (22, -1), (16, 1), (29, -1), (31, 1), (0, -1), (19, -1), (8, 1), (13, 1), (9, 1), (7, 1), (7, -1)],
    w=[[1, -1, 0, -1, 0, 0, 0, 0, 0], [0, 0, 0, 0, 1, 0, 0, 0, 0], [0, 1, 0, 0, 0, 0, 0, 0, 0], [0, -1, 1, 0, 0, 0, 0, -1, 1], [0, 0, -1, 0, 0, 0, 0, 1, -1], [0, 0, 0, 0, 0, 0, 0, 1, -1], [0, 0, 1, 0, 0, 0, 0, 0, 1], [1, -1, 0, -1, 1, 0, 0, 0, 0], [0, 0, 0, 0, 0, 0, 0, 1, 0], [0, 0, 0, 0, 0, -1, 0, -1, 1], [0, 0, 0, 0, -1, 1, 0, 1, -1], [-1, 0, 0, 1, 0, 0, 0, 0, 0], [0, 0, 0, 0, 0, -1, 0, 0, 1], [0, 0, 0, 0, 0, 1, 0, 0, 0], [0, 0, 1, 0, 0, 0, 0, 0, 0], [-1, 0, -1, 1, 0, 0, 0, 0, 0], [1, 0, 1, -1, 0, -1, 0, 0, 0], [0, 0, 0, -1, 0, 0, 0, 0, 0], [0, 0, 0, 0, 0, 1, -1, 0, -1], [0, 0, 0, 1, 0, 1, -1, 0, -1], [0, 0, 0, 0, 0, 0, 1, 0, 0], [-1, 0, 0, 0, 0, 0, -1, 0, 0], [-1, 0, -1, 0, 0, 0, 0, 0, 0], [0, 0, 1, 0, 0, 0, -1, 0, 0], [0, 0, 0, 0, 0, 0, 1, 0, 1], [-1, 1, 0, 0, 0, 0, -1, 0, 0], [-1, 1, 0, 0, 0, 0, 0, 0, 0], [0, 0, 0, 0, -1, 0, 0, 0, 0], [-1, 1, 0, 0, 0, 0, -1, 1, 0]])
S343 = dict(m=3, k=4, n=3,
    a_prog=[(0, 1, 10, -1), (4, 1, 5, 1), (6, 1, 5, 1), (7, 1, 5, 1), (11, 1, 4, 1), (3, 1, 6, 1), (9, 1, 8, 1), (11, 1, 9, 1), (2, 1, 1, 1), (0, 1, 18, -1), (3, 1, 15, 1), (20, 1, 10, -1), (14, 1, 11, -1), (22, 1, 13, -1), (21, 1, 19, 1), (24, 1, 15, -1), (23, 1, 24, -1), (28, 1, 19, -1), (12, 1, 26, -1), (30, 1, 16, 1), (1, 1, 3, 1), (32, -1, 23, 1), (33, -1, 12, 1), (34, 1, 17, -1), (32, 1, 21, 1), (15, 1, 36, 1)],
    a_use=[6, 13, 15, 14, 24, 22, 27, 29, 3, 20, 23, 6, 17, 25, 4, 16, 11, 31, 10, 12, 35, 33, 19, 18, 21, 37, 0, 26, 1],
    c_prog=[(0, 1, 2, -1), (5, 1, 8, -1), (0, 1, 6, 1), (6, 1, 8, -1), (2, 1, 6, 1), (2, 1, 8, 1), (3, -1, 0, 1), (7, 1, 8, -1), (0, 1, 1, -1), (1, -1, 15, 1), (2, 1, 16, -1), (15, 1, 2, -1), (5, 1, 16, 1), (6, 1, 17, 1), (6, 1, 10, 1), (19, -1, 1, 1), (3, 1, 23, -1), (18, 1, 4, 1), (22, 1, 7, -1), (4, 1, 21, -1), (20, 1, 5, 1)],
    c_use=[(4, -1), (4, 1), (26, 1), (28, -1), (21, 1), (18, 1), (5, -1), (16, 1), (15, -1), (24, -1), (19, 1), (29, 1), (20, -1), (3, 1), (25, 1), (23, 1), (10, -1), (12, -1), (14, -1), (13, 1), (9, -1), (2, -1), (7, -1), (27, -1), (22, -1), (17, -1), (11, 1), (6, -1), (1, -1)],
    w=[[0, -1, 0, 0, 1, 0, 0, -1, 0, 0, -1, 0], [0, 1, 0, 0, 0, 0, 0, 0, 0, 0, 0, 0], [0, 0, 0, 0, 0, 0, 0, 0, 0, 0, 1, 0], [0, 1, 0, 0, -1, 0, 0, 0, 0, 0, 1, 0], [0, -1, 0, 0, 1, 1, 0, 0, 0, 0, -1, 0], [0, 0, 0, -1, 0, 0, 0, 0, 0, 0, -1, 0], [0, 0, 0, 0, 0, 0, 0, 0, 0, 0, 0, 1], [0, 0, 0, 0, 0, 1, 0, 0, 0, 0, 0, 0], [0, 0, 0, 0, 0, 1, -1, 0, -1, -1, -1, -1], [0, 0, 0, 0, 0, 0, 0, -1, 0, 0, 0, 0], [0, 0, 0, 0, 0, 1, 0, 1, 0, 0, 0, 0], [0, 0, 0, 0, 0, -1, 0, 0, 1, 0, 0, 1], [0, 0, 0, 0, 0, -1, 1, 0, 1, 0, 0, 1], [0, 0, 0, -1, 0, 0, 0, 0, 0, 1, 0, 0], [1, 0, 0, -1, 0, 0, 0, 0, 0, 1, 0, 0], [1, 0, 1, -1, 0, 0, 0, 0, 0, 1, 0, 0], [1, 1, 1, -1, -1, -1, 0, 0, 0, 1, 1, 1], [0, 0, 1, 0, 0, 0, 0, 0, 0, 0, 0, 0], [0, 0, -1, 0, 0, 0, 0, -1, -1, 0, 0, 0], [0, 0, 1, 0, 0, 0, -1, 0, 0, 0, 0, 0], [0, 0, 0, 0, 0, 0, 1, 0, 0, 0, 0, 0], [0, 0, 0, 0, 0, 1, -1, 0, -1, 0, 0, 0], [0, 1, 0, 0, -1, -1, 0, 0, 0, 0, 0, 0], [0, 1, 0, 0, 0, 0, 0, 0, 0, 0, 0, 0], [0, 1, 0, 1, 0, 0, 0, 0, 0, 0, 0, 0], [0, 0, 0, -1, 0, 0, 0, 0, 0, 0, 0, 0], [1, 1, 0, 0, 0, 0, 1, 0, 0, 0, 0, 0], [1, 0, 1, -1, 0, 0, 0, 0, 0, 0, 0, 0], [0, 0, 0, -1, -1, 0, 0, 1, 0, 0, 0, 0]])
HK = dict(m=2, k=3, n=3,
    a_prog=[(5, 1, 4, 1), (5, -1, 3, 1), (0, 1, 2, -1), (0, 1, 3, -1), (2, 1, 3, -1), (5, -1, 2, 1), (0, 1, 1, -1), (12, 1, 3, -1), (6, -1, 2, 1), (1, 1, 14, 1), (13, 1, 4, 1)],
    a_use=[4, 14, 6, 1, 2, 12, 15, 8, 13, 16, 7, 3, 10, 11, 9],
    c_prog=[(5, -1, 0, 1), (5, 1, 3, 1), (3, 1, 0, 1), (1, 1, 2, -1), (4, -1, 3, 1), (0, 1, 2, 1), (5, 1, 2, 1), (12, -1, 1, 1), (0, 1, 10, 1), (1, -1, 14, 1), (4, 1, 13, 1)],
    c_use=[(4, 1), (13, -1), (16, 1), (1, 1), (12, 1), (15, 1), (9, -1), (11, -1), (14, -1), (10, 1), (7, 1), (8, -1), (6, -1), (5, -1), (0, 1)],
    w=[[0, 0, 0, 1, 1, 0, 0, -1, 0], [0, 0, 0, 0, 0, -1, 0, -1, 0], [0, 0, 0, 0, 0, 0, 0, 1, 0], [0, 1, 0, 0, 1, 1, 0, 0, 0], [0, 0, 1, 0, 0, 0, 0, 1, 1], [0, -1, 0, 0, 0, 0, 0, 0, 0], [0, 0, 0, 0, 0, 1, 0, 0, 0], [0, 0, -1, 0, 0, 0, 0, 0, 0], [0, -1, 0, 1, 0, 0, 0, 0, 0], [0, 0, 0, 1, 0, 0, 0, 0, 0], [0, 0, 0, 0, 0, 0, -1, 0, 0], [-1, -1, 0, 0, 0, 0, -1, 0, 0], [0, 0, -1, 0, 0, 0, -1, 0, 0], [0, 0, 0, 0, 0, -1, -1, 0, 1], [1, 0, -1, 1, 0, 0, 0, 0, 0]])
Sa = dict(m=4, k=3, n=3,
    a_prog=[(1, 1, 3, -1), (2, 1, 6, -1), (9, -1, 3, 1), (7, -1, 5, 1), (3, 1, 10, 1), (0, 1, 14, 1), (17, 1, 2, -1), (9, 1, 18, 1), (4, 1, 1, 1), (20, 1, 5, 1), (10, -1, 20, 1), (21, 1, 10, -1), (7, 1, 22, 1), (5, 1, 8, 1), (6, -1, 25, 1), (11, -1, 25, 1), (6, -1, 27, 1), (3, 1, 7, 1), (29, 1, 4, 1), (0, 1, 1, 1), (6, -1, 31, 1), (2, 1, 7, -1), (8, -1, 33, 1), (16, 1, 28, 1), (35, 1, 14, -1), (11, -1, 23, 1), (18, 1, 37, -1)],
    a_use=[14, 16, 1, 23, 11, 10, 3, 36, 17, 5, 22, 18, 38, 2, 28, 26, 21, 19, 12, 1, 30, 27, 15, 7, 32, 6, 24, 13, 34],
    c_prog=[(8, 1, 0, 1), (9, 1, 7, 1), (4, 1, 7, -1), (4, 1, 10, 1), (2, 1, 5, -1), (11, 1, 5, 1), (6, -1, 3, 1), (4, -1, 1, 1), (11, -1, 1, 1), (14, 1, 11, -1), (18, 1, 8, 1), (16, -1, 0, 1), (15, 1, 9, -1), (24, 1, 19, 1), (23, 1, 17, -1), (15, 1, 21, -1), (3, -1, 23, 1), (24, 1, 28, 1), (9, 1, 3, 1), (30, 1, 22, -1), (0, 1, 7, -1), (32, 1, 6, 1), (8, 1, 2, 1), (1, 1, 34, 1), (21, 1, 17, 1), (22, 1, 36, -1)],
    c_use=[(25, 1), (24, -1), (19, -1), (21, -1), (27, 1), (15, -1), (29, 1), (9, -1), (1, -1), (37, -1), (14, -1), (20, -1), (11, -1), (35, 1), (13, 1), (31, -1), (17, 1), (26, -1), (23, 1), (16, 1), (3, -1), (7, -1), (22, -1), (18, -1), (0, 1), (33, 1), (7, -1), (12, -1), (8, -1)],
    w=[[0, -1, 0, 0, 0, 0, 0, 0, 0], [-1, -1, 0, 1, 0, 0, 0, 0, 0], [0, 0, 0, 0, -1, 0, 0, 0, 0], [0, 0, 0, 0, 0, -1, 0, -1, 1], [0, 0, 0, 0, 0, 0, 0, 1, 0], [1, 1, 0, -1, -1, 0, 0, 0, 0], [-1, 0, 0, 1, 0, 0, 0, 0, 0], [-1, -1, 0, 0, 0, 0, 0, 0, 0], [0, -1, 1, 0, 0, 0, 0, -1, 1], [0, 0, 0, 0, 0, -1, 0, 0, 1], [0, 0, 0, 0, -1, 1, 0, 1, -1], [0, 0, -1, 0, 0, 0, 0, 1, -1], [0, 0, 0, 0, 0, 0, 0, 1, -1], [0, 0, 1, 0, 0, 0, 0, 0, 1], [-1, -1, 0, 0, 0, 0, -1, 0, 0], [0, 0, 0, 0, 0, 0, -1, 0, 0], [0, 0, 0, 0, 0, 1, 0, 0, 0], [0, 0, 1, 0, 0, 0, 0, 0, 0], [-1, 0, -1, 1, 0, 0, 0, 0, 0], [-1, 0, -1, 1, 0, 1, 0, 0, 0], [0, 0, 0, -1, 0, 0, 0, 0, 0], [-1, -1, 0, 0, 0, 0, -1, -1, 0], [0, 0, 0, 0, 0, 1, -1, 0, -1], [0, 0, 0, 1, 0, 1, -1, 0, -1], [1, 0, 1, 0, 0, 0, 0, 0, 0], [1, 0, 0, 0, 0, 0, 1, 0, 0], [0, 0, 0, 0, -1, 0, 0, 0, 0], [0, 0, 1, 0, 0, 0, -1, 0, 0], [0, 0, 0, 0, 0, 0, 1, 0, 1]])
Sb = dict(m=4, k=3, n=3,
    a_prog=[(3, -1, 1, 1), (2, 1, 6, -1), (9, -1, 3, 1), (5, 1, 7, -1), (10, 1, 3, 1), (0, 1, 14, 1), (17, 1, 2, -1), (18, 1, 9, 1), (5, 1, 8, 1), (6, -1, 20, 1), (11, -1, 20, 1), (6, -1, 22, 1), (4, 1, 1, 1), (5, 1, 24, 1), (24, 1, 10, -1), (5, 1, 26, 1), (7, 1, 26, 1), (27, 1, 11, -1), (29, -1, 18, 1), (1, 1, 6, -1), (0, 1, 31, 1), (9, 1, 23, 1), (33, 1, 10, 1), (12, 1, 10, -1), (35, -1, 28, 1), (2, 1, 15, 1), (37, 1, 20, -1)],
    a_use=[7, 3, 36, 15, 5, 6, 21, 38, 13, 32, 2, 19, 12, 16, 1, 23, 25, 34, 14, 11, 10, 1, 27, 26, 22, 28, 18, 17, 30],
    c_prog=[(8, 1, 0, 1), (9, 1, 7, 1), (4, 1, 7, -1), (4, 1, 10, 1), (2, 1, 5, -1), (11, 1, 5, 1), (6, -1, 3, 1), (1, 1, 4, -1), (1, 1, 11, -1), (14, 1, 11, -1), (18, 1, 8, 1), (16, -1, 0, 1), (9, -1, 15, 1), (19, 1, 24, 1), (17, -1, 23, 1), (15, 1, 21, -1), (9, -1, 8, 1), (6, 1, 28, -1), (17, -1, 22, 1), (21, -1, 30, 1), (24, 1, 23, 1), (32, 1, 3, -1), (8, 1, 1, 1), (2, 1, 34, 1), (13, -1, 12, 1), (36, 1, 29, 1)],
    c_use=[(18, -1), (33, -1), (3, -1), (22, 1), (31, 1), (37, -1), (29, 1), (8, -1), (12, 1), (0, -1), (35, 1), (26, -1), (23, 1), (24, 1), (16, 1), (13, -1), (17, 1), (9, 1), (25, 1), (27, -1), (15, -1), (19, -1), (21, 1), (14, 1), (7, 1), (7, -1), (20, 1), (1, 1), (11, 1)],
    w=[[0, 0, 0, 1, 0, 1, -1, 0, -1], [1, 0, 0, -1, 0, 0, 0, 0, 0], [0, 0, 0, -1, 0, 0, 0, 0, 0], [0, 0, 0, 0, 0, -1, 1, 0, 1], [0, 0, 0, 0, 0, 1, 0, 0, -1], [-1, 0, 0, 0, 0, 0, -1, 0, 0], [0, 0, 0, 0, 0, 0, 1, 0, 0], [0, 0, 0, 0, 0, 0, 1, 0, 1], [0, 0, -1, 0, 0, 0, 1, 0, 0], [-1, 0, -1, 0, 0, 0, 0, 0, 0], [0, 0, 1, 0, 0, 0, 0, 0, 1], [0, 0, 1, 0, 0, 0, 0, 0, 0], [-1, 0, -1, 1, 0, 0, 0, 0, 0], [1, 1, 0, -1, 0, 0, 0, 0, 0], [-1, 0, -1, 1, 0, 1, 0, 0, 0], [1, 1, 0, 0, 0, 0, 1, 0, 0], [0, 0, 0, 0, 0, 1, 0, 0, 0], [1, 1, 0, 0, 0, 0, 0, 0, 0], [0, -1, 0, 0, 0, 0, 0, 0, 0], [0, 0, 0, 0, 0, 0, 0, -1, 0], [1, 1, 0, -1, -1, 0, 0, 0, 0], [0, 0, 0, 0, -1, 0, 0, 0, 0], [0, 0, 0, 0, 0, 1, 0, 1, -1], [0, 0, 0, 0, 1, -1, 0, -1, 1], [1, 1, 0, 0, 0, 0, 1, 1, 0], [0, 0, 0, 0, -1, 0, 0, 0, 0], [0, 0, 1, 0, 0, 0, 0, -1, 1], [0, 1, -1, 0, 0, 0, 0, 1, -1], [0, 0, 0, 0, 0, 0, 0, -1, 1]])
Sc = dict(m=4, k=3, n=3,
    a_prog=[(1, 1, 3, -1), (10, -1, 3, 1), (2, 1, 6, 1), (5, 1, 7, 1), (9, 1, 3, 1), (16, 1, 0, 1), (2, -1, 17, 1), (9, -1, 18, 1), (4, 1, 1, 1), (20, 1, 10, 1), (20, 1, 5, 1), (7, -1, 21, 1), (22, 1, 10, 1), (8, -1, 5, 1), (11, 1, 25, 1), (6, 1, 25, 1), (11, 1, 27, 1), (28, 1, 10, -1), (29, 1, 9, -1), (2, 1, 7, 1), (8, 1, 31, 1), (23, 1, 12, -1), (10, -1, 33, 1), (6, 1, 0, 1), (1, 1, 35, 1), (24, -1, 18, 1), (37, 1, 11, -1)],
    a_use=[15, 30, 27, 34, 5, 7, 6, 32, 3, 2, 14, 12, 19, 36, 28, 1, 13, 16, 10, 11, 18, 22, 38, 1, 17, 23, 24, 26, 21],
    c_prog=[(4, 1, 7, 1), (7, 1, 9, -1), (11, -1, 5, 1), (5, -1, 2, 1), (6, 1, 3, 1), (4, 1, 10, -1), (4, -1, 1, 1), (8, -1, 0, 1), (11, 1, 1, 1), (9, -1, 17, 1), (8, -1, 16, 1), (15, -1, 0, 1), (11, 1, 12, 1), (23, 1, 14, -1), (17, -1, 24, 1), (18, 1, 21, 1), (9, 1, 22, 1), (3, -1, 28, 1), (6, 1, 7, 1), (30, -1, 0, 1), (22, 1, 24, -1), (14, -1, 32, 1), (23, 1, 3, -1), (21, -1, 34, 1), (20, 1, 19, 1), (36, 1, 25, -1)],
    c_use=[(22, 1), (9, -1), (29, -1), (3, 1), (33, -1), (16, -1), (31, -1), (8, 1), (35, 1), (37, 1), (19, -1), (23, -1), (25, -1), (0, 1), (13, 1), (15, 1), (21, -1), (27, -1), (17, -1), (26, 1), (20, -1), (14, 1), (11, 1), (18, 1), (1, -1), (7, -1), (24, -1), (7, 1), (12, -1)],
    w=[[0, 0, 0, 0, 0, -1, 1, 0, 1], [1, -1, 0, 0, 0, 0, 0, 0, 0], [0, 0, 0, 0, 0, 0, 1, 0, 0], [0, 0, 0, 1, 0, 0, 0, 0, 0], [0, 0, 0, 0, 0, -1, 0, 0, 1], [0, 0, 0, -1, 0, -1, 1, 0, 1], [1, 0, 0, 0, 0, 0, 1, 0, 0], [0, 0, 0, 0, 0, 0, 1, 0, 1], [-1, 0, 0, 1, 0, 0, 0, 0, 0], [0, 0, 1, 0, 0, 0, 0, 0, 1], [0, 0, 1, 0, 0, 0, -1, 0, 0], [1, 0, 1, -1, 0, 0, 0, 0, 0], [0, 0, 1, 0, 0, 0, 0, 0, 0], [1, 0, 1, 0, 0, 0, 0, 0, 0], [-1, 1, 0, 0, 0, 0, -1, 0, 0], [-1, 0, -1, 1, 0, 1, 0, 0, 0], [1, -1, 0, -1, 0, 0, 0, 0, 0], [0, 1, 0, 0, 0, 0, 0, 0, 0], [1, -1, 0, -1, 1, 0, 0, 0, 0], [0, 0, 0, 0, 0, 0, 0, 1, 0], [0, 0, -1, 0, 0, 0, 0, 1, -1], [0, 0, 0, 0, 0, 1, 0, 0, 0], [0, 0, 0, 0, 0, 0, 0, 1, -1], [0, 0, 0, 0, 1, 0, 0, 0, 0], [0, -1, 1, 0, 0, 0, 0, -1, 1], [0, 0, 0, 0, 1, 0, 0, 0, 0], [0, 0, 0, 0, 0, -1, 0, -1, 1], [1, -1, 0, 0, 0, 0, 1, -1, 0], [0, 0, 0, 0, -1, 1, 0, 1, -1]])
Sd = dict(m=4, k=3, n=3,
    a_prog=[(10, -1, 3, 1), (6, -1, 3, 1), (3, 1, 7, -1), (5, -1, 1, 1), (11, -1, 0, 1), (9, -1, 13, 1), (11, -1, 17, 1), (6, 1, 18, 1), (10, -1, 4, 1), (5, 1, 20, 1), (7, -1, 20, 1), (21, 1, 7, -1), (22, 1, 1, 1), (2, 1, 5, 1), (8, -1, 25, 1), (0, 1, 25, 1), (8, -1, 27, 1), (1, 1, 12, -1), (29, 1, 20, 1), (2, 1, 11, 1), (1, 1, 31, 1), (8, -1, 23, 1), (33, 1, 18, 1), (28, 1, 13, 1), (14, -1, 35, 1), (12, 1, 19, -1), (16, 1, 37, 1)],
    a_use=[1, 5, 32, 15, 27, 0, 30, 3, 11, 16, 12, 19, 38, 23, 10, 14, 21, 13, 8, 7, 10, 22, 24, 18, 34, 36, 17, 26, 28],
    c_prog=[(4, 1, 7, 1), (0, 1, 3, -1), (4, 1, 10, 1), (2, 1, 9, 1), (10, 1, 8, 1), (5, 1, 8, 1), (5, 1, 11, 1), (4, -1, 1, 1), (6, -1, 1, 1), (18, 1, 9, 1), (2, 1, 13, 1), (6, 1, 12, 1), (8, 1, 19, 1), (23, 1, 14, -1), (24, 1, 12, 1), (17, 1, 21, -1), (2, 1, 10, -1), (28, 1, 11, -1), (22, 1, 24, 1), (30, 1, 17, -1), (23, 1, 21, 1), (32, 1, 3, 1), (2, 1, 0, 1), (34, 1, 6, 1), (0, 1, 1, 1), (36, 1, 9, -1)],
    c_use=[(13, -1), (31, -1), (2, -1), (22, -1), (35, 1), (37, 1), (3, 1), (33, 1), (29, 1), (15, 1), (21, 1), (27, 1), (9, -1), (24, -1), (18, 1), (23, -1), (17, -1), (25, 1), (26, -1), (12, -1), (14, 1), (19, -1), (1, -1), (16, 1), (8, 1), (6, -1), (10, 1), (1, 1), (20, -1)],
    w=[[0, 0, 0, -1, 0, 1, 1, 0, -1], [0, 0, 0, 0, 0, -1, 0, 0, 1], [0, 0, 0, 0, 0, 0, 1, 0, -1], [0, 0, 0, 0, 0, -1, -1, 0, 1], [0, 0, 0, 0, 0, 0, 1, 0, 0], [1, 0, 0, 0, 0, 0, -1, 0, 0], [0, 0, 0, 1, 0, 0, 0, 0, 0], [1, 0, 0, 1, 0, 0, 0, 0, 0], [0, 0, 1, 0, 0, 0, 0, 0, -1], [0, 0, 1, 0, 0, 0, -1, 0, 0], [-1, 0, 1, -1, 0, 0, 0, 0, 0], [0, 0, 1, 0, 0, 0, 0, 0, 0], [-1, 0, 1, 0, 0, 0, 0, 0, 0], [0, 0, 0, 0, 0, 1, 0, 1, -1], [-1, 0, 1, -1, 0, 1, 0, 0, 0], [1, -1, 0, 1, 0, 0, 0, 0, 0], [0, 0, 0, 0, 0, -1, 0, 0, 0], [0, -1, 0, 0, 0, 0, 0, 0, 0], [0, 0, 0, 0, 0, 0, 0, -1, 0], [1, -1, 0, 1, -1, 0, 0, 0, 0], [0, 0, 0, 0, 1, 0, 0, 0, 0], [0, 0, 0, 0, 1, -1, 0, -1, 1], [0, 0, 0, 0, -1, 0, 0, 0, 0], [0, 0, -1, 0, 0, 0, 0, -1, 1], [0, 0, 0, 0, 0, 0, 0, 1, -1], [1, -1, 0, 0, 0, 0, 0, 0, 0], [0, -1, 1, 0, 0, 0, 0, 1, -1], [1, -1, 0, 0, 0, 0, -1, 1, 0], [1, -1, 0, 0, 0, 0, -1, 0, 0]])
H2 = dict(m=2, k=3, n=3,
    a_prog=[(5, 1, 4, 1), (5, -1, 3, 1), (2, -1, 0, 1), (3, -1, 0, 1), (3, -1, 2, 1), (5, -1, 2, 1), (1, -1, 0, 1), (9, 1, 1, -1), (11, 1, 4, -1), (14, 1, 1, 1), (4, 1, 13, 1)],
    a_use=[3, 13, 16, 12, 7, 4, 6, 14, 15, 1, 2, 8, 9, 10, 11],
    c_prog=[(0, 1, 5, -1), (5, 1, 3, 1), (0, 1, 3, 1), (1, 1, 2, -1), (4, -1, 3, 1), (0, 1, 2, 1), (5, 1, 2, 1), (5, -1, 9, 1), (8, 1, 4, -1), (14, 1, 1, -1), (4, 1, 13, 1)],
    c_use=[(8, 1), (14, -1), (10, -1), (15, 1), (7, 1), (4, -1), (16, -1), (13, 1), (9, 1), (1, 1), (12, 1), (11, 1), (0, -1), (6, 1), (5, 1)],
    w=[[1, 1, 0, 0, 0, 0, 1, 0, 0], [0, -1, 0, 1, 0, 0, 0, 0, 0], [0, 0, 0, -1, 0, 0, 0, 0, 0], [0, -1, 0, 0, 0, 0, 0, 0, 0], [0, 0, 0, 0, 0, 0, -1, 0, 0], [0, 0, 0, -1, -1, 0, 0, 1, 0], [0, 0, 0, 0, 0, 0, 0, -1, 0], [0, 0, 0, 0, 0, 1, 0, 1, 0], [0, 0, 0, 0, 0, -1, 0, 0, 0], [0, 1, 0, 0, 1, 1, 0, 0, 0], [0, 0, 1, 0, 0, 0, 0, 1, 1], [0, 0, 1, 0, 0, 0, 0, 0, 0], [-1, 0, 1, -1, 0, 0, 0, 0, 0], [0, 0, 1, 0, 0, 0, 1, 0, 0], [0, 0, 0, 0, 0, 1, 1, 0, -1]])
H3 = dict(m=2, k=3, n=3,
    a_prog=[(5, 1, 4, 1), (5, -1, 3, 1), (0, 1, 2, -1), (0, 1, 3, -1), (2, 1, 3, -1), (5, -1, 2, 1), (0, 1, 1, -1), (9, 1, 1, -1), (4, -1, 11, 1), (1, 1, 14, 1), (4, 1, 13, 1)],
    a_use=[1, 12, 13, 16, 4, 6, 3, 7, 14, 15, 2, 8, 9, 10, 11],
    c_prog=[(5, -1, 0, 1), (3, 1, 5, 1), (3, 1, 0, 1), (2, -1, 1, 1), (3, 1, 4, -1), (2, 1, 0, 1), (2, 1, 5, 1), (5, -1, 9, 1), (10, 1, 0, 1), (1, -1, 14, 1), (13, 1, 4, 1)],
    c_use=[(1, -1), (15, 1), (14, -1), (10, 1), (4, -1), (16, 1), (8, -1), (7, 1), (13, -1), (9, -1), (12, 1), (11, 1), (0, 1), (6, -1), (5, 1)],
    w=[[0, -1, 0, 0, -1, -1, 0, 0, 0], [0, -1, 0, 0, 0, 0, 0, 0, 0], [0, -1, 0, 1, 0, 0, 0, 0, 0], [0, 0, 0, 1, 0, 0, 0, 0, 0], [0, 0, 0, -1, -1, 0, 0, 1, 0], [0, 0, 0, 0, 0, 0, 0, 1, 0], [-1, -1, 0, 0, 0, 0, -1, 0, 0], [0, 0, 0, 0, 0, 0, -1, 0, 0], [0, 0, 0, 0, 0, -1, 0, -1, 0], [0, 0, 0, 0, 0, 1, 0, 0, 0], [0, 0, 1, 0, 0, 0, 0, 1, 1], [0, 0, 1, 0, 0, 0, 0, 0, 0], [1, 0, -1, 1, 0, 0, 0, 0, 0], [0, 0, -1, 0, 0, 0, -1, 0, 0], [0, 0, 0, 0, 0, 1, 1, 0, -1]])

Se = {'m': 4, 'k': 3, 'n': 3, 'a_prog': [(10, -1, 3, 1), (6, -1, 3, 1), (3, 1, 7, -1), (5, -1, 1, 1), (11, -1, 0, 1), (9, -1, 13, 1), (11, -1, 17, 1), (6, 1, 18, 1), (10, -1, 4, 1), (5, 1, 20, 1), (7, -1, 20, 1), (21, 1, 7, -1), (22, 1, 1, 1), (2, 1, 5, 1), (8, -1, 25, 1), (0, 1, 25, 1), (8, -1, 27, 1), (1, 1, 12, -1), (29, 1, 20, 1), (2, 1, 11, 1), (1, 1, 31, 1), (8, -1, 23, 1), (33, 1, 18, 1), (28, 1, 13, 1), (14, -1, 35, 1), (12, 1, 19, -1), (16, 1, 37, 1)], 'a_use': [5, 27, 32, 15, 0, 1, 30, 3, 16, 11, 12, 19, 38, 10, 14, 21, 13, 23, 8, 7, 10, 22, 18, 34, 24, 17, 26, 28, 36], 'c_prog': [(4, 1, 7, 1), (0, 1, 3, -1), (4, 1, 10, 1), (2, 1, 9, 1), (10, 1, 8, 1), (5, 1, 8, 1), (5, 1, 11, 1), (4, -1, 1, 1), (6, -1, 1, 1), (18, 1, 9, 1), (2, 1, 13, 1), (6, 1, 12, 1), (8, 1, 19, 1), (23, 1, 14, -1), (24, 1, 12, 1), (17, 1, 21, -1), (2, 1, 10, -1), (28, 1, 11, -1), (22, 1, 24, 1), (30, 1, 17, -1), (23, 1, 21, 1), (32, 1, 3, 1), (2, 1, 0, 1), (34, 1, 6, 1), (0, 1, 1, 1), (36, 1, 9, -1)], 'c_use': [(31, 1), (35, 1), (2, 1), (22, -1), (37, 1), (13, -1), (3, -1), (33, 1), (15, -1), (29, 1), (21, 1), (27, 1), (9, 1), (18, 1), (23, -1), (17, 1), (25, 1), (24, -1), (26, -1), (12, 1), (14, -1), (19, -1), (16, 1), (8, -1), (1, 1), (10, -1), (1, -1), (20, 1), (6, -1)], 'w': [[0, 0, 0, 0, 0, 1, 0, 0, -1], [0, 0, 0, 0, 0, 0, 1, 0, 0], [0, 0, 0, 0, 0, 0, -1, 0, 1], [0, 0, 0, 0, 0, -1, -1, 0, 1], [1, 0, 0, 0, 0, 0, -1, 0, 0], [0, 0, 0, -1, 0, 1, 1, 0, -1], [0, 0, 0, -1, 0, 0, 0, 0, 0], [1, 0, 0, 1, 0, 0, 0, 0, 0], [0, 0, -1, 0, 0, 0, 1, 0, 0], [0, 0, 1, 0, 0, 0, 0, 0, -1], [-1, 0, 1, -1, 0, 0, 0, 0, 0], [0, 0, 1, 0, 0, 0, 0, 0, 0], [1, 0, -1, 0, 0, 0, 0, 0, 0], [-1, 0, 1, -1, 0, 1, 0, 0, 0], [1, -1, 0, 1, 0, 0, 0, 0, 0], [0, 0, 0, 0, 0, 1, 0, 0, 0], [0, -1, 0, 0, 0, 0, 0, 0, 0], [0, 0, 0, 0, 0, 1, 0, 1, -1], [0, 0, 0, 0, 0, 0, 0, -1, 0], [-1, 1, 0, -1, 1, 0, 0, 0, 0], [0, 0, 0, 0, -1, 0, 0, 0, 0], [0, 0, 0, 0, 1, -1, 0, -1, 1], [0, 0, -1, 0, 0, 0, 0, -1, 1], [0, 0, 0, 0, 0, 0, 0, -1, 1], [0, 0, 0, 0, 1, 0, 0, 0, 0], [0, 1, -1, 0, 0, 0, 0, -1, 1], [-1, 1, 0, 0, 0, 0, 1, -1, 0], [-1, 1, 0, 0, 0, 0, 1, 0, 0], [1, -1, 0, 0, 0, 0, 0, 0, 0]]}


def lhs_operands(sc, block):
    m, k = sc["m"], sc["k"]
    memo, packed = {}, {}

    def node(v):
        if v not in memo:
            if v < m * k:
                memo[v] = (1, block(v // k, v % k))
            else:
                a, sa, b, sb = sc["a_prog"][v - m * k]
                (ta, xa), (tb, xb) = node(a), node(b)
                ta, tb = ta * sa, tb * sb
                memo[v] = (ta, xa + xb) if ta == tb else (1, xa - xb if ta > 0 else xb - xa)
        return memo[v]

    def op(p):
        v = sc["a_use"][p]
        if v not in packed:
            packed[v] = node(v)[1].astype(BF16)
        return packed[v]
    return op


def combine(sc, product, emit):
    m, n = sc["m"], sc["n"]
    fan = [0] * (m * n + len(sc["c_prog"]))
    for v, _ in sc["c_use"]:
        fan[v] += 1
    for a, _, b, _ in sc["c_prog"]:
        fan[a] += 1
        fan[b] += 1
    val = {}

    def push(v, t, x):
        if v in val:
            u, y = val[v]
            t, x = (t, y + x) if t == u else (1, x - y if t > 0 else y - x)
        val[v] = (t, x)
        fan[v] -= 1
        if fan[v] == 0:
            del val[v]
            if v >= m * n:
                a, sa, b, sb = sc["c_prog"][v - m * n]
                push(a, t * sa, x)
                push(b, t * sb, x)
            else:
                assert t == 1
                emit(v // n, v % n, x)

    for p, (v, t) in enumerate(sc["c_use"]):
        push(v, t, product(p))


def weight_form(sc, p, tile):
    n, acc = sc["n"], None
    for q in sorted(range(len(sc["w"][p])), key=lambda q: -sc["w"][p][q]):
        c = sc["w"][p][q]
        if c:
            v = tile(q // n, q % n)
            acc = (v if c > 0 else -v) if acc is None else (acc + v if c > 0 else acc - v)
    return acc


def make(CH=768, G1=4, G2=2, S=52, XC=8, XR2=4, MC1=48, MC2=48, mode2="k", vmem_mb=128, flags=None, E1=2, E2=2,
         run1=True, run2=True, dma=True, comp=True, pipe=True, YB=0, YD=0, LNR=16, F0=0.0, F1=0.65, F2=0.68, F3=0.97, sc1='S433', sc2='HK', rs=1, PX=0, PH=0, PO=0, A1=1, B1=1, A2=1, B2=1):
    sc1, sc2 = (dict(S433=S433, S343=S343, HK=HK, Sa=Sa, Sb=Sb, Sc=Sc, Sd=Sd, H2=H2, H3=H3, Se=Se)[z] if isinstance(z, str) else z for z in (sc1, sc2))
    NP1, NP2 = len(sc1["w"]), len(sc2["w"])
    PR = sc1["m"] * MC1
    KG2 = 12 // sc2["k"]
    TM1, TM2 = CH * G1, CH * G2
    XT = max(XC * CH, XR2 * TM2)
    W1ROW = (XT - HID - PR) // CH * CH

    @jax.jit
    def fn(x, dw, w1, w2, grn_g, grn_b):
        B, H, W, _ = x.shape
        N = B * H * W
        NT1, NT2 = N // TM1, N // TM2
        NCH = N // CH
        NHC = NCH - S
        R1 = -(-NHC * 65536 // (NT1 - E1))
        R2 = -(-NHC * 65536 // (NT2 - E2))
        assert R1 <= G1 * 65536 and R2 <= G2 * 65536 and S >= 2 * max(G1, G2) and TM1 >= HID and E1 >= 2 and E2 >= 2
        last = [(NCH - G1 + u) % XC for u in range(G1)]
        W2U, W2S = next((u, s0) for u in range(G1) for s0 in range(XC - 1)
                        if all(t not in last[u + 1:] for t in (s0, s0 + 1)))
        W2ROW = W2S * CH
        assert 2 * CH >= HID and XC >= G1

        def kernel(x_hbm, dw_ref, w1_hbm, w2_hbm, g_ref, b_ref, out_hbm, h_hbm,
                   xbuf, hbuf, ws, ssq, opbuf, ybuf, xsem, osem, hsem, wsem):
            class _Nop:
                def start(self, priority=0): pass
                def wait(self): pass
            mk = pltpu.make_async_copy if dma else (lambda *a: _Nop())

            def xrows(slot, tm):
                return xbuf.at[pl.ds(pl.multiple_of(slot * tm, tm), tm)]

            def x_copy(i, slot, tm):
                return mk(x_hbm.at[pl.ds(i * tm, tm)], xrows(slot, tm), xsem.at[slot])

            def o_copy(i, slot):
                return mk(xrows(slot, TM2), out_hbm.at[pl.ds(i * TM2, TM2)], osem.at[slot])

            def h_out(c, slot):
                return mk(hbuf.at[slot], h_hbm.at[c], hsem.at[slot])

            def h_in(c, slot):
                return mk(h_hbm.at[c], hbuf.at[slot], hsem.at[slot])

            def w1_copy(q):
                return pltpu.make_async_copy(w1_hbm.at[:, pl.ds(q * C, C)], xbuf.at[pl.ds(W1ROW + q * C, C)], wsem.at[q])

            def w2_copy():
                return pltpu.make_async_copy(w2_hbm, xbuf.at[pl.ds(W2ROW, HID)], wsem.at[0])

            def wrap(v, n):
                return jnp.where(v >= n, v - n, v)

            def wrapn(v, n):
                return jnp.where(v < 0, v + n, v)

            def x0_copy():
                return pltpu.make_async_copy(x_hbm.at[pl.ds(0, PR)], xbuf.at[pl.ds(W1ROW + HID, PR)], osem.at[0])

            for q in range(4):
                w1_copy(q).start()
            x0_copy().start()
            ssq[...] = jnp.zeros_like(ssq)
            dwv = dw_ref[...].astype(F32)
            NPRE = W1ROW // CH
            for c in range(NPRE):
                pltpu.make_async_copy(x_hbm.at[pl.ds(c * CH + PR, CH)], xbuf.at[pl.ds(c * CH, CH)], xsem.at[c]).start() if dma else None
            for q in range(4):
                w1_copy(q).wait()

            def w1_tile(k, n):
                r = W1ROW + (n // 3) * C + k * L
                return xbuf[r:r + L, (n % 3) * L:(n % 3 + 1) * L].astype(F32)

            for c in range(4):
                for p in range(NP1):
                    ws[p * 4 + c] = pk(weight_form(sc1, p, lambda k, j: w1_tile(k, 4 * j + c)))

            def layernorm(row):
                y = xbuf[pl.ds(pl.multiple_of(row, 16), LNR), :].astype(F32) * dwv
                mu = jnp.sum(y, axis=-1, keepdims=True) * (1.0 / C)
                d = y - mu
                ss = jnp.sum(d * d, axis=-1, keepdims=True)
                v = ss * (1.0 / (C * ALPHA * ALPHA)) + 1e-5 / (ALPHA * ALPHA)
                if rs == 0:
                    return d * lax.rsqrt(v)
                return d * jnp.exp2(-0.5 * jnp.log2(v))

            def act(y, hs, r0, c):
                t = jnp.tanh(y * (y * y + C0))
                h = y * t + y
                ssq[:, c * L:(c + 1) * L] += jnp.sum((h * h).reshape(MC1 // 8, 8, L), axis=0)
                hbuf[hs, pl.ds(r0 // 2, MC1 // 2), c * L:(c + 1) * L] = pack16(h)

            def operands(row):
                nl = MC1 // LNR
                a = {}
                def ln(t, q):
                    a[t, q] = layernorm(row + t * MC1 + q * LNR)
                op = lhs_operands(sc1, lambda t, k: jnp.concatenate([a[t, q][:, k * L:(k + 1) * L] for q in range(nl)], axis=0))
                lns = [functools.partial(ln, t, q) for t in range(sc1["m"]) for q in range(nl)]
                forms = [functools.partial(op, p) for p in range(NP1)]
                return op, lns, forms

            NB1 = TM1 // (PR)

            PPC = CH // PR

            def xc_copy(c, slot, n=CH):
                return mk(x_hbm.at[pl.ds(c * CH + PR, n)], xbuf.at[pl.ds(pl.multiple_of(slot * CH, CH), n)], xsem.at[slot])

            def xc_do(c, slot, what):
                @pl.when(c < NCH - 1)
                def _():
                    what(xc_copy(c, slot))
                @pl.when(c == NCH - 1)
                def _():
                    what(xc_copy(c, slot, CH - PR))

            def stage(row):
                op, lns, _ = operands(row)
                for f in lns:
                    f()
                for p in range(NP1):
                    opbuf[p] = op(p)

            def phase1(i, carry):
                xb, hb, q, qs = carry
                slots = [wrap(hb + u, S) for u in range(G1)]
                xsl = [wrap(xb + u, XC) for u in range(G1)]
                qn = jnp.minimum((i * R1) >> 16, NHC)
                for u in range(G1):
                    xc_do(i * G1 + u, xsl[u], lambda cp: cp.wait())
                    @pl.when(i * G1 + u >= S)
                    def _():
                        h_out(i * G1 + u - S, slots[u]).wait()
                for u in range(G1):
                    @pl.when(q + u < qn)
                    def _():
                        h_out(q + u, wrap(qs + u, S)).start()

                nxt = None
                parked = []
                park_product = lambda f: f
                def flush():
                    b, t, j, hs, r0, col = parked.pop(0)
                    act(ybuf[b, t * 3 + j], hs, r0, col)
                for m in range(NB1 if comp else 0):
                    u, r = divmod(m * PR, CH)
                    op = (lambda p: opbuf[p]) if m == 0 else nxt
                    nxt, lns, forms = operands(xsl[u] * CH + r)
                    if m == NB1 - 1:
                        def put(p):
                            opbuf[p] = nxt(p)
                        forms = [functools.partial(put, p) for p in range(NP1)]
                    ns = 4 * NP1
                    todo = {}
                    for e, f in enumerate(lns):
                        todo.setdefault(int(ns * (F0 + (F1 - F0) * e / len(lns))), []).append(f)
                    for e, f in enumerate(forms):
                        todo.setdefault(int(ns * (F2 + (F3 - F2) * e / len(forms))), []).append(f)
                    for c in range(4):
                        def product(p):
                            for f in todo.pop(c * NP1 + p, []):
                                f()
                            return jnp.dot(op(p), upk(ws[p * 4 + c]), preferred_element_type=F32)
                        if YB == 0:
                            combine(sc1, product, lambda t, j, y: act(y, slots[u], r + t * MC1, 4 * j + c))
                        else:
                            def park(t, j, y):
                                ybuf[c % YB, t * 3 + j] = y
                                parked.append((c % YB, t, j, slots[u], r + t * MC1, 4 * j + c))
                                while len(parked) > YD:
                                    flush()
                            combine(sc1, park_product(product), park)
                    assert not todo
                    if (m + 1) % PPC == 0:
                        xc_do(i * G1 + u + XC, xsl[u], lambda cp: cp.start())
                        if u == W2U:
                            @pl.when(i == NT1 - 1)
                            def _():
                                w2_copy().start()
                while parked:
                    flush()
                return wrap(xb + G1, XC), wrap(hb + G1, S), qn, wrap(qs + (qn - q), S)

            z = jnp.int32(0)
            x0_copy().wait()
            stage(W1ROW + HID)
            for c in range(NPRE, XC):
                xc_copy(c, c).start()
            if run1:
                lax.fori_loop(0, NT1, phase1, (z, z, z, z))
            else:
                for c in range(XC):
                    xc_copy(c, c).wait()
                w2_copy().start()

            free2 = [s for s in range(XR2) if (s + 1) * TM2 <= W2ROW or s * TM2 >= W2ROW + HID]
            first2 = [(j, (NT2 - 1 - j) % XR2) for j in range(XR2 - 1)]
            if run2:
                for j, s in first2:
                    if s in free2:
                        x_copy(NT2 - 1 - j, s, TM2).start()
            gx = jnp.sqrt(jnp.sum(ssq[...], axis=0, keepdims=True) * (HS * HS) + 1e-6)
            nx = gx / (jnp.mean(gx, axis=-1, keepdims=True) + 1e-6)
            sc = (g_ref[...].astype(F32) * nx + 1.0) * HS
            w2_copy().wait()
            for r in range(KG2):
                cols = [jnp.broadcast_to(sc[:, (KG2 * k + r) * L:(KG2 * k + r + 1) * L], (L, L)).T for k in range(sc2["k"])]
                tile = lambda k, j: xbuf[W2ROW + (KG2 * k + r) * L:W2ROW + (KG2 * k + r + 1) * L, j * L:(j + 1) * L].astype(F32) * cols[k]
                for p in range(NP2):
                    ws[p * KG2 + r] = pk(weight_form(sc2, p, tile))
            bias = jnp.dot(jnp.broadcast_to(b_ref[...], (16, HID)), xbuf[W2ROW:W2ROW + HID, :], preferred_element_type=F32)[0:1]
            if run2:
                for j, s in first2:
                    if s not in free2:
                        x_copy(NT2 - 1 - j, s, TM2).start()

            def phase2(j, carry):
                xs, hb, q, qs = carry
                i = NT2 - 1 - j
                slots = [wrap(hb + u, S) for u in range(G2)]
                qn = jnp.minimum((j * R2) >> 16, NHC)
                nxs, nhb = wrapn(xs - 1, XR2), wrapn(hb - G2, S)

                s2 = wrap(xs + 2, XR2)
                x_copy(i, xs, TM2).wait()
                for u in range(G2):
                    @pl.when(i * G2 + u < NHC)
                    def _():
                        h_in(i * G2 + u, slots[u]).wait()
                @pl.when(j >= 2)
                def _():
                    o_copy(i + 2, s2).wait()
                @pl.when(j >= 1)
                def _():
                    o_copy(i + 1, wrap(xs + 1, XR2)).start(priority=PO)
                @pl.when(jnp.logical_and(j >= 1, i + 2 - XR2 >= 0))
                def _():
                    x_copy(i + 2 - XR2, s2, TM2).start(priority=PX)

                NB2 = TM2 // (sc2['m'] * MC2)
                for m in range(NB2):
                    if m == A2:
                        for u in range(G2):
                            @pl.when(q + u < qn)
                            def _():
                                h_in(NHC - 1 - q - u, wrapn(qs - u, S)).start(priority=PH)
                    if not comp:
                        continue
                    r0 = [(sc2['m'] * m + t) * MC2 for t in range(sc2['m'])]
                    def emit(t, jj, o):
                        cs = slice(jj * L, (jj + 1) * L)
                        rows = pl.ds(pl.multiple_of(xs * TM2 + r0[t], 16), MC2)
                        xbuf[rows, cs] = (o + bias[:, cs] + xbuf[rows, cs].astype(F32)).astype(BF16)
                    hload = lambda t, c0, n: unpack16(hbuf[slots[r0[t] // CH], pl.ds(r0[t] % CH // 2, MC2 // 2), c0:c0 + n])
                    if mode2 == "k":
                        acc = {}
                        for r in range(KG2):
                            op = lhs_operands(sc2, lambda t, k: hload(t, (KG2 * k + r) * L, L))
                            def accum(t, jj, o):
                                acc[t, jj] = o if r == 0 else acc[t, jj] + o
                                if r == KG2 - 1:
                                    emit(t, jj, acc[t, jj])
                            combine(sc2, lambda p: jnp.dot(op(p), upk(ws[p * KG2 + r]), preferred_element_type=F32), accum)
                    else:
                        op = lhs_operands(sc2, lambda t, k: hload(t, k * KG2 * L, KG2 * L))
                        combine(sc2, lambda p: jnp.dot(op(p), upk(jnp.concatenate([ws[p * KG2 + c] for c in range(KG2)], axis=0)), preferred_element_type=F32), emit)
                return nxs, nhb, qn, wrapn(qs - (qn - q), S)

            if run2:
                lax.fori_loop(0, NT2, phase2, (z + (NT2 - 1) % XR2, z + (NCH - G2) % S, z, z + (NHC - 1) % S))
                o_copy(0, 0).start()
                o_copy(1, 1 % XR2).wait()
                o_copy(0, 0).wait()

        out, _ = pl.pallas_call(
            kernel,
            in_specs=[pl.BlockSpec(memory_space=pl.ANY), pl.BlockSpec(memory_space=pltpu.VMEM),
                      pl.BlockSpec(memory_space=pl.ANY), pl.BlockSpec(memory_space=pl.ANY),
                      pl.BlockSpec(memory_space=pltpu.VMEM), pl.BlockSpec(memory_space=pltpu.VMEM)],
            out_specs=[pl.BlockSpec(memory_space=pl.ANY)] * 2,
            out_shape=[jax.ShapeDtypeStruct((N, C), BF16), jax.ShapeDtypeStruct((NHC, CH // 2, HID), U32)],
            scratch_shapes=[
                pltpu.VMEM((XT, C), BF16),
                pltpu.VMEM((S, CH // 2, HID), U32),
                pltpu.VMEM((max(NP1 * 4, NP2 * KG2), L // 2, L), U32),
                pltpu.VMEM((8, HID), F32),
                pltpu.VMEM((NP1, MC1, L), BF16),
                pltpu.VMEM((max(YB, 1), 3 * sc1['m'], MC1 if YB else 8, L), F32),
                pltpu.SemaphoreType.DMA((max(XC, XR2),)),
                pltpu.SemaphoreType.DMA((XR2,)),
                pltpu.SemaphoreType.DMA((S,)),
                pltpu.SemaphoreType.DMA((4,)),
            ],
            compiler_params=pltpu.CompilerParams(vmem_limit_bytes=vmem_mb * 1024 * 1024, flags=flags),
        )(x.reshape(N, C), dw.reshape(1, C), w1, w2, grn_g.reshape(1, HID), grn_b.reshape(1, HID))
        return out.reshape(x.shape)
    return fn


pallas_standalone__modern_conv_block_slak__vision_kernel = make(S=53,E1=3,E2=3,MC1=48,sc1='HK')
```

```python
import functools
import numpy as np
import jax
import jax.numpy as jnp
from jax import lax
import jax.experimental.pallas as pl
import jax.experimental.pallas.tpu as pltpu

C = 384
HID = 1536
L = 128
F32 = jnp.float32
BF16 = jnp.bfloat16
U32 = jnp.uint32
pk = lambda v: pltpu.bitcast(v.astype(BF16), U32)
upk = lambda v: pltpu.bitcast(v, BF16)


def pack16(v):
    t = v.shape[0] // 16
    lo = jnp.concatenate([v[16 * g:16 * g + 8] for g in range(t)], axis=0)
    hi = jnp.concatenate([v[16 * g + 8:16 * g + 16] for g in range(t)], axis=0)
    return pltpu.pack_elementwise([lo, hi], packed_dtype=BF16)


def unpack16(w):
    lo = pltpu.unpack_elementwise(w, index=0, packed_dtype=BF16, unpacked_dtype=F32)
    hi = pltpu.unpack_elementwise(w, index=1, packed_dtype=BF16, unpacked_dtype=F32)
    parts = []
    for g in range(w.shape[0] // 8):
        parts += [lo[8 * g:8 * g + 8], hi[8 * g:8 * g + 8]]
    return jnp.concatenate(parts, axis=0)
K0 = float(np.sqrt(2.0 / np.pi))
ALPHA = float((K0 * 0.044715) ** (1.0 / 3.0))
C0 = K0 / ALPHA
HS = 0.5 / ALPHA

S433 = dict(m=4, k=3, n=3,
    a_prog=[(3, -1, 1, 1), (10, -1, 3, 1), (2, 1, 6, 1), (5, 1, 7, 1), (3, 1, 9, 1), (0, 1, 16, 1), (17, 1, 2, -1), (9, -1, 18, 1), (4, 1, 1, 1), (20, 1, 10, 1), (20, 1, 5, 1), (21, 1, 7, -1), (10, 1, 22, 1), (5, 1, 8, -1), (25, 1, 11, 1), (6, 1, 25, 1), (6, 1, 26, 1), (13, 1, 28, 1), (16, -1, 29, 1), (22, 1, 12, -1), (31, 1, 15, -1), (18, 1, 24, -1), (11, -1, 33, 1), (12, 1, 14, 1), (19, 1, 35, 1), (14, 1, 15, 1), (37, 1, 27, -1)],
    a_use=[13, 1, 16, 17, 18, 34, 2, 10, 11, 24, 21, 3, 5, 22, 19, 12, 1, 32, 15, 7, 27, 6, 36, 14, 38, 28, 30, 23, 26],
    c_prog=[(7, 1, 4, 1), (7, 1, 9, -1), (11, -1, 5, 1), (2, 1, 5, -1), (3, 1, 6, 1), (10, -1, 4, 1), (1, 1, 4, -1), (0, 1, 8, -1), (11, 1, 1, 1), (9, -1, 17, 1), (16, 1, 8, -1), (0, 1, 15, -1), (12, 1, 11, 1), (14, -1, 23, 1), (24, 1, 17, -1), (18, 1, 21, 1), (8, 1, 9, -1), (28, -1, 6, 1), (7, -1, 0, 1), (6, -1, 30, 1), (8, -1, 2, 1), (1, 1, 32, 1), (12, -1, 22, 1), (34, 1, 5, -1), (3, -1, 23, 1), (21, -1, 36, 1)],
    c_use=[(21, -1), (18, 1), (27, -1), (1, -1), (20, -1), (11, 1), (33, 1), (17, -1), (26, 1), (24, -1), (12, -1), (37, 1), (35, -1), (14, 1), (25, -1), (23, 1), (15, -1), (3, -1), (22, -1), (16, 1), (29, -1), (31, 1), (0, -1), (19, -1), (8, 1), (13, 1), (9, 1), (7, 1), (7, -1)],
    w=[[1, -1, 0, -1, 0, 0, 0, 0, 0], [0, 0, 0, 0, 1, 0, 0, 0, 0], [0, 1, 0, 0, 0, 0, 0, 0, 0], [0, -1, 1, 0, 0, 0, 0, -1, 1], [0, 0, -1, 0, 0, 0, 0, 1, -1], [0, 0, 0, 0, 0, 0, 0, 1, -1], [0, 0, 1, 0, 0, 0, 0, 0, 1], [1, -1, 0, -1, 1, 0, 0, 0, 0], [0, 0, 0, 0, 0, 0, 0, 1, 0], [0, 0, 0, 0, 0, -1, 0, -1, 1], [0, 0, 0, 0, -1, 1, 0, 1, -1], [-1, 0, 0, 1, 0, 0, 0, 0, 0], [0, 0, 0, 0, 0, -1, 0, 0, 1], [0, 0, 0, 0, 0, 1, 0, 0, 0], [0, 0, 1, 0, 0, 0, 0, 0, 0], [-1, 0, -1, 1, 0, 0, 0, 0, 0], [1, 0, 1, -1, 0, -1, 0, 0, 0], [0, 0, 0, -1, 0, 0, 0, 0, 0], [0, 0, 0, 0, 0, 1, -1, 0, -1], [0, 0, 0, 1, 0, 1, -1, 0, -1], [0, 0, 0, 0, 0, 0, 1, 0, 0], [-1, 0, 0, 0, 0, 0, -1, 0, 0], [-1, 0, -1, 0, 0, 0, 0, 0, 0], [0, 0, 1, 0, 0, 0, -1, 0, 0], [0, 0, 0, 0, 0, 0, 1, 0, 1], [-1, 1, 0, 0, 0, 0, -1, 0, 0], [-1, 1, 0, 0, 0, 0, 0, 0, 0], [0, 0, 0, 0, -1, 0, 0, 0, 0], [-1, 1, 0, 0, 0, 0, -1, 1, 0]])
S343 = dict(m=3, k=4, n=3,
    a_prog=[(0, 1, 10, -1), (4, 1, 5, 1), (6, 1, 5, 1), (7, 1, 5, 1), (11, 1, 4, 1), (3, 1, 6, 1), (9, 1, 8, 1), (11, 1, 9, 1), (2, 1, 1, 1), (0, 1, 18, -1), (3, 1, 15, 1), (20, 1, 10, -1), (14, 1, 11, -1), (22, 1, 13, -1), (21, 1, 19, 1), (24, 1, 15, -1), (23, 1, 24, -1), (28, 1, 19, -1), (12, 1, 26, -1), (30, 1, 16, 1), (1, 1, 3, 1), (32, -1, 23, 1), (33, -1, 12, 1), (34, 1, 17, -1), (32, 1, 21, 1), (15, 1, 36, 1)],
    a_use=[6, 13, 15, 14, 24, 22, 27, 29, 3, 20, 23, 6, 17, 25, 4, 16, 11, 31, 10, 12, 35, 33, 19, 18, 21, 37, 0, 26, 1],
    c_prog=[(0, 1, 2, -1), (5, 1, 8, -1), (0, 1, 6, 1), (6, 1, 8, -1), (2, 1, 6, 1), (2, 1, 8, 1), (3, -1, 0, 1), (7, 1, 8, -1), (0, 1, 1, -1), (1, -1, 15, 1), (2, 1, 16, -1), (15, 1, 2, -1), (5, 1, 16, 1), (6, 1, 17, 1), (6, 1, 10, 1), (19, -1, 1, 1), (3, 1, 23, -1), (18, 1, 4, 1), (22, 1, 7, -1), (4, 1, 21, -1), (20, 1, 5, 1)],
    c_use=[(4, -1), (4, 1), (26, 1), (28, -1), (21, 1), (18, 1), (5, -1), (16, 1), (15, -1), (24, -1), (19, 1), (29, 1), (20, -1), (3, 1), (25, 1), (23, 1), (10, -1), (12, -1), (14, -1), (13, 1), (9, -1), (2, -1), (7, -1), (27, -1), (22, -1), (17, -1), (11, 1), (6, -1), (1, -1)],
    w=[[0, -1, 0, 0, 1, 0, 0, -1, 0, 0, -1, 0], [0, 1, 0, 0, 0, 0, 0, 0, 0, 0, 0, 0], [0, 0, 0, 0, 0, 0, 0, 0, 0, 0, 1, 0], [0, 1, 0, 0, -1, 0, 0, 0, 0, 0, 1, 0], [0, -1, 0, 0, 1, 1, 0, 0, 0, 0, -1, 0], [0, 0, 0, -1, 0, 0, 0, 0, 0, 0, -1, 0], [0, 0, 0, 0, 0, 0, 0, 0, 0, 0, 0, 1], [0, 0, 0, 0, 0, 1, 0, 0, 0, 0, 0, 0], [0, 0, 0, 0, 0, 1, -1, 0, -1, -1, -1, -1], [0, 0, 0, 0, 0, 0, 0, -1, 0, 0, 0, 0], [0, 0, 0, 0, 0, 1, 0, 1, 0, 0, 0, 0], [0, 0, 0, 0, 0, -1, 0, 0, 1, 0, 0, 1], [0, 0, 0, 0, 0, -1, 1, 0, 1, 0, 0, 1], [0, 0, 0, -1, 0, 0, 0, 0, 0, 1, 0, 0], [1, 0, 0, -1, 0, 0, 0, 0, 0, 1, 0, 0], [1, 0, 1, -1, 0, 0, 0, 0, 0, 1, 0, 0], [1, 1, 1, -1, -1, -1, 0, 0, 0, 1, 1, 1], [0, 0, 1, 0, 0, 0, 0, 0, 0, 0, 0, 0], [0, 0, -1, 0, 0, 0, 0, -1, -1, 0, 0, 0], [0, 0, 1, 0, 0, 0, -1, 0, 0, 0, 0, 0], [0, 0, 0, 0, 0, 0, 1, 0, 0, 0, 0, 0], [0, 0, 0, 0, 0, 1, -1, 0, -1, 0, 0, 0], [0, 1, 0, 0, -1, -1, 0, 0, 0, 0, 0, 0], [0, 1, 0, 0, 0, 0, 0, 0, 0, 0, 0, 0], [0, 1, 0, 1, 0, 0, 0, 0, 0, 0, 0, 0], [0, 0, 0, -1, 0, 0, 0, 0, 0, 0, 0, 0], [1, 1, 0, 0, 0, 0, 1, 0, 0, 0, 0, 0], [1, 0, 1, -1, 0, 0, 0, 0, 0, 0, 0, 0], [0, 0, 0, -1, -1, 0, 0, 1, 0, 0, 0, 0]])
HK = dict(m=2, k=3, n=3,
    a_prog=[(5, 1, 4, 1), (5, -1, 3, 1), (0, 1, 2, -1), (0, 1, 3, -1), (2, 1, 3, -1), (5, -1, 2, 1), (0, 1, 1, -1), (12, 1, 3, -1), (6, -1, 2, 1), (1, 1, 14, 1), (13, 1, 4, 1)],
    a_use=[4, 14, 6, 1, 2, 12, 15, 8, 13, 16, 7, 3, 10, 11, 9],
    c_prog=[(5, -1, 0, 1), (5, 1, 3, 1), (3, 1, 0, 1), (1, 1, 2, -1), (4, -1, 3, 1), (0, 1, 2, 1), (5, 1, 2, 1), (12, -1, 1, 1), (0, 1, 10, 1), (1, -1, 14, 1), (4, 1, 13, 1)],
    c_use=[(4, 1), (13, -1), (16, 1), (1, 1), (12, 1), (15, 1), (9, -1), (11, -1), (14, -1), (10, 1), (7, 1), (8, -1), (6, -1), (5, -1), (0, 1)],
    w=[[0, 0, 0, 1, 1, 0, 0, -1, 0], [0, 0, 0, 0, 0, -1, 0, -1, 0], [0, 0, 0, 0, 0, 0, 0, 1, 0], [0, 1, 0, 0, 1, 1, 0, 0, 0], [0, 0, 1, 0, 0, 0, 0, 1, 1], [0, -1, 0, 0, 0, 0, 0, 0, 0], [0, 0, 0, 0, 0, 1, 0, 0, 0], [0, 0, -1, 0, 0, 0, 0, 0, 0], [0, -1, 0, 1, 0, 0, 0, 0, 0], [0, 0, 0, 1, 0, 0, 0, 0, 0], [0, 0, 0, 0, 0, 0, -1, 0, 0], [-1, -1, 0, 0, 0, 0, -1, 0, 0], [0, 0, -1, 0, 0, 0, -1, 0, 0], [0, 0, 0, 0, 0, -1, -1, 0, 1], [1, 0, -1, 1, 0, 0, 0, 0, 0]])
Sa = dict(m=4, k=3, n=3,
    a_prog=[(1, 1, 3, -1), (2, 1, 6, -1), (9, -1, 3, 1), (7, -1, 5, 1), (3, 1, 10, 1), (0, 1, 14, 1), (17, 1, 2, -1), (9, 1, 18, 1), (4, 1, 1, 1), (20, 1, 5, 1), (10, -1, 20, 1), (21, 1, 10, -1), (7, 1, 22, 1), (5, 1, 8, 1), (6, -1, 25, 1), (11, -1, 25, 1), (6, -1, 27, 1), (3, 1, 7, 1), (29, 1, 4, 1), (0, 1, 1, 1), (6, -1, 31, 1), (2, 1, 7, -1), (8, -1, 33, 1), (16, 1, 28, 1), (35, 1, 14, -1), (11, -1, 23, 1), (18, 1, 37, -1)],
    a_use=[14, 16, 1, 23, 11, 10, 3, 36, 17, 5, 22, 18, 38, 2, 28, 26, 21, 19, 12, 1, 30, 27, 15, 7, 32, 6, 24, 13, 34],
    c_prog=[(8, 1, 0, 1), (9, 1, 7, 1), (4, 1, 7, -1), (4, 1, 10, 1), (2, 1, 5, -1), (11, 1, 5, 1), (6, -1, 3, 1), (4, -1, 1, 1), (11, -1, 1, 1), (14, 1, 11, -1), (18, 1, 8, 1), (16, -1, 0, 1), (15, 1, 9, -1), (24, 1, 19, 1), (23, 1, 17, -1), (15, 1, 21, -1), (3, -1, 23, 1), (24, 1, 28, 1), (9, 1, 3, 1), (30, 1, 22, -1), (0, 1, 7, -1), (32, 1, 6, 1), (8, 1, 2, 1), (1, 1, 34, 1), (21, 1, 17, 1), (22, 1, 36, -1)],
    c_use=[(25, 1), (24, -1), (19, -1), (21, -1), (27, 1), (15, -1), (29, 1), (9, -1), (1, -1), (37, -1), (14, -1), (20, -1), (11, -1), (35, 1), (13, 1), (31, -1), (17, 1), (26, -1), (23, 1), (16, 1), (3, -1), (7, -1), (22, -1), (18, -1), (0, 1), (33, 1), (7, -1), (12, -1), (8, -1)],
    w=[[0, -1, 0, 0, 0, 0, 0, 0, 0], [-1, -1, 0, 1, 0, 0, 0, 0, 0], [0, 0, 0, 0, -1, 0, 0, 0, 0], [0, 0, 0, 0, 0, -1, 0, -1, 1], [0, 0, 0, 0, 0, 0, 0, 1, 0], [1, 1, 0, -1, -1, 0, 0, 0, 0], [-1, 0, 0, 1, 0, 0, 0, 0, 0], [-1, -1, 0, 0, 0, 0, 0, 0, 0], [0, -1, 1, 0, 0, 0, 0, -1, 1], [0, 0, 0, 0, 0, -1, 0, 0, 1], [0, 0, 0, 0, -1, 1, 0, 1, -1], [0, 0, -1, 0, 0, 0, 0, 1, -1], [0, 0, 0, 0, 0, 0, 0, 1, -1], [0, 0, 1, 0, 0, 0, 0, 0, 1], [-1, -1, 0, 0, 0, 0, -1, 0, 0], [0, 0, 0, 0, 0, 0, -1, 0, 0], [0, 0, 0, 0, 0, 1, 0, 0, 0], [0, 0, 1, 0, 0, 0, 0, 0, 0], [-1, 0, -1, 1, 0, 0, 0, 0, 0], [-1, 0, -1, 1, 0, 1, 0, 0, 0], [0, 0, 0, -1, 0, 0, 0, 0, 0], [-1, -1, 0, 0, 0, 0, -1, -1, 0], [0, 0, 0, 0, 0, 1, -1, 0, -1], [0, 0, 0, 1, 0, 1, -1, 0, -1], [1, 0, 1, 0, 0, 0, 0, 0, 0], [1, 0, 0, 0, 0, 0, 1, 0, 0], [0, 0, 0, 0, -1, 0, 0, 0, 0], [0, 0, 1, 0, 0, 0, -1, 0, 0], [0, 0, 0, 0, 0, 0, 1, 0, 1]])
Sb = dict(m=4, k=3, n=3,
    a_prog=[(3, -1, 1, 1), (2, 1, 6, -1), (9, -1, 3, 1), (5, 1, 7, -1), (10, 1, 3, 1), (0, 1, 14, 1), (17, 1, 2, -1), (18, 1, 9, 1), (5, 1, 8, 1), (6, -1, 20, 1), (11, -1, 20, 1), (6, -1, 22, 1), (4, 1, 1, 1), (5, 1, 24, 1), (24, 1, 10, -1), (5, 1, 26, 1), (7, 1, 26, 1), (27, 1, 11, -1), (29, -1, 18, 1), (1, 1, 6, -1), (0, 1, 31, 1), (9, 1, 23, 1), (33, 1, 10, 1), (12, 1, 10, -1), (35, -1, 28, 1), (2, 1, 15, 1), (37, 1, 20, -1)],
    a_use=[7, 3, 36, 15, 5, 6, 21, 38, 13, 32, 2, 19, 12, 16, 1, 23, 25, 34, 14, 11, 10, 1, 27, 26, 22, 28, 18, 17, 30],
    c_prog=[(8, 1, 0, 1), (9, 1, 7, 1), (4, 1, 7, -1), (4, 1, 10, 1), (2, 1, 5, -1), (11, 1, 5, 1), (6, -1, 3, 1), (1, 1, 4, -1), (1, 1, 11, -1), (14, 1, 11, -1), (18, 1, 8, 1), (16, -1, 0, 1), (9, -1, 15, 1), (19, 1, 24, 1), (17, -1, 23, 1), (15, 1, 21, -1), (9, -1, 8, 1), (6, 1, 28, -1), (17, -1, 22, 1), (21, -1, 30, 1), (24, 1, 23, 1), (32, 1, 3, -1), (8, 1, 1, 1), (2, 1, 34, 1), (13, -1, 12, 1), (36, 1, 29, 1)],
    c_use=[(18, -1), (33, -1), (3, -1), (22, 1), (31, 1), (37, -1), (29, 1), (8, -1), (12, 1), (0, -1), (35, 1), (26, -1), (23, 1), (24, 1), (16, 1), (13, -1), (17, 1), (9, 1), (25, 1), (27, -1), (15, -1), (19, -1), (21, 1), (14, 1), (7, 1), (7, -1), (20, 1), (1, 1), (11, 1)],
    w=[[0, 0, 0, 1, 0, 1, -1, 0, -1], [1, 0, 0, -1, 0, 0, 0, 0, 0], [0, 0, 0, -1, 0, 0, 0, 0, 0], [0, 0, 0, 0, 0, -1, 1, 0, 1], [0, 0, 0, 0, 0, 1, 0, 0, -1], [-1, 0, 0, 0, 0, 0, -1, 0, 0], [0, 0, 0, 0, 0, 0, 1, 0, 0], [0, 0, 0, 0, 0, 0, 1, 0, 1], [0, 0, -1, 0, 0, 0, 1, 0, 0], [-1, 0, -1, 0, 0, 0, 0, 0, 0], [0, 0, 1, 0, 0, 0, 0, 0, 1], [0, 0, 1, 0, 0, 0, 0, 0, 0], [-1, 0, -1, 1, 0, 0, 0, 0, 0], [1, 1, 0, -1, 0, 0, 0, 0, 0], [-1, 0, -1, 1, 0, 1, 0, 0, 0], [1, 1, 0, 0, 0, 0, 1, 0, 0], [0, 0, 0, 0, 0, 1, 0, 0, 0], [1, 1, 0, 0, 0, 0, 0, 0, 0], [0, -1, 0, 0, 0, 0, 0, 0, 0], [0, 0, 0, 0, 0, 0, 0, -1, 0], [1, 1, 0, -1, -1, 0, 0, 0, 0], [0, 0, 0, 0, -1, 0, 0, 0, 0], [0, 0, 0, 0, 0, 1, 0, 1, -1], [0, 0, 0, 0, 1, -1, 0, -1, 1], [1, 1, 0, 0, 0, 0, 1, 1, 0], [0, 0, 0, 0, -1, 0, 0, 0, 0], [0, 0, 1, 0, 0, 0, 0, -1, 1], [0, 1, -1, 0, 0, 0, 0, 1, -1], [0, 0, 0, 0, 0, 0, 0, -1, 1]])
Sc = dict(m=4, k=3, n=3,
    a_prog=[(1, 1, 3, -1), (10, -1, 3, 1), (2, 1, 6, 1), (5, 1, 7, 1), (9, 1, 3, 1), (16, 1, 0, 1), (2, -1, 17, 1), (9, -1, 18, 1), (4, 1, 1, 1), (20, 1, 10, 1), (20, 1, 5, 1), (7, -1, 21, 1), (22, 1, 10, 1), (8, -1, 5, 1), (11, 1, 25, 1), (6, 1, 25, 1), (11, 1, 27, 1), (28, 1, 10, -1), (29, 1, 9, -1), (2, 1, 7, 1), (8, 1, 31, 1), (23, 1, 12, -1), (10, -1, 33, 1), (6, 1, 0, 1), (1, 1, 35, 1), (24, -1, 18, 1), (37, 1, 11, -1)],
    a_use=[15, 30, 27, 34, 5, 7, 6, 32, 3, 2, 14, 12, 19, 36, 28, 1, 13, 16, 10, 11, 18, 22, 38, 1, 17, 23, 24, 26, 21],
    c_prog=[(4, 1, 7, 1), (7, 1, 9, -1), (11, -1, 5, 1), (5, -1, 2, 1), (6, 1, 3, 1), (4, 1, 10, -1), (4, -1, 1, 1), (8, -1, 0, 1), (11, 1, 1, 1), (9, -1, 17, 1), (8, -1, 16, 1), (15, -1, 0, 1), (11, 1, 12, 1), (23, 1, 14, -1), (17, -1, 24, 1), (18, 1, 21, 1), (9, 1, 22, 1), (3, -1, 28, 1), (6, 1, 7, 1), (30, -1, 0, 1), (22, 1, 24, -1), (14, -1, 32, 1), (23, 1, 3, -1), (21, -1, 34, 1), (20, 1, 19, 1), (36, 1, 25, -1)],
    c_use=[(22, 1), (9, -1), (29, -1), (3, 1), (33, -1), (16, -1), (31, -1), (8, 1), (35, 1), (37, 1), (19, -1), (23, -1), (25, -1), (0, 1), (13, 1), (15, 1), (21, -1), (27, -1), (17, -1), (26, 1), (20, -1), (14, 1), (11, 1), (18, 1), (1, -1), (7, -1), (24, -1), (7, 1), (12, -1)],
    w=[[0, 0, 0, 0, 0, -1, 1, 0, 1], [1, -1, 0, 0, 0, 0, 0, 0, 0], [0, 0, 0, 0, 0, 0, 1, 0, 0], [0, 0, 0, 1, 0, 0, 0, 0, 0], [0, 0, 0, 0, 0, -1, 0, 0, 1], [0, 0, 0, -1, 0, -1, 1, 0, 1], [1, 0, 0, 0, 0, 0, 1, 0, 0], [0, 0, 0, 0, 0, 0, 1, 0, 1], [-1, 0, 0, 1, 0, 0, 0, 0, 0], [0, 0, 1, 0, 0, 0, 0, 0, 1], [0, 0, 1, 0, 0, 0, -1, 0, 0], [1, 0, 1, -1, 0, 0, 0, 0, 0], [0, 0, 1, 0, 0, 0, 0, 0, 0], [1, 0, 1, 0, 0, 0, 0, 0, 0], [-1, 1, 0, 0, 0, 0, -1, 0, 0], [-1, 0, -1, 1, 0, 1, 0, 0, 0], [1, -1, 0, -1, 0, 0, 0, 0, 0], [0, 1, 0, 0, 0, 0, 0, 0, 0], [1, -1, 0, -1, 1, 0, 0, 0, 0], [0, 0, 0, 0, 0, 0, 0, 1, 0], [0, 0, -1, 0, 0, 0, 0, 1, -1], [0, 0, 0, 0, 0, 1, 0, 0, 0], [0, 0, 0, 0, 0, 0, 0, 1, -1], [0, 0, 0, 0, 1, 0, 0, 0, 0], [0, -1, 1, 0, 0, 0, 0, -1, 1], [0, 0, 0, 0, 1, 0, 0, 0, 0], [0, 0, 0, 0, 0, -1, 0, -1, 1], [1, -1, 0, 0, 0, 0, 1, -1, 0], [0, 0, 0, 0, -1, 1, 0, 1, -1]])
Sd = dict(m=4, k=3, n=3,
    a_prog=[(10, -1, 3, 1), (6, -1, 3, 1), (3, 1, 7, -1), (5, -1, 1, 1), (11, -1, 0, 1), (9, -1, 13, 1), (11, -1, 17, 1), (6, 1, 18, 1), (10, -1, 4, 1), (5, 1, 20, 1), (7, -1, 20, 1), (21, 1, 7, -1), (22, 1, 1, 1), (2, 1, 5, 1), (8, -1, 25, 1), (0, 1, 25, 1), (8, -1, 27, 1), (1, 1, 12, -1), (29, 1, 20, 1), (2, 1, 11, 1), (1, 1, 31, 1), (8, -1, 23, 1), (33, 1, 18, 1), (28, 1, 13, 1), (14, -1, 35, 1), (12, 1, 19, -1), (16, 1, 37, 1)],
    a_use=[1, 5, 32, 15, 27, 0, 30, 3, 11, 16, 12, 19, 38, 23, 10, 14, 21, 13, 8, 7, 10, 22, 24, 18, 34, 36, 17, 26, 28],
    c_prog=[(4, 1, 7, 1), (0, 1, 3, -1), (4, 1, 10, 1), (2, 1, 9, 1), (10, 1, 8, 1), (5, 1, 8, 1), (5, 1, 11, 1), (4, -1, 1, 1), (6, -1, 1, 1), (18, 1, 9, 1), (2, 1, 13, 1), (6, 1, 12, 1), (8, 1, 19, 1), (23, 1, 14, -1), (24, 1, 12, 1), (17, 1, 21, -1), (2, 1, 10, -1), (28, 1, 11, -1), (22, 1, 24, 1), (30, 1, 17, -1), (23, 1, 21, 1), (32, 1, 3, 1), (2, 1, 0, 1), (34, 1, 6, 1), (0, 1, 1, 1), (36, 1, 9, -1)],
    c_use=[(13, -1), (31, -1), (2, -1), (22, -1), (35, 1), (37, 1), (3, 1), (33, 1), (29, 1), (15, 1), (21, 1), (27, 1), (9, -1), (24, -1), (18, 1), (23, -1), (17, -1), (25, 1), (26, -1), (12, -1), (14, 1), (19, -1), (1, -1), (16, 1), (8, 1), (6, -1), (10, 1), (1, 1), (20, -1)],
    w=[[0, 0, 0, -1, 0, 1, 1, 0, -1], [0, 0, 0, 0, 0, -1, 0, 0, 1], [0, 0, 0, 0, 0, 0, 1, 0, -1], [0, 0, 0, 0, 0, -1, -1, 0, 1], [0, 0, 0, 0, 0, 0, 1, 0, 0], [1, 0, 0, 0, 0, 0, -1, 0, 0], [0, 0, 0, 1, 0, 0, 0, 0, 0], [1, 0, 0, 1, 0, 0, 0, 0, 0], [0, 0, 1, 0, 0, 0, 0, 0, -1], [0, 0, 1, 0, 0, 0, -1, 0, 0], [-1, 0, 1, -1, 0, 0, 0, 0, 0], [0, 0, 1, 0, 0, 0, 0, 0, 0], [-1, 0, 1, 0, 0, 0, 0, 0, 0], [0, 0, 0, 0, 0, 1, 0, 1, -1], [-1, 0, 1, -1, 0, 1, 0, 0, 0], [1, -1, 0, 1, 0, 0, 0, 0, 0], [0, 0, 0, 0, 0, -1, 0, 0, 0], [0, -1, 0, 0, 0, 0, 0, 0, 0], [0, 0, 0, 0, 0, 0, 0, -1, 0], [1, -1, 0, 1, -1, 0, 0, 0, 0], [0, 0, 0, 0, 1, 0, 0, 0, 0], [0, 0, 0, 0, 1, -1, 0, -1, 1], [0, 0, 0, 0, -1, 0, 0, 0, 0], [0, 0, -1, 0, 0, 0, 0, -1, 1], [0, 0, 0, 0, 0, 0, 0, 1, -1], [1, -1, 0, 0, 0, 0, 0, 0, 0], [0, -1, 1, 0, 0, 0, 0, 1, -1], [1, -1, 0, 0, 0, 0, -1, 1, 0], [1, -1, 0, 0, 0, 0, -1, 0, 0]])
H2 = dict(m=2, k=3, n=3,
    a_prog=[(5, 1, 4, 1), (5, -1, 3, 1), (2, -1, 0, 1), (3, -1, 0, 1), (3, -1, 2, 1), (5, -1, 2, 1), (1, -1, 0, 1), (9, 1, 1, -1), (11, 1, 4, -1), (14, 1, 1, 1), (4, 1, 13, 1)],
    a_use=[3, 13, 16, 12, 7, 4, 6, 14, 15, 1, 2, 8, 9, 10, 11],
    c_prog=[(0, 1, 5, -1), (5, 1, 3, 1), (0, 1, 3, 1), (1, 1, 2, -1), (4, -1, 3, 1), (0, 1, 2, 1), (5, 1, 2, 1), (5, -1, 9, 1), (8, 1, 4, -1), (14, 1, 1, -1), (4, 1, 13, 1)],
    c_use=[(8, 1), (14, -1), (10, -1), (15, 1), (7, 1), (4, -1), (16, -1), (13, 1), (9, 1), (1, 1), (12, 1), (11, 1), (0, -1), (6, 1), (5, 1)],
    w=[[1, 1, 0, 0, 0, 0, 1, 0, 0], [0, -1, 0, 1, 0, 0, 0, 0, 0], [0, 0, 0, -1, 0, 0, 0, 0, 0], [0, -1, 0, 0, 0, 0, 0, 0, 0], [0, 0, 0, 0, 0, 0, -1, 0, 0], [0, 0, 0, -1, -1, 0, 0, 1, 0], [0, 0, 0, 0, 0, 0, 0, -1, 0], [0, 0, 0, 0, 0, 1, 0, 1, 0], [0, 0, 0, 0, 0, -1, 0, 0, 0], [0, 1, 0, 0, 1, 1, 0, 0, 0], [0, 0, 1, 0, 0, 0, 0, 1, 1], [0, 0, 1, 0, 0, 0, 0, 0, 0], [-1, 0, 1, -1, 0, 0, 0, 0, 0], [0, 0, 1, 0, 0, 0, 1, 0, 0], [0, 0, 0, 0, 0, 1, 1, 0, -1]])
H3 = dict(m=2, k=3, n=3,
    a_prog=[(5, 1, 4, 1), (5, -1, 3, 1), (0, 1, 2, -1), (0, 1, 3, -1), (2, 1, 3, -1), (5, -1, 2, 1), (0, 1, 1, -1), (9, 1, 1, -1), (4, -1, 11, 1), (1, 1, 14, 1), (4, 1, 13, 1)],
    a_use=[1, 12, 13, 16, 4, 6, 3, 7, 14, 15, 2, 8, 9, 10, 11],
    c_prog=[(5, -1, 0, 1), (3, 1, 5, 1), (3, 1, 0, 1), (2, -1, 1, 1), (3, 1, 4, -1), (2, 1, 0, 1), (2, 1, 5, 1), (5, -1, 9, 1), (10, 1, 0, 1), (1, -1, 14, 1), (13, 1, 4, 1)],
    c_use=[(1, -1), (15, 1), (14, -1), (10, 1), (4, -1), (16, 1), (8, -1), (7, 1), (13, -1), (9, -1), (12, 1), (11, 1), (0, 1), (6, -1), (5, 1)],
    w=[[0, -1, 0, 0, -1, -1, 0, 0, 0], [0, -1, 0, 0, 0, 0, 0, 0, 0], [0, -1, 0, 1, 0, 0, 0, 0, 0], [0, 0, 0, 1, 0, 0, 0, 0, 0], [0, 0, 0, -1, -1, 0, 0, 1, 0], [0, 0, 0, 0, 0, 0, 0, 1, 0], [-1, -1, 0, 0, 0, 0, -1, 0, 0], [0, 0, 0, 0, 0, 0, -1, 0, 0], [0, 0, 0, 0, 0, -1, 0, -1, 0], [0, 0, 0, 0, 0, 1, 0, 0, 0], [0, 0, 1, 0, 0, 0, 0, 1, 1], [0, 0, 1, 0, 0, 0, 0, 0, 0], [1, 0, -1, 1, 0, 0, 0, 0, 0], [0, 0, -1, 0, 0, 0, -1, 0, 0], [0, 0, 0, 0, 0, 1, 1, 0, -1]])

Se = {'m': 4, 'k': 3, 'n': 3, 'a_prog': [(10, -1, 3, 1), (6, -1, 3, 1), (3, 1, 7, -1), (5, -1, 1, 1), (11, -1, 0, 1), (9, -1, 13, 1), (11, -1, 17, 1), (6, 1, 18, 1), (10, -1, 4, 1), (5, 1, 20, 1), (7, -1, 20, 1), (21, 1, 7, -1), (22, 1, 1, 1), (2, 1, 5, 1), (8, -1, 25, 1), (0, 1, 25, 1), (8, -1, 27, 1), (1, 1, 12, -1), (29, 1, 20, 1), (2, 1, 11, 1), (1, 1, 31, 1), (8, -1, 23, 1), (33, 1, 18, 1), (28, 1, 13, 1), (14, -1, 35, 1), (12, 1, 19, -1), (16, 1, 37, 1)], 'a_use': [5, 27, 32, 15, 0, 1, 30, 3, 16, 11, 12, 19, 38, 10, 14, 21, 13, 23, 8, 7, 10, 22, 18, 34, 24, 17, 26, 28, 36], 'c_prog': [(4, 1, 7, 1), (0, 1, 3, -1), (4, 1, 10, 1), (2, 1, 9, 1), (10, 1, 8, 1), (5, 1, 8, 1), (5, 1, 11, 1), (4, -1, 1, 1), (6, -1, 1, 1), (18, 1, 9, 1), (2, 1, 13, 1), (6, 1, 12, 1), (8, 1, 19, 1), (23, 1, 14, -1), (24, 1, 12, 1), (17, 1, 21, -1), (2, 1, 10, -1), (28, 1, 11, -1), (22, 1, 24, 1), (30, 1, 17, -1), (23, 1, 21, 1), (32, 1, 3, 1), (2, 1, 0, 1), (34, 1, 6, 1), (0, 1, 1, 1), (36, 1, 9, -1)], 'c_use': [(31, 1), (35, 1), (2, 1), (22, -1), (37, 1), (13, -1), (3, -1), (33, 1), (15, -1), (29, 1), (21, 1), (27, 1), (9, 1), (18, 1), (23, -1), (17, 1), (25, 1), (24, -1), (26, -1), (12, 1), (14, -1), (19, -1), (16, 1), (8, -1), (1, 1), (10, -1), (1, -1), (20, 1), (6, -1)], 'w': [[0, 0, 0, 0, 0, 1, 0, 0, -1], [0, 0, 0, 0, 0, 0, 1, 0, 0], [0, 0, 0, 0, 0, 0, -1, 0, 1], [0, 0, 0, 0, 0, -1, -1, 0, 1], [1, 0, 0, 0, 0, 0, -1, 0, 0], [0, 0, 0, -1, 0, 1, 1, 0, -1], [0, 0, 0, -1, 0, 0, 0, 0, 0], [1, 0, 0, 1, 0, 0, 0, 0, 0], [0, 0, -1, 0, 0, 0, 1, 0, 0], [0, 0, 1, 0, 0, 0, 0, 0, -1], [-1, 0, 1, -1, 0, 0, 0, 0, 0], [0, 0, 1, 0, 0, 0, 0, 0, 0], [1, 0, -1, 0, 0, 0, 0, 0, 0], [-1, 0, 1, -1, 0, 1, 0, 0, 0], [1, -1, 0, 1, 0, 0, 0, 0, 0], [0, 0, 0, 0, 0, 1, 0, 0, 0], [0, -1, 0, 0, 0, 0, 0, 0, 0], [0, 0, 0, 0, 0, 1, 0, 1, -1], [0, 0, 0, 0, 0, 0, 0, -1, 0], [-1, 1, 0, -1, 1, 0, 0, 0, 0], [0, 0, 0, 0, -1, 0, 0, 0, 0], [0, 0, 0, 0, 1, -1, 0, -1, 1], [0, 0, -1, 0, 0, 0, 0, -1, 1], [0, 0, 0, 0, 0, 0, 0, -1, 1], [0, 0, 0, 0, 1, 0, 0, 0, 0], [0, 1, -1, 0, 0, 0, 0, -1, 1], [-1, 1, 0, 0, 0, 0, 1, -1, 0], [-1, 1, 0, 0, 0, 0, 1, 0, 0], [1, -1, 0, 0, 0, 0, 0, 0, 0]]}

Sf = {'m': 4, 'k': 3, 'n': 3, 'a_prog': [(10, -1, 3, 1), (6, -1, 3, 1), (3, 1, 7, -1), (5, -1, 1, 1), (11, -1, 0, 1), (9, -1, 13, 1), (11, -1, 17, 1), (6, 1, 18, 1), (10, -1, 4, 1), (5, 1, 20, 1), (7, -1, 20, 1), (21, 1, 7, -1), (22, 1, 1, 1), (2, 1, 5, 1), (8, -1, 25, 1), (0, 1, 25, 1), (8, -1, 27, 1), (1, 1, 12, -1), (29, 1, 20, 1), (2, 1, 11, 1), (1, 1, 31, 1), (8, -1, 23, 1), (33, 1, 18, 1), (28, 1, 13, 1), (14, -1, 35, 1), (12, 1, 19, -1), (16, 1, 37, 1)], 'a_use': [5, 0, 27, 32, 1, 3, 30, 11, 15, 16, 10, 14, 12, 19, 38, 21, 13, 8, 7, 10, 23, 18, 22, 34, 24, 26, 28, 17, 36], 'c_prog': [(4, 1, 7, 1), (0, 1, 3, -1), (4, 1, 10, 1), (2, 1, 9, 1), (10, 1, 8, 1), (5, 1, 8, 1), (5, 1, 11, 1), (4, -1, 1, 1), (6, -1, 1, 1), (18, 1, 9, 1), (2, 1, 13, 1), (6, 1, 12, 1), (8, 1, 19, 1), (23, 1, 14, -1), (24, 1, 12, 1), (17, 1, 21, -1), (2, 1, 10, -1), (28, 1, 11, -1), (22, 1, 24, 1), (30, 1, 17, -1), (23, 1, 21, 1), (32, 1, 3, 1), (2, 1, 0, 1), (34, 1, 6, 1), (0, 1, 1, 1), (36, 1, 9, -1)], 'c_use': [(31, -1), (37, -1), (35, 1), (2, -1), (13, -1), (33, -1), (3, -1), (29, -1), (22, -1), (15, 1), (18, 1), (23, -1), (21, 1), (27, 1), (9, -1), (17, 1), (25, -1), (26, 1), (12, 1), (14, -1), (24, -1), (16, 1), (19, -1), (8, -1), (1, -1), (1, 1), (20, -1), (10, -1), (6, -1)], 'w': [[0, 0, 0, 0, 0, -1, 0, 0, 1], [-1, 0, 0, 0, 0, 0, 1, 0, 0], [0, 0, 0, 0, 0, 0, 1, 0, 0], [0, 0, 0, 0, 0, 0, 1, 0, -1], [0, 0, 0, -1, 0, 1, 1, 0, -1], [-1, 0, 0, -1, 0, 0, 0, 0, 0], [0, 0, 0, -1, 0, 0, 0, 0, 0], [0, 0, -1, 0, 0, 0, 0, 0, 1], [0, 0, 0, 0, 0, -1, -1, 0, 1], [0, 0, 1, 0, 0, 0, -1, 0, 0], [-1, 0, 1, -1, 0, 1, 0, 0, 0], [1, -1, 0, 1, 0, 0, 0, 0, 0], [-1, 0, 1, -1, 0, 0, 0, 0, 0], [0, 0, 1, 0, 0, 0, 0, 0, 0], [-1, 0, 1, 0, 0, 0, 0, 0, 0], [0, 0, 0, 0, 0, 1, 0, 0, 0], [0, 1, 0, 0, 0, 0, 0, 0, 0], [0, 0, 0, 0, 0, 0, 0, 1, 0], [-1, 1, 0, -1, 1, 0, 0, 0, 0], [0, 0, 0, 0, -1, 0, 0, 0, 0], [0, 0, 0, 0, 0, 1, 0, 1, -1], [0, 0, -1, 0, 0, 0, 0, -1, 1], [0, 0, 0, 0, 1, -1, 0, -1, 1], [0, 0, 0, 0, 0, 0, 0, -1, 1], [0, 0, 0, 0, -1, 0, 0, 0, 0], [1, -1, 0, 0, 0, 0, -1, 1, 0], [1, -1, 0, 0, 0, 0, -1, 0, 0], [0, 1, -1, 0, 0, 0, 0, -1, 1], [1, -1, 0, 0, 0, 0, 0, 0, 0]]}

Sg = {'m': 4, 'k': 3, 'n': 3, 'a_prog': [(10, -1, 3, 1), (6, -1, 3, 1), (3, 1, 7, -1), (5, -1, 1, 1), (11, -1, 0, 1), (9, -1, 13, 1), (11, -1, 17, 1), (6, 1, 18, 1), (10, -1, 4, 1), (5, 1, 20, 1), (7, -1, 20, 1), (21, 1, 7, -1), (22, 1, 1, 1), (2, 1, 5, 1), (8, -1, 25, 1), (0, 1, 25, 1), (8, -1, 27, 1), (1, 1, 12, -1), (29, 1, 20, 1), (2, 1, 11, 1), (1, 1, 31, 1), (8, -1, 23, 1), (33, 1, 18, 1), (28, 1, 13, 1), (14, -1, 35, 1), (12, 1, 19, -1), (16, 1, 37, 1)], 'a_use': [5, 0, 27, 1, 32, 15, 30, 3, 11, 16, 10, 14, 12, 19, 21, 38, 13, 7, 8, 10, 23, 18, 22, 34, 24, 28, 26, 17, 36], 'c_prog': [(4, 1, 7, 1), (0, 1, 3, -1), (4, 1, 10, 1), (2, 1, 9, 1), (10, 1, 8, 1), (5, 1, 8, 1), (5, 1, 11, 1), (4, -1, 1, 1), (6, -1, 1, 1), (18, 1, 9, 1), (2, 1, 13, 1), (6, 1, 12, 1), (8, 1, 19, 1), (23, 1, 14, -1), (24, 1, 12, 1), (17, 1, 21, -1), (2, 1, 10, -1), (28, 1, 11, -1), (22, 1, 24, 1), (30, 1, 17, -1), (23, 1, 21, 1), (32, 1, 3, 1), (2, 1, 0, 1), (34, 1, 6, 1), (0, 1, 1, 1), (36, 1, 9, -1)], 'c_use': [(31, -1), (37, -1), (35, 1), (13, -1), (2, -1), (22, -1), (3, -1), (33, -1), (29, -1), (15, 1), (18, 1), (23, -1), (21, 1), (27, 1), (17, -1), (9, 1), (25, -1), (12, 1), (26, 1), (14, -1), (24, -1), (16, 1), (19, -1), (8, -1), (1, -1), (20, 1), (1, -1), (10, -1), (6, -1)], 'w': [[0, 0, 0, 0, 0, -1, 0, 0, 1], [-1, 0, 0, 0, 0, 0, 1, 0, 0], [0, 0, 0, 0, 0, 0, 1, 0, 0], [0, 0, 0, -1, 0, 1, 1, 0, -1], [0, 0, 0, 0, 0, 0, 1, 0, -1], [0, 0, 0, 0, 0, -1, -1, 0, 1], [0, 0, 0, -1, 0, 0, 0, 0, 0], [-1, 0, 0, -1, 0, 0, 0, 0, 0], [0, 0, -1, 0, 0, 0, 0, 0, 1], [0, 0, 1, 0, 0, 0, -1, 0, 0], [-1, 0, 1, -1, 0, 1, 0, 0, 0], [1, -1, 0, 1, 0, 0, 0, 0, 0], [-1, 0, 1, -1, 0, 0, 0, 0, 0], [0, 0, 1, 0, 0, 0, 0, 0, 0], [0, 0, 0, 0, 0, -1, 0, 0, 0], [1, 0, -1, 0, 0, 0, 0, 0, 0], [0, 1, 0, 0, 0, 0, 0, 0, 0], [-1, 1, 0, -1, 1, 0, 0, 0, 0], [0, 0, 0, 0, 0, 0, 0, 1, 0], [0, 0, 0, 0, -1, 0, 0, 0, 0], [0, 0, 0, 0, 0, 1, 0, 1, -1], [0, 0, -1, 0, 0, 0, 0, -1, 1], [0, 0, 0, 0, 1, -1, 0, -1, 1], [0, 0, 0, 0, 0, 0, 0, -1, 1], [0, 0, 0, 0, -1, 0, 0, 0, 0], [-1, 1, 0, 0, 0, 0, 1, 0, 0], [-1, 1, 0, 0, 0, 0, 1, -1, 0], [0, 1, -1, 0, 0, 0, 0, -1, 1], [1, -1, 0, 0, 0, 0, 0, 0, 0]]}


SCHEMES = dict(S433=S433, S343=S343, HK=HK, Se=Se, Sf=Sf, Sg=Sg)


def gelu(y):
    return y * jnp.tanh(y * (y * y + C0)) + y


def lhs_operands(sc, block):
    m, k = sc["m"], sc["k"]
    memo, packed = {}, {}

    def node(v):
        if v not in memo:
            if v < m * k:
                memo[v] = (1, block(v // k, v % k))
            else:
                a, sa, b, sb = sc["a_prog"][v - m * k]
                (ta, xa), (tb, xb) = node(a), node(b)
                ta, tb = ta * sa, tb * sb
                memo[v] = (ta, xa + xb) if ta == tb else (1, xa - xb if ta > 0 else xb - xa)
        return memo[v]

    def op(p):
        v = sc["a_use"][p]
        if v not in packed:
            packed[v] = node(v)[1].astype(BF16)
        return packed[v]
    return op


def combine(sc, product, emit):
    m, n = sc["m"], sc["n"]
    fan = [0] * (m * n + len(sc["c_prog"]))
    for v, _ in sc["c_use"]:
        fan[v] += 1
    for a, _, b, _ in sc["c_prog"]:
        fan[a] += 1
        fan[b] += 1
    val = {}

    def push(v, t, x):
        if v in val:
            u, y = val[v]
            t, x = (t, y + x) if t == u else (1, x - y if t > 0 else y - x)
        val[v] = (t, x)
        fan[v] -= 1
        if fan[v] == 0:
            del val[v]
            if v >= m * n:
                a, sa, b, sb = sc["c_prog"][v - m * n]
                push(a, t * sa, x)
                push(b, t * sb, x)
            else:
                assert t == 1
                emit(v // n, v % n, x)

    for p, (v, t) in enumerate(sc["c_use"]):
        push(v, t, product(p))


def weight_form(sc, p, tile):
    n, acc = sc["n"], None
    for q in sorted(range(len(sc["w"][p])), key=lambda q: -sc["w"][p][q]):
        c = sc["w"][p][q]
        if c:
            v = tile(q // n, q % n)
            acc = (v if c > 0 else -v) if acc is None else (acc + v if c > 0 else acc - v)
    return acc


def make(CH=768, G1=4, G2=2, S=52, XC=8, XR2=4, MC1=48, MC2=48, mode2="k", vmem_mb=128, flags=None, E1=2, E2=2,
         run1=True, run2=True, dma=True, comp=True, pipe=True, PT=0, OFF=0, MCR=64, PADV=0, XW=C, RX=2, RB=2, OR=1, HL=False, RCH=256, nobc=False, TD=3, MID=True, LEAD=1, YB=0, YD=0, LNR=16, F0=0.0, F1=0.65, F2=0.68, F3=0.97, sc1='S433', sc2='HK', rs=1, PX=0, PH=0, PO=0, A1=1, B1=1, A2=1, B2=1):
    sc1, sc2 = (SCHEMES[z] if isinstance(z, str) else z for z in (sc1, sc2))
    NP1, NP2 = len(sc1["w"]), len(sc2["w"])
    PR = sc1["m"] * MC1
    KG2 = 12 // sc2["k"]
    TM1, TM2 = CH * G1, CH * G2
    XT = max(XC * CH, XR2 * TM2)
    W1ROW = (XT - HID - PR) // CH * CH

    @jax.jit
    def fn(x, dw, w1, w2, grn_g, grn_b):
        B, H, W, _ = x.shape
        N = B * H * W
        NT1, NT2 = N // TM1, N // TM2
        NCH = N // CH
        NHC = NCH - S
        R1 = -(-NHC * 65536 // (NT1 - E1))
        R2 = -(-NHC * 65536 * 2 // int(2 * NT2 - 2 * E2))
        PER, RF = PT * G2, OFF * G2
        NREC = len(range(RF, NHC, PER)) if PT else 0
        assert R1 <= G1 * 65536 and R2 <= G2 * 65536 and S >= 2 * max(G1, G2) and TM1 >= HID and E1 >= 2 and E2 >= (1.5 if MID and G2 == 2 else 2) and TD < XR2
        last = [(NCH - G1 + u) % XC for u in range(G1)]
        W2U, W2S = next((u, s0) for u in range(G1) for s0 in range(XC - 1)
                        if all(t not in last[u + 1:] for t in (s0, s0 + 1)))
        W2ROW = W2S * CH
        assert 2 * CH >= HID and XC >= G1

        def kernel(x_hbm, dw_ref, w1_hbm, w2_hbm, g_ref, b_ref, out_hbm, h_hbm,
                   xbuf, hbuf, ws, ssq, vec, abuf, w1p, ybuf, xsem, osem, hsem, wsem):
            class _Nop:
                def start(self, priority=0): pass
                def wait(self): pass
            mk = pltpu.make_async_copy if dma else (lambda *a: _Nop())

            def xrows(slot, tm):
                return xbuf.at[pl.ds(pl.multiple_of(slot * tm, tm), tm), pl.ds(0, C)]

            def x_copy(i, slot, tm):
                return mk(x_hbm.at[pl.ds(i * tm, tm)], xrows(slot, tm), xsem.at[slot])

            def o_copy(i, slot):
                return mk(xrows(slot, TM2), out_hbm.at[pl.ds(i * TM2, TM2)], osem.at[slot])

            def stored(c):
                return (c + (PER - RF)) % PER != 0 if PT else True

            def h_index(c):
                return c - (c + (PER - 1 - RF)) // PER if PT else c

            def h_out(c, slot):
                return mk(hbuf.at[slot], h_hbm.at[h_index(c)], hsem.at[slot])

            def h_in(c, slot):
                return mk(h_hbm.at[h_index(c)], hbuf.at[slot], hsem.at[slot])

            def w1_copy(q):
                return pltpu.make_async_copy(w1_hbm.at[:, pl.ds(q * C, C)], xbuf.at[pl.ds(W1ROW + q * C, C), pl.ds(0, C)], wsem.at[q])

            def w2_copy():
                return pltpu.make_async_copy(w2_hbm, xbuf.at[pl.ds(W2ROW, HID), pl.ds(0, C)], wsem.at[0])

            def wrap(v, n):
                return jnp.where(v >= n, v - n, v)

            def wrapn(v, n):
                return jnp.where(v < 0, v + n, v)

            def x0_copy():
                return pltpu.make_async_copy(x_hbm.at[pl.ds(0, PR)], xbuf.at[pl.ds(W1ROW + HID, PR), pl.ds(0, C)], osem.at[0])

            for q in range(4):
                w1_copy(q).start()
            x0_copy().start()
            ssq[...] = jnp.zeros_like(ssq)
            vec[0:8, :] = jnp.broadcast_to(dw_ref[...].astype(F32), (8, C))
            NPRE = W1ROW // CH
            for c in range(NPRE):
                pltpu.make_async_copy(x_hbm.at[pl.ds(c * CH + PR, CH)], xbuf.at[pl.ds(c * CH, CH), pl.ds(0, C)], xsem.at[c]).start() if dma else None
            for q in range(4):
                w1_copy(q).wait()

            def w1_tile(k, n):
                r = W1ROW + (n // 3) * C + k * L
                return xbuf[r:r + L, (n % 3) * L:(n % 3 + 1) * L].astype(F32)

            for c in range(4):
                for p in range(NP1):
                    ws[p * 4 + c] = pk(weight_form(sc1, p, lambda k, j: w1_tile(k, 4 * j + c)))

            if PT:
                for k in range(3):
                    for n in range(HID // L):
                        w1p[k * 64:(k + 1) * 64, n * L:(n + 1) * L] = pk(w1_tile(k, n))

            def layernorm(row, n=LNR):
                y = xbuf[pl.ds(pl.multiple_of(row, 16), n), :C].astype(F32) * jnp.concatenate([vec[0:8, :]] * (n // 8), axis=0)
                mu = jnp.sum(y, axis=-1, keepdims=True) * (1.0 / C)
                d = y - mu
                ss = jnp.sum(d * d, axis=-1, keepdims=True)
                v = ss * (1.0 / (C * ALPHA * ALPHA)) + 1e-5 / (ALPHA * ALPHA)
                if rs == 0:
                    return d * lax.rsqrt(v)
                return d * jnp.exp2(-0.5 * jnp.log2(v))

            def act(y, hs, r0, c):
                h = gelu(y)
                ssq[:, c * L:(c + 1) * L] += jnp.sum((h * h).reshape(MC1 // 8, 8, L), axis=0)
                if HL:
                    hbuf[hs, c, pl.ds(r0 // 2, MC1 // 2), :] = pack16(h)
                else:
                    hbuf[hs, pl.ds(r0 // 2, MC1 // 2), c * L:(c + 1) * L] = pack16(h)

            def operands(row):
                nl = MC1 // LNR
                a = {}
                def ln(t, q):
                    a[t, q] = layernorm(row + t * MC1 + q * LNR)
                op = lhs_operands(sc1, lambda t, k: jnp.concatenate([a[t, q][:, k * L:(k + 1) * L] for q in range(nl)], axis=0))
                lns = [functools.partial(ln, t, q) for t in range(sc1["m"]) for q in range(nl)]
                forms = [functools.partial(op, p) for p in range(NP1)]
                return op, lns, forms

            NB1 = TM1 // (PR)

            PPC = CH // PR

            def xc_copy(c, slot, n=CH):
                return mk(x_hbm.at[pl.ds(c * CH + PR, n)], xbuf.at[pl.ds(pl.multiple_of(slot * CH, CH), n), pl.ds(0, C)], xsem.at[slot])

            def xc_do(c, slot, what):
                @pl.when(c < NCH - 1)
                def _():
                    what(xc_copy(c, slot))
                @pl.when(c == NCH - 1)
                def _():
                    what(xc_copy(c, slot, CH - PR))

            def stage(row):
                for t in range(sc1["m"]):
                    abuf[t * MC1:(t + 1) * MC1, :] = layernorm(row + t * MC1, MC1)

            def phase1(i, carry):
                xb, hb, q, qs = carry
                slots = [wrap(hb + u, S) for u in range(G1)]
                xsl = [wrap(xb + u, XC) for u in range(G1)]
                qn = jnp.minimum((i * R1) >> 16, NHC)
                for u in range(G1):
                    xc_do(i * G1 + u, xsl[u], lambda cp: cp.wait())
                    @pl.when(jnp.logical_and(i * G1 + u >= S, stored(jnp.maximum(i * G1 + u - S, 0))))
                    def _():
                        h_out(i * G1 + u - S, slots[u]).wait()
                for u in range(G1):
                    @pl.when(jnp.logical_and(q + u < qn, stored(q + u)))
                    def _():
                        h_out(q + u, wrap(qs + u, S)).start()

                nxt = None
                parked = []
                park_product = lambda f: f
                def flush():
                    b, t, j, hs, r0, col = parked.pop(0)
                    act(ybuf[b, t * 3 + j], hs, r0, col)
                for m in range(NB1 if comp else 0):
                    u, r = divmod(m * PR, CH)
                    op = lhs_operands(sc1, lambda t, k: abuf[t * MC1:(t + 1) * MC1, k * L:(k + 1) * L]) if m == 0 else nxt
                    nxt, lns, forms = operands(xsl[u] * CH + r)
                    if m == NB1 - 1:
                        def put(t):
                            abuf[t * MC1:(t + 1) * MC1, :] = layernorm(xsl[u] * CH + r + t * MC1, MC1)
                        lns, forms = [functools.partial(put, t) for t in range(sc1["m"])], []
                    ns = 4 * NP1
                    todo = {}
                    for e, f in enumerate(lns):
                        todo.setdefault(int(ns * (F0 + (F1 - F0) * e / len(lns))), []).append(f)
                    for e, f in enumerate(forms):
                        todo.setdefault(int(ns * (F2 + (F3 - F2) * e / len(forms))), []).append(f)
                    for c in range(4):
                        def product(p):
                            for f in todo.pop(c * NP1 + p, []):
                                f()
                            return jnp.dot(op(p), upk(ws[p * 4 + c]), preferred_element_type=F32)
                        if YB == 0:
                            combine(sc1, product, lambda t, j, y: act(y, slots[u], r + t * MC1, 4 * j + c))
                        else:
                            def park(t, j, y):
                                ybuf[c % YB, t * 3 + j] = y
                                parked.append((c % YB, t, j, slots[u], r + t * MC1, 4 * j + c))
                                while len(parked) > YD:
                                    flush()
                            combine(sc1, park_product(product), park)
                    assert not todo
                    if (m + 1) % PPC == 0:
                        xc_do(i * G1 + u + XC, xsl[u], lambda cp: cp.start())
                        if u == W2U:
                            @pl.when(i == NT1 - 1)
                            def _():
                                w2_copy().start()
                while parked:
                    flush()
                return wrap(xb + G1, XC), wrap(hb + G1, S), qn, wrap(qs + (qn - q), S)

            z = jnp.int32(0)
            x0_copy().wait()
            stage(W1ROW + HID)
            for c in range(NPRE, XC):
                xc_copy(c, c).start()
            if run1:
                lax.fori_loop(0, NT1, phase1, (z, z, z, z))
            else:
                for c in range(XC):
                    xc_copy(c, c).wait()
                w2_copy().start()

            free2 = [s for s in range(XR2) if (s + 1) * TM2 <= W2ROW or s * TM2 >= W2ROW + HID]
            first2 = [(j, (NT2 - 1 - j) % XR2) for j in range(XR2 - 1)]
            if run2:
                for j, s in first2:
                    if s in free2:
                        x_copy(NT2 - 1 - j, s, TM2).start()
            gx = jnp.sqrt(jnp.sum(ssq[...], axis=0, keepdims=True) * (HS * HS) + 1e-6)
            nx = gx / (jnp.mean(gx, axis=-1, keepdims=True) + 1e-6)
            sc = (g_ref[...].astype(F32) * nx + 1.0) * HS
            w2_copy().wait()
            for r in range(KG2):
                cols = [jnp.broadcast_to(sc[:, (KG2 * k + r) * L:(KG2 * k + r + 1) * L], (L, L)).T for k in range(sc2["k"])]
                tile = lambda k, j: xbuf[W2ROW + (KG2 * k + r) * L:W2ROW + (KG2 * k + r + 1) * L, j * L:(j + 1) * L].astype(F32) * cols[k]
                for p in range(NP2):
                    ws[p * KG2 + r] = pk(weight_form(sc2, p, tile))
            bv = b_ref[...].astype(F32)
            bias = jnp.zeros((8, C), F32)
            for k in range(HID // L):
                col = jnp.broadcast_to(bv[:, k * L:(k + 1) * L], (L, L)).T
                prod = xbuf[W2ROW + k * L:W2ROW + (k + 1) * L, :C].astype(F32) * jnp.concatenate([col] * 3, axis=1)
                bias = bias + jnp.sum(prod.reshape(L // 8, 8, C), axis=0)
            bias = jnp.broadcast_to(jnp.sum(bias, axis=0, keepdims=True), (8, C))
            vec[0:8, :] = bias
            if run2:
                for j, s in first2:
                    if s not in free2:
                        x_copy(NT2 - 1 - j, s, TM2).start()

            def phase2(j, carry):
                xs, hb, q, qs = carry
                i = NT2 - 1 - j
                slots = [wrap(hb + u, S) for u in range(G2)]
                nxs, nhb = wrapn(xs - 1, XR2), wrapn(hb - G2, S)

                s2 = wrap(xs + 2, XR2)
                x_copy(i, xs, TM2).wait()
                for u in range(G2):
                    @pl.when(jnp.logical_and(i * G2 + u < NHC, stored(i * G2 + u)))
                    def _():
                        h_in(i * G2 + u, slots[u]).wait()
                @pl.when(jnp.logical_and(j >= 2, i + 2 > TD))
                def _():
                    o_copy(i + 2, s2).wait()
                @pl.when(jnp.logical_and(j >= 1, i + 1 > TD))
                def _():
                    o_copy(i + 1, wrap(xs + 1, XR2)).start(priority=PO)
                if TD:
                    @pl.when(i == 0)
                    def _():
                        for t in range(TD, 0, -1):
                            o_copy(t, t % XR2).start(priority=PO)
                @pl.when(jnp.logical_and(j >= 1, i + 2 - XR2 >= 0))
                def _():
                    x_copy(i + 2 - XR2, s2, TM2).start(priority=PX)

                if PT and comp:
                    @pl.when(jnp.logical_and(i * G2 < NHC, jnp.logical_not(stored(i * G2))))
                    def _():
                        def rows(g, carry):
                            for r in range(0, RCH, MCR):
                                r = pl.multiple_of(g * RCH + r, MCR)
                                a = layernorm(xs * TM2 + r, MCR).astype(BF16)
                                for n in range(0, HID, 512):
                                    y = jnp.dot(a, upk(w1p[:, n:n + 512]), preferred_element_type=F32)
                                    w = pack16(gelu(y))
                                    rr = pl.ds(pl.multiple_of(r // 2, MCR // 2), MCR // 2)
                                    if HL:
                                        for c in range(4):
                                            hbuf[slots[0], n // L + c, rr, :] = w[:, c * L:(c + 1) * L]
                                    else:
                                        hbuf[slots[0], rr, n:n + 512] = w
                            return carry
                        lax.fori_loop(0, CH // RCH, rows, 0)

                NB2 = TM2 // (sc2['m'] * MC2)
                for mi, m in enumerate(reversed(range(NB2))):
                    if mi % (NB2 // G2) == A2 and (MID or mi == A2):
                        e = mi // (NB2 // G2)
                        qn = jnp.minimum(jnp.minimum((((j * G2 + e) * R2) >> 16) // G2 + LEAD, j * G2 + e), NHC)
                        for u in range(G2):
                            @pl.when(jnp.logical_and(q + u < qn, stored(jnp.maximum(NHC - 1 - q - u, 0))))
                            def _():
                                h_in(NHC - 1 - q - u, wrapn(qs - u, S)).start(priority=PH)
                        qn = jnp.clip(qn, q, q + G2)
                        q, qs = qn, wrapn(qs - (qn - q), S)
                    if not comp:
                        continue
                    r0 = [(sc2['m'] * m + t) * MC2 for t in range(sc2['m'])]
                    orow = lambda t: pl.ds(pl.multiple_of(xs * TM2 + r0[t], 16), MC2)
                    hload = (lambda t, c0, n: unpack16(hbuf[slots[r0[t] // CH], c0 // L, pl.ds(r0[t] % CH // 2, MC2 // 2), :])) if HL else (lambda t, c0, n: unpack16(hbuf[slots[r0[t] // CH], pl.ds(r0[t] % CH // 2, MC2 // 2), c0:c0 + n]))
                    acc = {}
                    for r in range(KG2):
                        op = lhs_operands(sc2, lambda t, k: hload(t, (KG2 * k + r) * L, L))
                        def accum(t, jj, o):
                            cs = slice(jj * L, (jj + 1) * L)
                            terms = [o] if r == 0 else ([acc[t, jj], o] if OR & 1 else [o, acc[t, jj]])
                            extra = ([xbuf[orow(t), cs].astype(F32)] if r == RX else []) + ([jnp.concatenate([vec[0:8, cs]] * (MC2 // 8), axis=0)] if r == RB else [])
                            if OR & 2:
                                extra = extra[::-1]
                            terms = extra + terms if OR & 4 else terms + extra
                            acc[t, jj] = functools.reduce(lambda a, b: a + b, terms)
                            if r == KG2 - 1:
                                xbuf[orow(t), cs] = acc[t, jj].astype(BF16)
                        combine(sc2, lambda p: jnp.dot(op(p), upk(ws[p * KG2 + r]), preferred_element_type=F32), accum)
                return nxs, nhb, q, qs

            if run2:
                lax.fori_loop(0, NT2, phase2, (z + (NT2 - 1) % XR2, z + (NCH - G2) % S, z, z + (NHC - 1) % S))
                o_copy(0, 0).start()
                for t in range(max(TD, 1), -1, -1):
                    o_copy(t, t % XR2).wait()

        out, _ = pl.pallas_call(
            kernel,
            in_specs=[pl.BlockSpec(memory_space=pl.ANY), pl.BlockSpec(memory_space=pltpu.VMEM),
                      pl.BlockSpec(memory_space=pl.ANY), pl.BlockSpec(memory_space=pl.ANY),
                      pl.BlockSpec(memory_space=pltpu.VMEM), pl.BlockSpec(memory_space=pltpu.VMEM)],
            out_specs=[pl.BlockSpec(memory_space=pl.ANY)] * 2,
            out_shape=[jax.ShapeDtypeStruct((N, C), BF16), jax.ShapeDtypeStruct((NHC - NREC,) + ((HID // L, CH // 2, L) if HL else (CH // 2, HID)), U32)],
            scratch_shapes=[
                pltpu.VMEM((XT, XW), BF16),
                pltpu.VMEM((S,) + ((HID // L, CH // 2, L) if HL else (CH // 2, HID)), U32),
                pltpu.VMEM((max(NP1 * 4, NP2 * KG2), L // 2, L), U32),
                pltpu.VMEM((8, HID), F32),
                pltpu.VMEM((8 + PADV, C), F32),
                pltpu.VMEM((PR, C), F32),
                pltpu.VMEM((C // 2, HID) if PT else (8, L), U32),
                pltpu.VMEM((max(YB, 1), 3 * sc1['m'], MC1 if YB else 8, L), F32),
                pltpu.SemaphoreType.DMA((max(XC, XR2),)),
                pltpu.SemaphoreType.DMA((XR2,)),
                pltpu.SemaphoreType.DMA((S,)),
                pltpu.SemaphoreType.DMA((4,)),
            ],
            compiler_params=pltpu.CompilerParams(vmem_limit_bytes=vmem_mb * 1024 * 1024, flags=flags, disable_bounds_checks=nobc),
        )(x.reshape(N, C), dw.reshape(1, C), w1, w2, grn_g.reshape(1, HID), grn_b.reshape(1, HID))
        return out.reshape(x.shape)
    return fn


pallas_standalone__modern_conv_block_slak__vision_kernel = make(E1=3,E2=1.5,MC1=48,LNR=48,sc1='Sg',nobc=True,sc2='S343',MC2=32,S=52,PT=16,OFF=3,LEAD=2)
```

```python
import functools
import numpy as np
import jax
import jax.numpy as jnp
from jax import lax
import jax.experimental.pallas as pl
import jax.experimental.pallas.tpu as pltpu

C = 384
HID = 1536
L = 128
F32 = jnp.float32
BF16 = jnp.bfloat16
U32 = jnp.uint32
pk = lambda v: pltpu.bitcast(v.astype(BF16), U32)
upk = lambda v: pltpu.bitcast(v, BF16)


def pack16(v):
    t = v.shape[0] // 16
    lo = jnp.concatenate([v[16 * g:16 * g + 8] for g in range(t)], axis=0)
    hi = jnp.concatenate([v[16 * g + 8:16 * g + 16] for g in range(t)], axis=0)
    return pltpu.pack_elementwise([lo, hi], packed_dtype=BF16)


def unpack16(w):
    lo = pltpu.unpack_elementwise(w, index=0, packed_dtype=BF16, unpacked_dtype=F32)
    hi = pltpu.unpack_elementwise(w, index=1, packed_dtype=BF16, unpacked_dtype=F32)
    parts = []
    for g in range(w.shape[0] // 8):
        parts += [lo[8 * g:8 * g + 8], hi[8 * g:8 * g + 8]]
    return jnp.concatenate(parts, axis=0)
K0 = float(np.sqrt(2.0 / np.pi))
ALPHA = float((K0 * 0.044715) ** (1.0 / 3.0))
C0 = K0 / ALPHA
HS = 0.5 / ALPHA

S433 = dict(m=4, k=3, n=3,
    a_prog=[(3, -1, 1, 1), (10, -1, 3, 1), (2, 1, 6, 1), (5, 1, 7, 1), (3, 1, 9, 1), (0, 1, 16, 1), (17, 1, 2, -1), (9, -1, 18, 1), (4, 1, 1, 1), (20, 1, 10, 1), (20, 1, 5, 1), (21, 1, 7, -1), (10, 1, 22, 1), (5, 1, 8, -1), (25, 1, 11, 1), (6, 1, 25, 1), (6, 1, 26, 1), (13, 1, 28, 1), (16, -1, 29, 1), (22, 1, 12, -1), (31, 1, 15, -1), (18, 1, 24, -1), (11, -1, 33, 1), (12, 1, 14, 1), (19, 1, 35, 1), (14, 1, 15, 1), (37, 1, 27, -1)],
    a_use=[13, 1, 16, 17, 18, 34, 2, 10, 11, 24, 21, 3, 5, 22, 19, 12, 1, 32, 15, 7, 27, 6, 36, 14, 38, 28, 30, 23, 26],
    c_prog=[(7, 1, 4, 1), (7, 1, 9, -1), (11, -1, 5, 1), (2, 1, 5, -1), (3, 1, 6, 1), (10, -1, 4, 1), (1, 1, 4, -1), (0, 1, 8, -1), (11, 1, 1, 1), (9, -1, 17, 1), (16, 1, 8, -1), (0, 1, 15, -1), (12, 1, 11, 1), (14, -1, 23, 1), (24, 1, 17, -1), (18, 1, 21, 1), (8, 1, 9, -1), (28, -1, 6, 1), (7, -1, 0, 1), (6, -1, 30, 1), (8, -1, 2, 1), (1, 1, 32, 1), (12, -1, 22, 1), (34, 1, 5, -1), (3, -1, 23, 1), (21, -1, 36, 1)],
    c_use=[(21, -1), (18, 1), (27, -1), (1, -1), (20, -1), (11, 1), (33, 1), (17, -1), (26, 1), (24, -1), (12, -1), (37, 1), (35, -1), (14, 1), (25, -1), (23, 1), (15, -1), (3, -1), (22, -1), (16, 1), (29, -1), (31, 1), (0, -1), (19, -1), (8, 1), (13, 1), (9, 1), (7, 1), (7, -1)],
    w=[[1, -1, 0, -1, 0, 0, 0, 0, 0], [0, 0, 0, 0, 1, 0, 0, 0, 0], [0, 1, 0, 0, 0, 0, 0, 0, 0], [0, -1, 1, 0, 0, 0, 0, -1, 1], [0, 0, -1, 0, 0, 0, 0, 1, -1], [0, 0, 0, 0, 0, 0, 0, 1, -1], [0, 0, 1, 0, 0, 0, 0, 0, 1], [1, -1, 0, -1, 1, 0, 0, 0, 0], [0, 0, 0, 0, 0, 0, 0, 1, 0], [0, 0, 0, 0, 0, -1, 0, -1, 1], [0, 0, 0, 0, -1, 1, 0, 1, -1], [-1, 0, 0, 1, 0, 0, 0, 0, 0], [0, 0, 0, 0, 0, -1, 0, 0, 1], [0, 0, 0, 0, 0, 1, 0, 0, 0], [0, 0, 1, 0, 0, 0, 0, 0, 0], [-1, 0, -1, 1, 0, 0, 0, 0, 0], [1, 0, 1, -1, 0, -1, 0, 0, 0], [0, 0, 0, -1, 0, 0, 0, 0, 0], [0, 0, 0, 0, 0, 1, -1, 0, -1], [0, 0, 0, 1, 0, 1, -1, 0, -1], [0, 0, 0, 0, 0, 0, 1, 0, 0], [-1, 0, 0, 0, 0, 0, -1, 0, 0], [-1, 0, -1, 0, 0, 0, 0, 0, 0], [0, 0, 1, 0, 0, 0, -1, 0, 0], [0, 0, 0, 0, 0, 0, 1, 0, 1], [-1, 1, 0, 0, 0, 0, -1, 0, 0], [-1, 1, 0, 0, 0, 0, 0, 0, 0], [0, 0, 0, 0, -1, 0, 0, 0, 0], [-1, 1, 0, 0, 0, 0, -1, 1, 0]])
S343 = dict(m=3, k=4, n=3,
    a_prog=[(0, 1, 10, -1), (4, 1, 5, 1), (6, 1, 5, 1), (7, 1, 5, 1), (11, 1, 4, 1), (3, 1, 6, 1), (9, 1, 8, 1), (11, 1, 9, 1), (2, 1, 1, 1), (0, 1, 18, -1), (3, 1, 15, 1), (20, 1, 10, -1), (14, 1, 11, -1), (22, 1, 13, -1), (21, 1, 19, 1), (24, 1, 15, -1), (23, 1, 24, -1), (28, 1, 19, -1), (12, 1, 26, -1), (30, 1, 16, 1), (1, 1, 3, 1), (32, -1, 23, 1), (33, -1, 12, 1), (34, 1, 17, -1), (32, 1, 21, 1), (15, 1, 36, 1)],
    a_use=[6, 13, 15, 14, 24, 22, 27, 29, 3, 20, 23, 6, 17, 25, 4, 16, 11, 31, 10, 12, 35, 33, 19, 18, 21, 37, 0, 26, 1],
    c_prog=[(0, 1, 2, -1), (5, 1, 8, -1), (0, 1, 6, 1), (6, 1, 8, -1), (2, 1, 6, 1), (2, 1, 8, 1), (3, -1, 0, 1), (7, 1, 8, -1), (0, 1, 1, -1), (1, -1, 15, 1), (2, 1, 16, -1), (15, 1, 2, -1), (5, 1, 16, 1), (6, 1, 17, 1), (6, 1, 10, 1), (19, -1, 1, 1), (3, 1, 23, -1), (18, 1, 4, 1), (22, 1, 7, -1), (4, 1, 21, -1), (20, 1, 5, 1)],
    c_use=[(4, -1), (4, 1), (26, 1), (28, -1), (21, 1), (18, 1), (5, -1), (16, 1), (15, -1), (24, -1), (19, 1), (29, 1), (20, -1), (3, 1), (25, 1), (23, 1), (10, -1), (12, -1), (14, -1), (13, 1), (9, -1), (2, -1), (7, -1), (27, -1), (22, -1), (17, -1), (11, 1), (6, -1), (1, -1)],
    w=[[0, -1, 0, 0, 1, 0, 0, -1, 0, 0, -1, 0], [0, 1, 0, 0, 0, 0, 0, 0, 0, 0, 0, 0], [0, 0, 0, 0, 0, 0, 0, 0, 0, 0, 1, 0], [0, 1, 0, 0, -1, 0, 0, 0, 0, 0, 1, 0], [0, -1, 0, 0, 1, 1, 0, 0, 0, 0, -1, 0], [0, 0, 0, -1, 0, 0, 0, 0, 0, 0, -1, 0], [0, 0, 0, 0, 0, 0, 0, 0, 0, 0, 0, 1], [0, 0, 0, 0, 0, 1, 0, 0, 0, 0, 0, 0], [0, 0, 0, 0, 0, 1, -1, 0, -1, -1, -1, -1], [0, 0, 0, 0, 0, 0, 0, -1, 0, 0, 0, 0], [0, 0, 0, 0, 0, 1, 0, 1, 0, 0, 0, 0], [0, 0, 0, 0, 0, -1, 0, 0, 1, 0, 0, 1], [0, 0, 0, 0, 0, -1, 1, 0, 1, 0, 0, 1], [0, 0, 0, -1, 0, 0, 0, 0, 0, 1, 0, 0], [1, 0, 0, -1, 0, 0, 0, 0, 0, 1, 0, 0], [1, 0, 1, -1, 0, 0, 0, 0, 0, 1, 0, 0], [1, 1, 1, -1, -1, -1, 0, 0, 0, 1, 1, 1], [0, 0, 1, 0, 0, 0, 0, 0, 0, 0, 0, 0], [0, 0, -1, 0, 0, 0, 0, -1, -1, 0, 0, 0], [0, 0, 1, 0, 0, 0, -1, 0, 0, 0, 0, 0], [0, 0, 0, 0, 0, 0, 1, 0, 0, 0, 0, 0], [0, 0, 0, 0, 0, 1, -1, 0, -1, 0, 0, 0], [0, 1, 0, 0, -1, -1, 0, 0, 0, 0, 0, 0], [0, 1, 0, 0, 0, 0, 0, 0, 0, 0, 0, 0], [0, 1, 0, 1, 0, 0, 0, 0, 0, 0, 0, 0], [0, 0, 0, -1, 0, 0, 0, 0, 0, 0, 0, 0], [1, 1, 0, 0, 0, 0, 1, 0, 0, 0, 0, 0], [1, 0, 1, -1, 0, 0, 0, 0, 0, 0, 0, 0], [0, 0, 0, -1, -1, 0, 0, 1, 0, 0, 0, 0]])
HK = dict(m=2, k=3, n=3,
    a_prog=[(5, 1, 4, 1), (5, -1, 3, 1), (0, 1, 2, -1), (0, 1, 3, -1), (2, 1, 3, -1), (5, -1, 2, 1), (0, 1, 1, -1), (12, 1, 3, -1), (6, -1, 2, 1), (1, 1, 14, 1), (13, 1, 4, 1)],
    a_use=[4, 14, 6, 1, 2, 12, 15, 8, 13, 16, 7, 3, 10, 11, 9],
    c_prog=[(5, -1, 0, 1), (5, 1, 3, 1), (3, 1, 0, 1), (1, 1, 2, -1), (4, -1, 3, 1), (0, 1, 2, 1), (5, 1, 2, 1), (12, -1, 1, 1), (0, 1, 10, 1), (1, -1, 14, 1), (4, 1, 13, 1)],
    c_use=[(4, 1), (13, -1), (16, 1), (1, 1), (12, 1), (15, 1), (9, -1), (11, -1), (14, -1), (10, 1), (7, 1), (8, -1), (6, -1), (5, -1), (0, 1)],
    w=[[0, 0, 0, 1, 1, 0, 0, -1, 0], [0, 0, 0, 0, 0, -1, 0, -1, 0], [0, 0, 0, 0, 0, 0, 0, 1, 0], [0, 1, 0, 0, 1, 1, 0, 0, 0], [0, 0, 1, 0, 0, 0, 0, 1, 1], [0, -1, 0, 0, 0, 0, 0, 0, 0], [0, 0, 0, 0, 0, 1, 0, 0, 0], [0, 0, -1, 0, 0, 0, 0, 0, 0], [0, -1, 0, 1, 0, 0, 0, 0, 0], [0, 0, 0, 1, 0, 0, 0, 0, 0], [0, 0, 0, 0, 0, 0, -1, 0, 0], [-1, -1, 0, 0, 0, 0, -1, 0, 0], [0, 0, -1, 0, 0, 0, -1, 0, 0], [0, 0, 0, 0, 0, -1, -1, 0, 1], [1, 0, -1, 1, 0, 0, 0, 0, 0]])
Sa = dict(m=4, k=3, n=3,
    a_prog=[(1, 1, 3, -1), (2, 1, 6, -1), (9, -1, 3, 1), (7, -1, 5, 1), (3, 1, 10, 1), (0, 1, 14, 1), (17, 1, 2, -1), (9, 1, 18, 1), (4, 1, 1, 1), (20, 1, 5, 1), (10, -1, 20, 1), (21, 1, 10, -1), (7, 1, 22, 1), (5, 1, 8, 1), (6, -1, 25, 1), (11, -1, 25, 1), (6, -1, 27, 1), (3, 1, 7, 1), (29, 1, 4, 1), (0, 1, 1, 1), (6, -1, 31, 1), (2, 1, 7, -1), (8, -1, 33, 1), (16, 1, 28, 1), (35, 1, 14, -1), (11, -1, 23, 1), (18, 1, 37, -1)],
    a_use=[14, 16, 1, 23, 11, 10, 3, 36, 17, 5, 22, 18, 38, 2, 28, 26, 21, 19, 12, 1, 30, 27, 15, 7, 32, 6, 24, 13, 34],
    c_prog=[(8, 1, 0, 1), (9, 1, 7, 1), (4, 1, 7, -1), (4, 1, 10, 1), (2, 1, 5, -1), (11, 1, 5, 1), (6, -1, 3, 1), (4, -1, 1, 1), (11, -1, 1, 1), (14, 1, 11, -1), (18, 1, 8, 1), (16, -1, 0, 1), (15, 1, 9, -1), (24, 1, 19, 1), (23, 1, 17, -1), (15, 1, 21, -1), (3, -1, 23, 1), (24, 1, 28, 1), (9, 1, 3, 1), (30, 1, 22, -1), (0, 1, 7, -1), (32, 1, 6, 1), (8, 1, 2, 1), (1, 1, 34, 1), (21, 1, 17, 1), (22, 1, 36, -1)],
    c_use=[(25, 1), (24, -1), (19, -1), (21, -1), (27, 1), (15, -1), (29, 1), (9, -1), (1, -1), (37, -1), (14, -1), (20, -1), (11, -1), (35, 1), (13, 1), (31, -1), (17, 1), (26, -1), (23, 1), (16, 1), (3, -1), (7, -1), (22, -1), (18, -1), (0, 1), (33, 1), (7, -1), (12, -1), (8, -1)],
    w=[[0, -1, 0, 0, 0, 0, 0, 0, 0], [-1, -1, 0, 1, 0, 0, 0, 0, 0], [0, 0, 0, 0, -1, 0, 0, 0, 0], [0, 0, 0, 0, 0, -1, 0, -1, 1], [0, 0, 0, 0, 0, 0, 0, 1, 0], [1, 1, 0, -1, -1, 0, 0, 0, 0], [-1, 0, 0, 1, 0, 0, 0, 0, 0], [-1, -1, 0, 0, 0, 0, 0, 0, 0], [0, -1, 1, 0, 0, 0, 0, -1, 1], [0, 0, 0, 0, 0, -1, 0, 0, 1], [0, 0, 0, 0, -1, 1, 0, 1, -1], [0, 0, -1, 0, 0, 0, 0, 1, -1], [0, 0, 0, 0, 0, 0, 0, 1, -1], [0, 0, 1, 0, 0, 0, 0, 0, 1], [-1, -1, 0, 0, 0, 0, -1, 0, 0], [0, 0, 0, 0, 0, 0, -1, 0, 0], [0, 0, 0, 0, 0, 1, 0, 0, 0], [0, 0, 1, 0, 0, 0, 0, 0, 0], [-1, 0, -1, 1, 0, 0, 0, 0, 0], [-1, 0, -1, 1, 0, 1, 0, 0, 0], [0, 0, 0, -1, 0, 0, 0, 0, 0], [-1, -1, 0, 0, 0, 0, -1, -1, 0], [0, 0, 0, 0, 0, 1, -1, 0, -1], [0, 0, 0, 1, 0, 1, -1, 0, -1], [1, 0, 1, 0, 0, 0, 0, 0, 0], [1, 0, 0, 0, 0, 0, 1, 0, 0], [0, 0, 0, 0, -1, 0, 0, 0, 0], [0, 0, 1, 0, 0, 0, -1, 0, 0], [0, 0, 0, 0, 0, 0, 1, 0, 1]])
Sb = dict(m=4, k=3, n=3,
    a_prog=[(3, -1, 1, 1), (2, 1, 6, -1), (9, -1, 3, 1), (5, 1, 7, -1), (10, 1, 3, 1), (0, 1, 14, 1), (17, 1, 2, -1), (18, 1, 9, 1), (5, 1, 8, 1), (6, -1, 20, 1), (11, -1, 20, 1), (6, -1, 22, 1), (4, 1, 1, 1), (5, 1, 24, 1), (24, 1, 10, -1), (5, 1, 26, 1), (7, 1, 26, 1), (27, 1, 11, -1), (29, -1, 18, 1), (1, 1, 6, -1), (0, 1, 31, 1), (9, 1, 23, 1), (33, 1, 10, 1), (12, 1, 10, -1), (35, -1, 28, 1), (2, 1, 15, 1), (37, 1, 20, -1)],
    a_use=[7, 3, 36, 15, 5, 6, 21, 38, 13, 32, 2, 19, 12, 16, 1, 23, 25, 34, 14, 11, 10, 1, 27, 26, 22, 28, 18, 17, 30],
    c_prog=[(8, 1, 0, 1), (9, 1, 7, 1), (4, 1, 7, -1), (4, 1, 10, 1), (2, 1, 5, -1), (11, 1, 5, 1), (6, -1, 3, 1), (1, 1, 4, -1), (1, 1, 11, -1), (14, 1, 11, -1), (18, 1, 8, 1), (16, -1, 0, 1), (9, -1, 15, 1), (19, 1, 24, 1), (17, -1, 23, 1), (15, 1, 21, -1), (9, -1, 8, 1), (6, 1, 28, -1), (17, -1, 22, 1), (21, -1, 30, 1), (24, 1, 23, 1), (32, 1, 3, -1), (8, 1, 1, 1), (2, 1, 34, 1), (13, -1, 12, 1), (36, 1, 29, 1)],
    c_use=[(18, -1), (33, -1), (3, -1), (22, 1), (31, 1), (37, -1), (29, 1), (8, -1), (12, 1), (0, -1), (35, 1), (26, -1), (23, 1), (24, 1), (16, 1), (13, -1), (17, 1), (9, 1), (25, 1), (27, -1), (15, -1), (19, -1), (21, 1), (14, 1), (7, 1), (7, -1), (20, 1), (1, 1), (11, 1)],
    w=[[0, 0, 0, 1, 0, 1, -1, 0, -1], [1, 0, 0, -1, 0, 0, 0, 0, 0], [0, 0, 0, -1, 0, 0, 0, 0, 0], [0, 0, 0, 0, 0, -1, 1, 0, 1], [0, 0, 0, 0, 0, 1, 0, 0, -1], [-1, 0, 0, 0, 0, 0, -1, 0, 0], [0, 0, 0, 0, 0, 0, 1, 0, 0], [0, 0, 0, 0, 0, 0, 1, 0, 1], [0, 0, -1, 0, 0, 0, 1, 0, 0], [-1, 0, -1, 0, 0, 0, 0, 0, 0], [0, 0, 1, 0, 0, 0, 0, 0, 1], [0, 0, 1, 0, 0, 0, 0, 0, 0], [-1, 0, -1, 1, 0, 0, 0, 0, 0], [1, 1, 0, -1, 0, 0, 0, 0, 0], [-1, 0, -1, 1, 0, 1, 0, 0, 0], [1, 1, 0, 0, 0, 0, 1, 0, 0], [0, 0, 0, 0, 0, 1, 0, 0, 0], [1, 1, 0, 0, 0, 0, 0, 0, 0], [0, -1, 0, 0, 0, 0, 0, 0, 0], [0, 0, 0, 0, 0, 0, 0, -1, 0], [1, 1, 0, -1, -1, 0, 0, 0, 0], [0, 0, 0, 0, -1, 0, 0, 0, 0], [0, 0, 0, 0, 0, 1, 0, 1, -1], [0, 0, 0, 0, 1, -1, 0, -1, 1], [1, 1, 0, 0, 0, 0, 1, 1, 0], [0, 0, 0, 0, -1, 0, 0, 0, 0], [0, 0, 1, 0, 0, 0, 0, -1, 1], [0, 1, -1, 0, 0, 0, 0, 1, -1], [0, 0, 0, 0, 0, 0, 0, -1, 1]])
Sc = dict(m=4, k=3, n=3,
    a_prog=[(1, 1, 3, -1), (10, -1, 3, 1), (2, 1, 6, 1), (5, 1, 7, 1), (9, 1, 3, 1), (16, 1, 0, 1), (2, -1, 17, 1), (9, -1, 18, 1), (4, 1, 1, 1), (20, 1, 10, 1), (20, 1, 5, 1), (7, -1, 21, 1), (22, 1, 10, 1), (8, -1, 5, 1), (11, 1, 25, 1), (6, 1, 25, 1), (11, 1, 27, 1), (28, 1, 10, -1), (29, 1, 9, -1), (2, 1, 7, 1), (8, 1, 31, 1), (23, 1, 12, -1), (10, -1, 33, 1), (6, 1, 0, 1), (1, 1, 35, 1), (24, -1, 18, 1), (37, 1, 11, -1)],
    a_use=[15, 30, 27, 34, 5, 7, 6, 32, 3, 2, 14, 12, 19, 36, 28, 1, 13, 16, 10, 11, 18, 22, 38, 1, 17, 23, 24, 26, 21],
    c_prog=[(4, 1, 7, 1), (7, 1, 9, -1), (11, -1, 5, 1), (5, -1, 2, 1), (6, 1, 3, 1), (4, 1, 10, -1), (4, -1, 1, 1), (8, -1, 0, 1), (11, 1, 1, 1), (9, -1, 17, 1), (8, -1, 16, 1), (15, -1, 0, 1), (11, 1, 12, 1), (23, 1, 14, -1), (17, -1, 24, 1), (18, 1, 21, 1), (9, 1, 22, 1), (3, -1, 28, 1), (6, 1, 7, 1), (30, -1, 0, 1), (22, 1, 24, -1), (14, -1, 32, 1), (23, 1, 3, -1), (21, -1, 34, 1), (20, 1, 19, 1), (36, 1, 25, -1)],
    c_use=[(22, 1), (9, -1), (29, -1), (3, 1), (33, -1), (16, -1), (31, -1), (8, 1), (35, 1), (37, 1), (19, -1), (23, -1), (25, -1), (0, 1), (13, 1), (15, 1), (21, -1), (27, -1), (17, -1), (26, 1), (20, -1), (14, 1), (11, 1), (18, 1), (1, -1), (7, -1), (24, -1), (7, 1), (12, -1)],
    w=[[0, 0, 0, 0, 0, -1, 1, 0, 1], [1, -1, 0, 0, 0, 0, 0, 0, 0], [0, 0, 0, 0, 0, 0, 1, 0, 0], [0, 0, 0, 1, 0, 0, 0, 0, 0], [0, 0, 0, 0, 0, -1, 0, 0, 1], [0, 0, 0, -1, 0, -1, 1, 0, 1], [1, 0, 0, 0, 0, 0, 1, 0, 0], [0, 0, 0, 0, 0, 0, 1, 0, 1], [-1, 0, 0, 1, 0, 0, 0, 0, 0], [0, 0, 1, 0, 0, 0, 0, 0, 1], [0, 0, 1, 0, 0, 0, -1, 0, 0], [1, 0, 1, -1, 0, 0, 0, 0, 0], [0, 0, 1, 0, 0, 0, 0, 0, 0], [1, 0, 1, 0, 0, 0, 0, 0, 0], [-1, 1, 0, 0, 0, 0, -1, 0, 0], [-1, 0, -1, 1, 0, 1, 0, 0, 0], [1, -1, 0, -1, 0, 0, 0, 0, 0], [0, 1, 0, 0, 0, 0, 0, 0, 0], [1, -1, 0, -1, 1, 0, 0, 0, 0], [0, 0, 0, 0, 0, 0, 0, 1, 0], [0, 0, -1, 0, 0, 0, 0, 1, -1], [0, 0, 0, 0, 0, 1, 0, 0, 0], [0, 0, 0, 0, 0, 0, 0, 1, -1], [0, 0, 0, 0, 1, 0, 0, 0, 0], [0, -1, 1, 0, 0, 0, 0, -1, 1], [0, 0, 0, 0, 1, 0, 0, 0, 0], [0, 0, 0, 0, 0, -1, 0, -1, 1], [1, -1, 0, 0, 0, 0, 1, -1, 0], [0, 0, 0, 0, -1, 1, 0, 1, -1]])
Sd = dict(m=4, k=3, n=3,
    a_prog=[(10, -1, 3, 1), (6, -1, 3, 1), (3, 1, 7, -1), (5, -1, 1, 1), (11, -1, 0, 1), (9, -1, 13, 1), (11, -1, 17, 1), (6, 1, 18, 1), (10, -1, 4, 1), (5, 1, 20, 1), (7, -1, 20, 1), (21, 1, 7, -1), (22, 1, 1, 1), (2, 1, 5, 1), (8, -1, 25, 1), (0, 1, 25, 1), (8, -1, 27, 1), (1, 1, 12, -1), (29, 1, 20, 1), (2, 1, 11, 1), (1, 1, 31, 1), (8, -1, 23, 1), (33, 1, 18, 1), (28, 1, 13, 1), (14, -1, 35, 1), (12, 1, 19, -1), (16, 1, 37, 1)],
    a_use=[1, 5, 32, 15, 27, 0, 30, 3, 11, 16, 12, 19, 38, 23, 10, 14, 21, 13, 8, 7, 10, 22, 24, 18, 34, 36, 17, 26, 28],
    c_prog=[(4, 1, 7, 1), (0, 1, 3, -1), (4, 1, 10, 1), (2, 1, 9, 1), (10, 1, 8, 1), (5, 1, 8, 1), (5, 1, 11, 1), (4, -1, 1, 1), (6, -1, 1, 1), (18, 1, 9, 1), (2, 1, 13, 1), (6, 1, 12, 1), (8, 1, 19, 1), (23, 1, 14, -1), (24, 1, 12, 1), (17, 1, 21, -1), (2, 1, 10, -1), (28, 1, 11, -1), (22, 1, 24, 1), (30, 1, 17, -1), (23, 1, 21, 1), (32, 1, 3, 1), (2, 1, 0, 1), (34, 1, 6, 1), (0, 1, 1, 1), (36, 1, 9, -1)],
    c_use=[(13, -1), (31, -1), (2, -1), (22, -1), (35, 1), (37, 1), (3, 1), (33, 1), (29, 1), (15, 1), (21, 1), (27, 1), (9, -1), (24, -1), (18, 1), (23, -1), (17, -1), (25, 1), (26, -1), (12, -1), (14, 1), (19, -1), (1, -1), (16, 1), (8, 1), (6, -1), (10, 1), (1, 1), (20, -1)],
    w=[[0, 0, 0, -1, 0, 1, 1, 0, -1], [0, 0, 0, 0, 0, -1, 0, 0, 1], [0, 0, 0, 0, 0, 0, 1, 0, -1], [0, 0, 0, 0, 0, -1, -1, 0, 1], [0, 0, 0, 0, 0, 0, 1, 0, 0], [1, 0, 0, 0, 0, 0, -1, 0, 0], [0, 0, 0, 1, 0, 0, 0, 0, 0], [1, 0, 0, 1, 0, 0, 0, 0, 0], [0, 0, 1, 0, 0, 0, 0, 0, -1], [0, 0, 1, 0, 0, 0, -1, 0, 0], [-1, 0, 1, -1, 0, 0, 0, 0, 0], [0, 0, 1, 0, 0, 0, 0, 0, 0], [-1, 0, 1, 0, 0, 0, 0, 0, 0], [0, 0, 0, 0, 0, 1, 0, 1, -1], [-1, 0, 1, -1, 0, 1, 0, 0, 0], [1, -1, 0, 1, 0, 0, 0, 0, 0], [0, 0, 0, 0, 0, -1, 0, 0, 0], [0, -1, 0, 0, 0, 0, 0, 0, 0], [0, 0, 0, 0, 0, 0, 0, -1, 0], [1, -1, 0, 1, -1, 0, 0, 0, 0], [0, 0, 0, 0, 1, 0, 0, 0, 0], [0, 0, 0, 0, 1, -1, 0, -1, 1], [0, 0, 0, 0, -1, 0, 0, 0, 0], [0, 0, -1, 0, 0, 0, 0, -1, 1], [0, 0, 0, 0, 0, 0, 0, 1, -1], [1, -1, 0, 0, 0, 0, 0, 0, 0], [0, -1, 1, 0, 0, 0, 0, 1, -1], [1, -1, 0, 0, 0, 0, -1, 1, 0], [1, -1, 0, 0, 0, 0, -1, 0, 0]])
H2 = dict(m=2, k=3, n=3,
    a_prog=[(5, 1, 4, 1), (5, -1, 3, 1), (2, -1, 0, 1), (3, -1, 0, 1), (3, -1, 2, 1), (5, -1, 2, 1), (1, -1, 0, 1), (9, 1, 1, -1), (11, 1, 4, -1), (14, 1, 1, 1), (4, 1, 13, 1)],
    a_use=[3, 13, 16, 12, 7, 4, 6, 14, 15, 1, 2, 8, 9, 10, 11],
    c_prog=[(0, 1, 5, -1), (5, 1, 3, 1), (0, 1, 3, 1), (1, 1, 2, -1), (4, -1, 3, 1), (0, 1, 2, 1), (5, 1, 2, 1), (5, -1, 9, 1), (8, 1, 4, -1), (14, 1, 1, -1), (4, 1, 13, 1)],
    c_use=[(8, 1), (14, -1), (10, -1), (15, 1), (7, 1), (4, -1), (16, -1), (13, 1), (9, 1), (1, 1), (12, 1), (11, 1), (0, -1), (6, 1), (5, 1)],
    w=[[1, 1, 0, 0, 0, 0, 1, 0, 0], [0, -1, 0, 1, 0, 0, 0, 0, 0], [0, 0, 0, -1, 0, 0, 0, 0, 0], [0, -1, 0, 0, 0, 0, 0, 0, 0], [0, 0, 0, 0, 0, 0, -1, 0, 0], [0, 0, 0, -1, -1, 0, 0, 1, 0], [0, 0, 0, 0, 0, 0, 0, -1, 0], [0, 0, 0, 0, 0, 1, 0, 1, 0], [0, 0, 0, 0, 0, -1, 0, 0, 0], [0, 1, 0, 0, 1, 1, 0, 0, 0], [0, 0, 1, 0, 0, 0, 0, 1, 1], [0, 0, 1, 0, 0, 0, 0, 0, 0], [-1, 0, 1, -1, 0, 0, 0, 0, 0], [0, 0, 1, 0, 0, 0, 1, 0, 0], [0, 0, 0, 0, 0, 1, 1, 0, -1]])
H3 = dict(m=2, k=3, n=3,
    a_prog=[(5, 1, 4, 1), (5, -1, 3, 1), (0, 1, 2, -1), (0, 1, 3, -1), (2, 1, 3, -1), (5, -1, 2, 1), (0, 1, 1, -1), (9, 1, 1, -1), (4, -1, 11, 1), (1, 1, 14, 1), (4, 1, 13, 1)],
    a_use=[1, 12, 13, 16, 4, 6, 3, 7, 14, 15, 2, 8, 9, 10, 11],
    c_prog=[(5, -1, 0, 1), (3, 1, 5, 1), (3, 1, 0, 1), (2, -1, 1, 1), (3, 1, 4, -1), (2, 1, 0, 1), (2, 1, 5, 1), (5, -1, 9, 1), (10, 1, 0, 1), (1, -1, 14, 1), (13, 1, 4, 1)],
    c_use=[(1, -1), (15, 1), (14, -1), (10, 1), (4, -1), (16, 1), (8, -1), (7, 1), (13, -1), (9, -1), (12, 1), (11, 1), (0, 1), (6, -1), (5, 1)],
    w=[[0, -1, 0, 0, -1, -1, 0, 0, 0], [0, -1, 0, 0, 0, 0, 0, 0, 0], [0, -1, 0, 1, 0, 0, 0, 0, 0], [0, 0, 0, 1, 0, 0, 0, 0, 0], [0, 0, 0, -1, -1, 0, 0, 1, 0], [0, 0, 0, 0, 0, 0, 0, 1, 0], [-1, -1, 0, 0, 0, 0, -1, 0, 0], [0, 0, 0, 0, 0, 0, -1, 0, 0], [0, 0, 0, 0, 0, -1, 0, -1, 0], [0, 0, 0, 0, 0, 1, 0, 0, 0], [0, 0, 1, 0, 0, 0, 0, 1, 1], [0, 0, 1, 0, 0, 0, 0, 0, 0], [1, 0, -1, 1, 0, 0, 0, 0, 0], [0, 0, -1, 0, 0, 0, -1, 0, 0], [0, 0, 0, 0, 0, 1, 1, 0, -1]])

Se = {'m': 4, 'k': 3, 'n': 3, 'a_prog': [(10, -1, 3, 1), (6, -1, 3, 1), (3, 1, 7, -1), (5, -1, 1, 1), (11, -1, 0, 1), (9, -1, 13, 1), (11, -1, 17, 1), (6, 1, 18, 1), (10, -1, 4, 1), (5, 1, 20, 1), (7, -1, 20, 1), (21, 1, 7, -1), (22, 1, 1, 1), (2, 1, 5, 1), (8, -1, 25, 1), (0, 1, 25, 1), (8, -1, 27, 1), (1, 1, 12, -1), (29, 1, 20, 1), (2, 1, 11, 1), (1, 1, 31, 1), (8, -1, 23, 1), (33, 1, 18, 1), (28, 1, 13, 1), (14, -1, 35, 1), (12, 1, 19, -1), (16, 1, 37, 1)], 'a_use': [5, 27, 32, 15, 0, 1, 30, 3, 16, 11, 12, 19, 38, 10, 14, 21, 13, 23, 8, 7, 10, 22, 18, 34, 24, 17, 26, 28, 36], 'c_prog': [(4, 1, 7, 1), (0, 1, 3, -1), (4, 1, 10, 1), (2, 1, 9, 1), (10, 1, 8, 1), (5, 1, 8, 1), (5, 1, 11, 1), (4, -1, 1, 1), (6, -1, 1, 1), (18, 1, 9, 1), (2, 1, 13, 1), (6, 1, 12, 1), (8, 1, 19, 1), (23, 1, 14, -1), (24, 1, 12, 1), (17, 1, 21, -1), (2, 1, 10, -1), (28, 1, 11, -1), (22, 1, 24, 1), (30, 1, 17, -1), (23, 1, 21, 1), (32, 1, 3, 1), (2, 1, 0, 1), (34, 1, 6, 1), (0, 1, 1, 1), (36, 1, 9, -1)], 'c_use': [(31, 1), (35, 1), (2, 1), (22, -1), (37, 1), (13, -1), (3, -1), (33, 1), (15, -1), (29, 1), (21, 1), (27, 1), (9, 1), (18, 1), (23, -1), (17, 1), (25, 1), (24, -1), (26, -1), (12, 1), (14, -1), (19, -1), (16, 1), (8, -1), (1, 1), (10, -1), (1, -1), (20, 1), (6, -1)], 'w': [[0, 0, 0, 0, 0, 1, 0, 0, -1], [0, 0, 0, 0, 0, 0, 1, 0, 0], [0, 0, 0, 0, 0, 0, -1, 0, 1], [0, 0, 0, 0, 0, -1, -1, 0, 1], [1, 0, 0, 0, 0, 0, -1, 0, 0], [0, 0, 0, -1, 0, 1, 1, 0, -1], [0, 0, 0, -1, 0, 0, 0, 0, 0], [1, 0, 0, 1, 0, 0, 0, 0, 0], [0, 0, -1, 0, 0, 0, 1, 0, 0], [0, 0, 1, 0, 0, 0, 0, 0, -1], [-1, 0, 1, -1, 0, 0, 0, 0, 0], [0, 0, 1, 0, 0, 0, 0, 0, 0], [1, 0, -1, 0, 0, 0, 0, 0, 0], [-1, 0, 1, -1, 0, 1, 0, 0, 0], [1, -1, 0, 1, 0, 0, 0, 0, 0], [0, 0, 0, 0, 0, 1, 0, 0, 0], [0, -1, 0, 0, 0, 0, 0, 0, 0], [0, 0, 0, 0, 0, 1, 0, 1, -1], [0, 0, 0, 0, 0, 0, 0, -1, 0], [-1, 1, 0, -1, 1, 0, 0, 0, 0], [0, 0, 0, 0, -1, 0, 0, 0, 0], [0, 0, 0, 0, 1, -1, 0, -1, 1], [0, 0, -1, 0, 0, 0, 0, -1, 1], [0, 0, 0, 0, 0, 0, 0, -1, 1], [0, 0, 0, 0, 1, 0, 0, 0, 0], [0, 1, -1, 0, 0, 0, 0, -1, 1], [-1, 1, 0, 0, 0, 0, 1, -1, 0], [-1, 1, 0, 0, 0, 0, 1, 0, 0], [1, -1, 0, 0, 0, 0, 0, 0, 0]]}

Sf = {'m': 4, 'k': 3, 'n': 3, 'a_prog': [(10, -1, 3, 1), (6, -1, 3, 1), (3, 1, 7, -1), (5, -1, 1, 1), (11, -1, 0, 1), (9, -1, 13, 1), (11, -1, 17, 1), (6, 1, 18, 1), (10, -1, 4, 1), (5, 1, 20, 1), (7, -1, 20, 1), (21, 1, 7, -1), (22, 1, 1, 1), (2, 1, 5, 1), (8, -1, 25, 1), (0, 1, 25, 1), (8, -1, 27, 1), (1, 1, 12, -1), (29, 1, 20, 1), (2, 1, 11, 1), (1, 1, 31, 1), (8, -1, 23, 1), (33, 1, 18, 1), (28, 1, 13, 1), (14, -1, 35, 1), (12, 1, 19, -1), (16, 1, 37, 1)], 'a_use': [5, 0, 27, 32, 1, 3, 30, 11, 15, 16, 10, 14, 12, 19, 38, 21, 13, 8, 7, 10, 23, 18, 22, 34, 24, 26, 28, 17, 36], 'c_prog': [(4, 1, 7, 1), (0, 1, 3, -1), (4, 1, 10, 1), (2, 1, 9, 1), (10, 1, 8, 1), (5, 1, 8, 1), (5, 1, 11, 1), (4, -1, 1, 1), (6, -1, 1, 1), (18, 1, 9, 1), (2, 1, 13, 1), (6, 1, 12, 1), (8, 1, 19, 1), (23, 1, 14, -1), (24, 1, 12, 1), (17, 1, 21, -1), (2, 1, 10, -1), (28, 1, 11, -1), (22, 1, 24, 1), (30, 1, 17, -1), (23, 1, 21, 1), (32, 1, 3, 1), (2, 1, 0, 1), (34, 1, 6, 1), (0, 1, 1, 1), (36, 1, 9, -1)], 'c_use': [(31, -1), (37, -1), (35, 1), (2, -1), (13, -1), (33, -1), (3, -1), (29, -1), (22, -1), (15, 1), (18, 1), (23, -1), (21, 1), (27, 1), (9, -1), (17, 1), (25, -1), (26, 1), (12, 1), (14, -1), (24, -1), (16, 1), (19, -1), (8, -1), (1, -1), (1, 1), (20, -1), (10, -1), (6, -1)], 'w': [[0, 0, 0, 0, 0, -1, 0, 0, 1], [-1, 0, 0, 0, 0, 0, 1, 0, 0], [0, 0, 0, 0, 0, 0, 1, 0, 0], [0, 0, 0, 0, 0, 0, 1, 0, -1], [0, 0, 0, -1, 0, 1, 1, 0, -1], [-1, 0, 0, -1, 0, 0, 0, 0, 0], [0, 0, 0, -1, 0, 0, 0, 0, 0], [0, 0, -1, 0, 0, 0, 0, 0, 1], [0, 0, 0, 0, 0, -1, -1, 0, 1], [0, 0, 1, 0, 0, 0, -1, 0, 0], [-1, 0, 1, -1, 0, 1, 0, 0, 0], [1, -1, 0, 1, 0, 0, 0, 0, 0], [-1, 0, 1, -1, 0, 0, 0, 0, 0], [0, 0, 1, 0, 0, 0, 0, 0, 0], [-1, 0, 1, 0, 0, 0, 0, 0, 0], [0, 0, 0, 0, 0, 1, 0, 0, 0], [0, 1, 0, 0, 0, 0, 0, 0, 0], [0, 0, 0, 0, 0, 0, 0, 1, 0], [-1, 1, 0, -1, 1, 0, 0, 0, 0], [0, 0, 0, 0, -1, 0, 0, 0, 0], [0, 0, 0, 0, 0, 1, 0, 1, -1], [0, 0, -1, 0, 0, 0, 0, -1, 1], [0, 0, 0, 0, 1, -1, 0, -1, 1], [0, 0, 0, 0, 0, 0, 0, -1, 1], [0, 0, 0, 0, -1, 0, 0, 0, 0], [1, -1, 0, 0, 0, 0, -1, 1, 0], [1, -1, 0, 0, 0, 0, -1, 0, 0], [0, 1, -1, 0, 0, 0, 0, -1, 1], [1, -1, 0, 0, 0, 0, 0, 0, 0]]}

Sg = {'m': 4, 'k': 3, 'n': 3, 'a_prog': [(10, -1, 3, 1), (6, -1, 3, 1), (3, 1, 7, -1), (5, -1, 1, 1), (11, -1, 0, 1), (9, -1, 13, 1), (11, -1, 17, 1), (6, 1, 18, 1), (10, -1, 4, 1), (5, 1, 20, 1), (7, -1, 20, 1), (21, 1, 7, -1), (22, 1, 1, 1), (2, 1, 5, 1), (8, -1, 25, 1), (0, 1, 25, 1), (8, -1, 27, 1), (1, 1, 12, -1), (29, 1, 20, 1), (2, 1, 11, 1), (1, 1, 31, 1), (8, -1, 23, 1), (33, 1, 18, 1), (28, 1, 13, 1), (14, -1, 35, 1), (12, 1, 19, -1), (16, 1, 37, 1)], 'a_use': [5, 0, 27, 1, 32, 15, 30, 3, 11, 16, 10, 14, 12, 19, 21, 38, 13, 7, 8, 10, 23, 18, 22, 34, 24, 28, 26, 17, 36], 'c_prog': [(4, 1, 7, 1), (0, 1, 3, -1), (4, 1, 10, 1), (2, 1, 9, 1), (10, 1, 8, 1), (5, 1, 8, 1), (5, 1, 11, 1), (4, -1, 1, 1), (6, -1, 1, 1), (18, 1, 9, 1), (2, 1, 13, 1), (6, 1, 12, 1), (8, 1, 19, 1), (23, 1, 14, -1), (24, 1, 12, 1), (17, 1, 21, -1), (2, 1, 10, -1), (28, 1, 11, -1), (22, 1, 24, 1), (30, 1, 17, -1), (23, 1, 21, 1), (32, 1, 3, 1), (2, 1, 0, 1), (34, 1, 6, 1), (0, 1, 1, 1), (36, 1, 9, -1)], 'c_use': [(31, -1), (37, -1), (35, 1), (13, -1), (2, -1), (22, -1), (3, -1), (33, -1), (29, -1), (15, 1), (18, 1), (23, -1), (21, 1), (27, 1), (17, -1), (9, 1), (25, -1), (12, 1), (26, 1), (14, -1), (24, -1), (16, 1), (19, -1), (8, -1), (1, -1), (20, 1), (1, -1), (10, -1), (6, -1)], 'w': [[0, 0, 0, 0, 0, -1, 0, 0, 1], [-1, 0, 0, 0, 0, 0, 1, 0, 0], [0, 0, 0, 0, 0, 0, 1, 0, 0], [0, 0, 0, -1, 0, 1, 1, 0, -1], [0, 0, 0, 0, 0, 0, 1, 0, -1], [0, 0, 0, 0, 0, -1, -1, 0, 1], [0, 0, 0, -1, 0, 0, 0, 0, 0], [-1, 0, 0, -1, 0, 0, 0, 0, 0], [0, 0, -1, 0, 0, 0, 0, 0, 1], [0, 0, 1, 0, 0, 0, -1, 0, 0], [-1, 0, 1, -1, 0, 1, 0, 0, 0], [1, -1, 0, 1, 0, 0, 0, 0, 0], [-1, 0, 1, -1, 0, 0, 0, 0, 0], [0, 0, 1, 0, 0, 0, 0, 0, 0], [0, 0, 0, 0, 0, -1, 0, 0, 0], [1, 0, -1, 0, 0, 0, 0, 0, 0], [0, 1, 0, 0, 0, 0, 0, 0, 0], [-1, 1, 0, -1, 1, 0, 0, 0, 0], [0, 0, 0, 0, 0, 0, 0, 1, 0], [0, 0, 0, 0, -1, 0, 0, 0, 0], [0, 0, 0, 0, 0, 1, 0, 1, -1], [0, 0, -1, 0, 0, 0, 0, -1, 1], [0, 0, 0, 0, 1, -1, 0, -1, 1], [0, 0, 0, 0, 0, 0, 0, -1, 1], [0, 0, 0, 0, -1, 0, 0, 0, 0], [-1, 1, 0, 0, 0, 0, 1, 0, 0], [-1, 1, 0, 0, 0, 0, 1, -1, 0], [0, 1, -1, 0, 0, 0, 0, -1, 1], [1, -1, 0, 0, 0, 0, 0, 0, 0]]}


SCHEMES = dict(S433=S433, S343=S343, HK=HK, Se=Se, Sf=Sf, Sg=Sg)


def gelu(y):
    return y * jnp.tanh(y * (y * y + C0)) + y


def lhs_operands(sc, block):
    m, k = sc["m"], sc["k"]
    memo, packed = {}, {}

    def node(v):
        if v not in memo:
            if v < m * k:
                memo[v] = (1, block(v // k, v % k))
            else:
                a, sa, b, sb = sc["a_prog"][v - m * k]
                (ta, xa), (tb, xb) = node(a), node(b)
                ta, tb = ta * sa, tb * sb
                memo[v] = (ta, xa + xb) if ta == tb else (1, xa - xb if ta > 0 else xb - xa)
        return memo[v]

    def op(p):
        v = sc["a_use"][p]
        if v not in packed:
            packed[v] = node(v)[1].astype(BF16)
        return packed[v]
    return op


def combine(sc, product, emit):
    m, n = sc["m"], sc["n"]
    fan = [0] * (m * n + len(sc["c_prog"]))
    for v, _ in sc["c_use"]:
        fan[v] += 1
    for a, _, b, _ in sc["c_prog"]:
        fan[a] += 1
        fan[b] += 1
    val = {}

    def push(v, t, x):
        if v in val:
            u, y = val[v]
            t, x = (t, y + x) if t == u else (1, x - y if t > 0 else y - x)
        val[v] = (t, x)
        fan[v] -= 1
        if fan[v] == 0:
            del val[v]
            if v >= m * n:
                a, sa, b, sb = sc["c_prog"][v - m * n]
                push(a, t * sa, x)
                push(b, t * sb, x)
            else:
                assert t == 1
                emit(v // n, v % n, x)

    for p, (v, t) in enumerate(sc["c_use"]):
        push(v, t, product(p))


def weight_form(sc, p, tile):
    n, acc = sc["n"], None
    for q in sorted(range(len(sc["w"][p])), key=lambda q: -sc["w"][p][q]):
        c = sc["w"][p][q]
        if c:
            v = tile(q // n, q % n)
            acc = (v if c > 0 else -v) if acc is None else (acc + v if c > 0 else acc - v)
    return acc


def make(CH=768, G1=4, G2=2, S=52, XC=8, XR2=4, MC1=48, MC2=48, mode2="k", vmem_mb=128, flags=None, E1=2, E2=2,
         run1=True, run2=True, dma=True, comp=True, pipe=True, PT=0, OFF=0, MCR=64, PADV=0, XW=C, RX=2, RB=2, OR=1, HL=False, RCH=256, nobc=False, TD=3, MID=True, LEAD=1, YB=0, YD=0, LNR=16, F0=0.0, F1=0.65, F2=0.68, F3=0.97, sc1='S433', sc2='HK', rs=1, PX=0, PH=0, PO=0, A1=1, B1=1, A2=1, B2=1):
    sc1, sc2 = (SCHEMES[z] if isinstance(z, str) else z for z in (sc1, sc2))
    NP1, NP2 = len(sc1["w"]), len(sc2["w"])
    PR = sc1["m"] * MC1
    KG2 = 12 // sc2["k"]
    TM1, TM2 = CH * G1, CH * G2
    XT = max(XC * CH, XR2 * TM2)
    W1ROW = (XT - HID - PR) // CH * CH

    @jax.jit
    def fn(x, dw, w1, w2, grn_g, grn_b):
        B, H, W, _ = x.shape
        N = B * H * W
        NT1, NT2 = N // TM1, N // TM2
        NCH = N // CH
        NHC = NCH - S
        R1 = -(-NHC * 65536 // (NT1 - E1))
        R2 = -(-NHC * 65536 * 2 // int(2 * NT2 - 2 * E2))
        PER, RF = PT * G2, OFF * G2
        NREC = len(range(RF, NHC, PER)) if PT else 0
        assert R1 <= G1 * 65536 and R2 <= G2 * 65536 and S >= 2 * max(G1, G2) and TM1 >= HID and E1 >= 2 and E2 >= (1.5 if MID and G2 == 2 else 2) and TD < XR2
        last = [(NCH - G1 + u) % XC for u in range(G1)]
        W2U, W2S = next((u, s0) for u in range(G1) for s0 in range(XC - 1)
                        if all(t not in last[u + 1:] for t in (s0, s0 + 1)))
        W2ROW = W2S * CH
        assert 2 * CH >= HID and XC >= G1

        def kernel(x_hbm, dw_ref, w1_hbm, w2_hbm, g_ref, b_ref, out_hbm, h_hbm,
                   xbuf, hbuf, ws, ssq, vec, abuf, w1p, ybuf, xsem, osem, hsem, wsem):
            class _Nop:
                def start(self, priority=0): pass
                def wait(self): pass
            mk = pltpu.make_async_copy if dma else (lambda *a: _Nop())

            def xrows(slot, tm):
                return xbuf.at[pl.ds(pl.multiple_of(slot * tm, tm), tm), pl.ds(0, C)]

            def x_copy(i, slot, tm):
                return mk(x_hbm.at[pl.ds(i * tm, tm)], xrows(slot, tm), xsem.at[slot])

            def o_copy(i, slot):
                return mk(xrows(slot, TM2), out_hbm.at[pl.ds(i * TM2, TM2)], osem.at[slot])

            def stored(c):
                return (c + (PER - RF)) % PER != 0 if PT else True

            def h_index(c):
                return c - (c + (PER - 1 - RF)) // PER if PT else c

            def h_out(c, slot):
                return mk(hbuf.at[slot], h_hbm.at[h_index(c)], hsem.at[slot])

            def h_in(c, slot):
                return mk(h_hbm.at[h_index(c)], hbuf.at[slot], hsem.at[slot])

            def w1_copy(q):
                return pltpu.make_async_copy(w1_hbm.at[:, pl.ds(q * C, C)], xbuf.at[pl.ds(W1ROW + q * C, C), pl.ds(0, C)], wsem.at[q])

            def w2_copy():
                return pltpu.make_async_copy(w2_hbm, xbuf.at[pl.ds(W2ROW, HID), pl.ds(0, C)], wsem.at[0])

            def wrap(v, n):
                return jnp.where(v >= n, v - n, v)

            def wrapn(v, n):
                return jnp.where(v < 0, v + n, v)

            def x0_copy():
                return pltpu.make_async_copy(x_hbm.at[pl.ds(0, PR)], xbuf.at[pl.ds(W1ROW + HID, PR), pl.ds(0, C)], osem.at[0])

            for q in range(4):
                w1_copy(q).start()
            x0_copy().start()
            ssq[...] = jnp.zeros_like(ssq)
            vec[0:8, :] = jnp.broadcast_to(dw_ref[...].astype(F32), (8, C))
            NPRE = W1ROW // CH
            for c in range(NPRE):
                pltpu.make_async_copy(x_hbm.at[pl.ds(c * CH + PR, CH)], xbuf.at[pl.ds(c * CH, CH), pl.ds(0, C)], xsem.at[c]).start() if dma else None
            for q in range(4):
                w1_copy(q).wait()

            def w1_tile(k, n):
                r = W1ROW + (n // 3) * C + k * L
                return xbuf[r:r + L, (n % 3) * L:(n % 3 + 1) * L].astype(F32)

            for c in range(4):
                for p in range(NP1):
                    ws[p * 4 + c] = pk(weight_form(sc1, p, lambda k, j: w1_tile(k, 4 * j + c)))

            if PT:
                for k in range(3):
                    for n in range(HID // L):
                        w1p[k * 64:(k + 1) * 64, n * L:(n + 1) * L] = pk(w1_tile(k, n))

            def layernorm(row, n=LNR):
                y = xbuf[pl.ds(pl.multiple_of(row, 16), n), :C].astype(F32) * jnp.concatenate([vec[0:8, :]] * (n // 8), axis=0)
                mu = jnp.sum(y, axis=-1, keepdims=True) * (1.0 / C)
                d = y - mu
                ss = jnp.sum(d * d, axis=-1, keepdims=True)
                v = ss * (1.0 / (C * ALPHA * ALPHA)) + 1e-5 / (ALPHA * ALPHA)
                if rs == 0:
                    return d * lax.rsqrt(v)
                return d * jnp.exp2(-0.5 * jnp.log2(v))

            def act(y, hs, r0, c):
                h = gelu(y)
                ssq[:, c * L:(c + 1) * L] += jnp.sum((h * h).reshape(MC1 // 8, 8, L), axis=0)
                if HL:
                    hbuf[hs, c, pl.ds(r0 // 2, MC1 // 2), :] = pack16(h)
                else:
                    hbuf[hs, pl.ds(r0 // 2, MC1 // 2), c * L:(c + 1) * L] = pack16(h)

            def operands(row):
                nl = MC1 // LNR
                a = {}
                def ln(t, q):
                    a[t, q] = layernorm(row + t * MC1 + q * LNR)
                op = lhs_operands(sc1, lambda t, k: jnp.concatenate([a[t, q][:, k * L:(k + 1) * L] for q in range(nl)], axis=0))
                lns = [functools.partial(ln, t, q) for t in range(sc1["m"]) for q in range(nl)]
                forms = [functools.partial(op, p) for p in range(NP1)]
                return op, lns, forms

            NB1 = TM1 // (PR)

            PPC = CH // PR

            def xc_copy(c, slot, n=CH):
                return mk(x_hbm.at[pl.ds(c * CH + PR, n)], xbuf.at[pl.ds(pl.multiple_of(slot * CH, CH), n), pl.ds(0, C)], xsem.at[slot])

            def xc_do(c, slot, what):
                @pl.when(c < NCH - 1)
                def _():
                    what(xc_copy(c, slot))
                @pl.when(c == NCH - 1)
                def _():
                    what(xc_copy(c, slot, CH - PR))

            def stage(row):
                for t in range(sc1["m"]):
                    abuf[t * MC1:(t + 1) * MC1, :] = layernorm(row + t * MC1, MC1)

            def phase1(i, carry):
                xb, hb, q, qs = carry
                slots = [wrap(hb + u, S) for u in range(G1)]
                xsl = [wrap(xb + u, XC) for u in range(G1)]
                qn = jnp.minimum((i * R1) >> 16, NHC)
                for u in range(G1):
                    xc_do(i * G1 + u, xsl[u], lambda cp: cp.wait())
                    @pl.when(jnp.logical_and(i * G1 + u >= S, stored(jnp.maximum(i * G1 + u - S, 0))))
                    def _():
                        h_out(i * G1 + u - S, slots[u]).wait()
                for u in range(G1):
                    @pl.when(jnp.logical_and(q + u < qn, stored(q + u)))
                    def _():
                        h_out(q + u, wrap(qs + u, S)).start()

                nxt = None
                parked = []
                park_product = lambda f: f
                def flush():
                    b, t, j, hs, r0, col = parked.pop(0)
                    act(ybuf[b, t * 3 + j], hs, r0, col)
                for m in range(NB1 if comp else 0):
                    u, r = divmod(m * PR, CH)
                    op = lhs_operands(sc1, lambda t, k: abuf[t * MC1:(t + 1) * MC1, k * L:(k + 1) * L]) if m == 0 else nxt
                    nxt, lns, forms = operands(xsl[u] * CH + r)
                    if m == NB1 - 1:
                        def put(t):
                            abuf[t * MC1:(t + 1) * MC1, :] = layernorm(xsl[u] * CH + r + t * MC1, MC1)
                        lns, forms = [functools.partial(put, t) for t in range(sc1["m"])], []
                    ns = 4 * NP1
                    todo = {}
                    for e, f in enumerate(lns):
                        todo.setdefault(int(ns * (F0 + (F1 - F0) * e / len(lns))), []).append(f)
                    for e, f in enumerate(forms):
                        todo.setdefault(int(ns * (F2 + (F3 - F2) * e / len(forms))), []).append(f)
                    for c in range(4):
                        def product(p):
                            for f in todo.pop(c * NP1 + p, []):
                                f()
                            return jnp.dot(op(p), upk(ws[p * 4 + c]), preferred_element_type=F32)
                        if YB == 0:
                            combine(sc1, product, lambda t, j, y: act(y, slots[u], r + t * MC1, 4 * j + c))
                        else:
                            def park(t, j, y):
                                ybuf[c % YB, t * 3 + j] = y
                                parked.append((c % YB, t, j, slots[u], r + t * MC1, 4 * j + c))
                                while len(parked) > YD:
                                    flush()
                            combine(sc1, park_product(product), park)
                    assert not todo
                    if (m + 1) % PPC == 0:
                        xc_do(i * G1 + u + XC, xsl[u], lambda cp: cp.start())
                        if u == W2U:
                            @pl.when(i == NT1 - 1)
                            def _():
                                w2_copy().start()
                while parked:
                    flush()
                return wrap(xb + G1, XC), wrap(hb + G1, S), qn, wrap(qs + (qn - q), S)

            z = jnp.int32(0)
            x0_copy().wait()
            stage(W1ROW + HID)
            for c in range(NPRE, XC):
                xc_copy(c, c).start()
            if run1:
                lax.fori_loop(0, NT1, phase1, (z, z, z, z))
            else:
                for c in range(XC):
                    xc_copy(c, c).wait()
                w2_copy().start()

            free2 = [s for s in range(XR2) if (s + 1) * TM2 <= W2ROW or s * TM2 >= W2ROW + HID]
            first2 = [(j, (NT2 - 1 - j) % XR2) for j in range(XR2 - 1)]
            if run2:
                for j, s in first2:
                    if s in free2:
                        x_copy(NT2 - 1 - j, s, TM2).start()
            gx = jnp.sqrt(jnp.sum(ssq[...], axis=0, keepdims=True) * (HS * HS) + 1e-6)
            nx = gx / (jnp.mean(gx, axis=-1, keepdims=True) + 1e-6)
            sc = (g_ref[...].astype(F32) * nx + 1.0) * HS
            w2_copy().wait()
            for r in range(KG2):
                cols = [jnp.broadcast_to(sc[:, (KG2 * k + r) * L:(KG2 * k + r + 1) * L], (L, L)).T for k in range(sc2["k"])]
                tile = lambda k, j: xbuf[W2ROW + (KG2 * k + r) * L:W2ROW + (KG2 * k + r + 1) * L, j * L:(j + 1) * L].astype(F32) * cols[k]
                for p in range(NP2):
                    ws[p * KG2 + r] = pk(weight_form(sc2, p, tile))
            bv = b_ref[...].astype(F32)
            bias = jnp.zeros((8, C), F32)
            for k in range(HID // L):
                col = jnp.broadcast_to(bv[:, k * L:(k + 1) * L], (L, L)).T
                prod = xbuf[W2ROW + k * L:W2ROW + (k + 1) * L, :C].astype(F32) * jnp.concatenate([col] * 3, axis=1)
                bias = bias + jnp.sum(prod.reshape(L // 8, 8, C), axis=0)
            bias = jnp.broadcast_to(jnp.sum(bias, axis=0, keepdims=True), (8, C))
            vec[8:16, :] = bias
            if run2:
                for j, s in first2:
                    if s not in free2:
                        x_copy(NT2 - 1 - j, s, TM2).start()

            def phase2(j, carry):
                xs, hb, q, qs = carry
                i = NT2 - 1 - j
                slots = [wrap(hb + u, S) for u in range(G2)]
                nxs, nhb = wrapn(xs - 1, XR2), wrapn(hb - G2, S)

                s2 = wrap(xs + 2, XR2)
                x_copy(i, xs, TM2).wait()
                for u in range(G2):
                    @pl.when(jnp.logical_and(i * G2 + u < NHC, stored(i * G2 + u)))
                    def _():
                        h_in(i * G2 + u, slots[u]).wait()
                @pl.when(jnp.logical_and(j >= 2, i + 2 > TD))
                def _():
                    o_copy(i + 2, s2).wait()
                @pl.when(jnp.logical_and(j >= 1, i + 1 > TD))
                def _():
                    o_copy(i + 1, wrap(xs + 1, XR2)).start(priority=PO)
                if TD:
                    @pl.when(i == 0)
                    def _():
                        for t in range(TD, 0, -1):
                            o_copy(t, t % XR2).start(priority=PO)
                @pl.when(jnp.logical_and(j >= 1, i + 2 - XR2 >= 0))
                def _():
                    x_copy(i + 2 - XR2, s2, TM2).start(priority=PX)

                if PT and comp:
                    @pl.when(jnp.logical_and(i * G2 < NHC, jnp.logical_not(stored(i * G2))))
                    def _():
                        def rows(g, carry):
                            for r in range(0, RCH, MCR):
                                r = pl.multiple_of(g * RCH + r, MCR)
                                a = layernorm(xs * TM2 + r, MCR).astype(BF16)
                                for n in range(0, HID, 512):
                                    y = jnp.dot(a, upk(w1p[:, n:n + 512]), preferred_element_type=F32)
                                    w = pack16(gelu(y))
                                    rr = pl.ds(pl.multiple_of(r // 2, MCR // 2), MCR // 2)
                                    if HL:
                                        for c in range(4):
                                            hbuf[slots[0], n // L + c, rr, :] = w[:, c * L:(c + 1) * L]
                                    else:
                                        hbuf[slots[0], rr, n:n + 512] = w
                            return carry
                        lax.fori_loop(0, CH // RCH, rows, 0)

                NB2 = TM2 // (sc2['m'] * MC2)
                for mi, m in enumerate(reversed(range(NB2))):
                    if mi % (NB2 // G2) == A2 and (MID or mi == A2):
                        e = mi // (NB2 // G2)
                        qn = jnp.minimum(jnp.minimum((((j * G2 + e) * R2) >> 16) // G2 + LEAD, j * G2 + e), NHC)
                        for u in range(G2):
                            @pl.when(jnp.logical_and(q + u < qn, stored(jnp.maximum(NHC - 1 - q - u, 0))))
                            def _():
                                h_in(NHC - 1 - q - u, wrapn(qs - u, S)).start(priority=PH)
                        qn = jnp.clip(qn, q, q + G2)
                        q, qs = qn, wrapn(qs - (qn - q), S)
                    if not comp:
                        continue
                    r0 = [(sc2['m'] * m + t) * MC2 for t in range(sc2['m'])]
                    orow = lambda t: pl.ds(pl.multiple_of(xs * TM2 + r0[t], 16), MC2)
                    hload = (lambda t, c0, n: unpack16(hbuf[slots[r0[t] // CH], c0 // L, pl.ds(r0[t] % CH // 2, MC2 // 2), :])) if HL else (lambda t, c0, n: unpack16(hbuf[slots[r0[t] // CH], pl.ds(r0[t] % CH // 2, MC2 // 2), c0:c0 + n]))
                    acc = {}
                    for r in range(KG2):
                        op = lhs_operands(sc2, lambda t, k: hload(t, (KG2 * k + r) * L, L))
                        def accum(t, jj, o):
                            cs = slice(jj * L, (jj + 1) * L)
                            terms = [o] if r == 0 else ([acc[t, jj], o] if OR & 1 else [o, acc[t, jj]])
                            extra = ([xbuf[orow(t), cs].astype(F32)] if r == RX else []) + ([jnp.concatenate([vec[8:16, cs]] * (MC2 // 8), axis=0)] if r == RB else [])
                            if OR & 2:
                                extra = extra[::-1]
                            terms = extra + terms if OR & 4 else terms + extra
                            acc[t, jj] = functools.reduce(lambda a, b: a + b, terms)
                            if r == KG2 - 1:
                                xbuf[orow(t), cs] = acc[t, jj].astype(BF16)
                        combine(sc2, lambda p: jnp.dot(op(p), upk(ws[p * KG2 + r]), preferred_element_type=F32), accum)
                return nxs, nhb, q, qs

            if run2:
                lax.fori_loop(0, NT2, phase2, (z + (NT2 - 1) % XR2, z + (NCH - G2) % S, z, z + (NHC - 1) % S))
                o_copy(0, 0).start()
                for t in range(max(TD, 1), -1, -1):
                    o_copy(t, t % XR2).wait()

        out, _ = pl.pallas_call(
            kernel,
            in_specs=[pl.BlockSpec(memory_space=pl.ANY), pl.BlockSpec(memory_space=pltpu.VMEM),
                      pl.BlockSpec(memory_space=pl.ANY), pl.BlockSpec(memory_space=pl.ANY),
                      pl.BlockSpec(memory_space=pltpu.VMEM), pl.BlockSpec(memory_space=pltpu.VMEM)],
            out_specs=[pl.BlockSpec(memory_space=pl.ANY)] * 2,
            out_shape=[jax.ShapeDtypeStruct((N, C), BF16), jax.ShapeDtypeStruct((NHC - NREC,) + ((HID // L, CH // 2, L) if HL else (CH // 2, HID)), U32)],
            scratch_shapes=[
                pltpu.VMEM((XT, XW), BF16),
                pltpu.VMEM((S,) + ((HID // L, CH // 2, L) if HL else (CH // 2, HID)), U32),
                pltpu.VMEM((max(NP1 * 4, NP2 * KG2), L // 2, L), U32),
                pltpu.VMEM((8, HID), F32),
                pltpu.VMEM((16, C), F32),
                pltpu.VMEM((PR, C), F32),
                pltpu.VMEM((C // 2, HID) if PT else (8, L), U32),
                pltpu.VMEM((max(YB, 1), 3 * sc1['m'], MC1 if YB else 8, L), F32),
                pltpu.SemaphoreType.DMA((max(XC, XR2),)),
                pltpu.SemaphoreType.DMA((XR2,)),
                pltpu.SemaphoreType.DMA((S,)),
                pltpu.SemaphoreType.DMA((4,)),
            ],
            compiler_params=pltpu.CompilerParams(vmem_limit_bytes=vmem_mb * 1024 * 1024, flags=flags, disable_bounds_checks=nobc),
        )(x.reshape(N, C), dw.reshape(1, C), w1, w2, grn_g.reshape(1, HID), grn_b.reshape(1, HID))
        return out.reshape(x.shape)
    return fn


pallas_standalone__modern_conv_block_slak__vision_kernel = make(E1=3,E2=1.5,MC1=48,LNR=48,sc1='Sg',nobc=True,sc2='S343',MC2=32,S=52,PT=16,OFF=3,LEAD=1)
```

```python
import functools
import numpy as np
import jax
import jax.numpy as jnp
from jax import lax
import jax.experimental.pallas as pl
import jax.experimental.pallas.tpu as pltpu

C = 384
HID = 1536
L = 128
F32 = jnp.float32
BF16 = jnp.bfloat16
U32 = jnp.uint32
pk = lambda v: pltpu.bitcast(v.astype(BF16), U32)
upk = lambda v: pltpu.bitcast(v, BF16)


def pack16(v):
    t = v.shape[0] // 16
    lo = jnp.concatenate([v[16 * g:16 * g + 8] for g in range(t)], axis=0)
    hi = jnp.concatenate([v[16 * g + 8:16 * g + 16] for g in range(t)], axis=0)
    return pltpu.pack_elementwise([lo, hi], packed_dtype=BF16)


def unpack16(w):
    lo = pltpu.unpack_elementwise(w, index=0, packed_dtype=BF16, unpacked_dtype=F32)
    hi = pltpu.unpack_elementwise(w, index=1, packed_dtype=BF16, unpacked_dtype=F32)
    parts = []
    for g in range(w.shape[0] // 8):
        parts += [lo[8 * g:8 * g + 8], hi[8 * g:8 * g + 8]]
    return jnp.concatenate(parts, axis=0)
K0 = float(np.sqrt(2.0 / np.pi))
ALPHA = float((K0 * 0.044715) ** (1.0 / 3.0))
C0 = K0 / ALPHA
HS = 0.5 / ALPHA

S433 = dict(m=4, k=3, n=3,
    a_prog=[(3, -1, 1, 1), (10, -1, 3, 1), (2, 1, 6, 1), (5, 1, 7, 1), (3, 1, 9, 1), (0, 1, 16, 1), (17, 1, 2, -1), (9, -1, 18, 1), (4, 1, 1, 1), (20, 1, 10, 1), (20, 1, 5, 1), (21, 1, 7, -1), (10, 1, 22, 1), (5, 1, 8, -1), (25, 1, 11, 1), (6, 1, 25, 1), (6, 1, 26, 1), (13, 1, 28, 1), (16, -1, 29, 1), (22, 1, 12, -1), (31, 1, 15, -1), (18, 1, 24, -1), (11, -1, 33, 1), (12, 1, 14, 1), (19, 1, 35, 1), (14, 1, 15, 1), (37, 1, 27, -1)],
    a_use=[13, 1, 16, 17, 18, 34, 2, 10, 11, 24, 21, 3, 5, 22, 19, 12, 1, 32, 15, 7, 27, 6, 36, 14, 38, 28, 30, 23, 26],
    c_prog=[(7, 1, 4, 1), (7, 1, 9, -1), (11, -1, 5, 1), (2, 1, 5, -1), (3, 1, 6, 1), (10, -1, 4, 1), (1, 1, 4, -1), (0, 1, 8, -1), (11, 1, 1, 1), (9, -1, 17, 1), (16, 1, 8, -1), (0, 1, 15, -1), (12, 1, 11, 1), (14, -1, 23, 1), (24, 1, 17, -1), (18, 1, 21, 1), (8, 1, 9, -1), (28, -1, 6, 1), (7, -1, 0, 1), (6, -1, 30, 1), (8, -1, 2, 1), (1, 1, 32, 1), (12, -1, 22, 1), (34, 1, 5, -1), (3, -1, 23, 1), (21, -1, 36, 1)],
    c_use=[(21, -1), (18, 1), (27, -1), (1, -1), (20, -1), (11, 1), (33, 1), (17, -1), (26, 1), (24, -1), (12, -1), (37, 1), (35, -1), (14, 1), (25, -1), (23, 1), (15, -1), (3, -1), (22, -1), (16, 1), (29, -1), (31, 1), (0, -1), (19, -1), (8, 1), (13, 1), (9, 1), (7, 1), (7, -1)],
    w=[[1, -1, 0, -1, 0, 0, 0, 0, 0], [0, 0, 0, 0, 1, 0, 0, 0, 0], [0, 1, 0, 0, 0, 0, 0, 0, 0], [0, -1, 1, 0, 0, 0, 0, -1, 1], [0, 0, -1, 0, 0, 0, 0, 1, -1], [0, 0, 0, 0, 0, 0, 0, 1, -1], [0, 0, 1, 0, 0, 0, 0, 0, 1], [1, -1, 0, -1, 1, 0, 0, 0, 0], [0, 0, 0, 0, 0, 0, 0, 1, 0], [0, 0, 0, 0, 0, -1, 0, -1, 1], [0, 0, 0, 0, -1, 1, 0, 1, -1], [-1, 0, 0, 1, 0, 0, 0, 0, 0], [0, 0, 0, 0, 0, -1, 0, 0, 1], [0, 0, 0, 0, 0, 1, 0, 0, 0], [0, 0, 1, 0, 0, 0, 0, 0, 0], [-1, 0, -1, 1, 0, 0, 0, 0, 0], [1, 0, 1, -1, 0, -1, 0, 0, 0], [0, 0, 0, -1, 0, 0, 0, 0, 0], [0, 0, 0, 0, 0, 1, -1, 0, -1], [0, 0, 0, 1, 0, 1, -1, 0, -1], [0, 0, 0, 0, 0, 0, 1, 0, 0], [-1, 0, 0, 0, 0, 0, -1, 0, 0], [-1, 0, -1, 0, 0, 0, 0, 0, 0], [0, 0, 1, 0, 0, 0, -1, 0, 0], [0, 0, 0, 0, 0, 0, 1, 0, 1], [-1, 1, 0, 0, 0, 0, -1, 0, 0], [-1, 1, 0, 0, 0, 0, 0, 0, 0], [0, 0, 0, 0, -1, 0, 0, 0, 0], [-1, 1, 0, 0, 0, 0, -1, 1, 0]])
S343 = dict(m=3, k=4, n=3,
    a_prog=[(0, 1, 10, -1), (4, 1, 5, 1), (6, 1, 5, 1), (7, 1, 5, 1), (11, 1, 4, 1), (3, 1, 6, 1), (9, 1, 8, 1), (11, 1, 9, 1), (2, 1, 1, 1), (0, 1, 18, -1), (3, 1, 15, 1), (20, 1, 10, -1), (14, 1, 11, -1), (22, 1, 13, -1), (21, 1, 19, 1), (24, 1, 15, -1), (23, 1, 24, -1), (28, 1, 19, -1), (12, 1, 26, -1), (30, 1, 16, 1), (1, 1, 3, 1), (32, -1, 23, 1), (33, -1, 12, 1), (34, 1, 17, -1), (32, 1, 21, 1), (15, 1, 36, 1)],
    a_use=[6, 13, 15, 14, 24, 22, 27, 29, 3, 20, 23, 6, 17, 25, 4, 16, 11, 31, 10, 12, 35, 33, 19, 18, 21, 37, 0, 26, 1],
    c_prog=[(0, 1, 2, -1), (5, 1, 8, -1), (0, 1, 6, 1), (6, 1, 8, -1), (2, 1, 6, 1), (2, 1, 8, 1), (3, -1, 0, 1), (7, 1, 8, -1), (0, 1, 1, -1), (1, -1, 15, 1), (2, 1, 16, -1), (15, 1, 2, -1), (5, 1, 16, 1), (6, 1, 17, 1), (6, 1, 10, 1), (19, -1, 1, 1), (3, 1, 23, -1), (18, 1, 4, 1), (22, 1, 7, -1), (4, 1, 21, -1), (20, 1, 5, 1)],
    c_use=[(4, -1), (4, 1), (26, 1), (28, -1), (21, 1), (18, 1), (5, -1), (16, 1), (15, -1), (24, -1), (19, 1), (29, 1), (20, -1), (3, 1), (25, 1), (23, 1), (10, -1), (12, -1), (14, -1), (13, 1), (9, -1), (2, -1), (7, -1), (27, -1), (22, -1), (17, -1), (11, 1), (6, -1), (1, -1)],
    w=[[0, -1, 0, 0, 1, 0, 0, -1, 0, 0, -1, 0], [0, 1, 0, 0, 0, 0, 0, 0, 0, 0, 0, 0], [0, 0, 0, 0, 0, 0, 0, 0, 0, 0, 1, 0], [0, 1, 0, 0, -1, 0, 0, 0, 0, 0, 1, 0], [0, -1, 0, 0, 1, 1, 0, 0, 0, 0, -1, 0], [0, 0, 0, -1, 0, 0, 0, 0, 0, 0, -1, 0], [0, 0, 0, 0, 0, 0, 0, 0, 0, 0, 0, 1], [0, 0, 0, 0, 0, 1, 0, 0, 0, 0, 0, 0], [0, 0, 0, 0, 0, 1, -1, 0, -1, -1, -1, -1], [0, 0, 0, 0, 0, 0, 0, -1, 0, 0, 0, 0], [0, 0, 0, 0, 0, 1, 0, 1, 0, 0, 0, 0], [0, 0, 0, 0, 0, -1, 0, 0, 1, 0, 0, 1], [0, 0, 0, 0, 0, -1, 1, 0, 1, 0, 0, 1], [0, 0, 0, -1, 0, 0, 0, 0, 0, 1, 0, 0], [1, 0, 0, -1, 0, 0, 0, 0, 0, 1, 0, 0], [1, 0, 1, -1, 0, 0, 0, 0, 0, 1, 0, 0], [1, 1, 1, -1, -1, -1, 0, 0, 0, 1, 1, 1], [0, 0, 1, 0, 0, 0, 0, 0, 0, 0, 0, 0], [0, 0, -1, 0, 0, 0, 0, -1, -1, 0, 0, 0], [0, 0, 1, 0, 0, 0, -1, 0, 0, 0, 0, 0], [0, 0, 0, 0, 0, 0, 1, 0, 0, 0, 0, 0], [0, 0, 0, 0, 0, 1, -1, 0, -1, 0, 0, 0], [0, 1, 0, 0, -1, -1, 0, 0, 0, 0, 0, 0], [0, 1, 0, 0, 0, 0, 0, 0, 0, 0, 0, 0], [0, 1, 0, 1, 0, 0, 0, 0, 0, 0, 0, 0], [0, 0, 0, -1, 0, 0, 0, 0, 0, 0, 0, 0], [1, 1, 0, 0, 0, 0, 1, 0, 0, 0, 0, 0], [1, 0, 1, -1, 0, 0, 0, 0, 0, 0, 0, 0], [0, 0, 0, -1, -1, 0, 0, 1, 0, 0, 0, 0]])
HK = dict(m=2, k=3, n=3,
    a_prog=[(5, 1, 4, 1), (5, -1, 3, 1), (0, 1, 2, -1), (0, 1, 3, -1), (2, 1, 3, -1), (5, -1, 2, 1), (0, 1, 1, -1), (12, 1, 3, -1), (6, -1, 2, 1), (1, 1, 14, 1), (13, 1, 4, 1)],
    a_use=[4, 14, 6, 1, 2, 12, 15, 8, 13, 16, 7, 3, 10, 11, 9],
    c_prog=[(5, -1, 0, 1), (5, 1, 3, 1), (3, 1, 0, 1), (1, 1, 2, -1), (4, -1, 3, 1), (0, 1, 2, 1), (5, 1, 2, 1), (12, -1, 1, 1), (0, 1, 10, 1), (1, -1, 14, 1), (4, 1, 13, 1)],
    c_use=[(4, 1), (13, -1), (16, 1), (1, 1), (12, 1), (15, 1), (9, -1), (11, -1), (14, -1), (10, 1), (7, 1), (8, -1), (6, -1), (5, -1), (0, 1)],
    w=[[0, 0, 0, 1, 1, 0, 0, -1, 0], [0, 0, 0, 0, 0, -1, 0, -1, 0], [0, 0, 0, 0, 0, 0, 0, 1, 0], [0, 1, 0, 0, 1, 1, 0, 0, 0], [0, 0, 1, 0, 0, 0, 0, 1, 1], [0, -1, 0, 0, 0, 0, 0, 0, 0], [0, 0, 0, 0, 0, 1, 0, 0, 0], [0, 0, -1, 0, 0, 0, 0, 0, 0], [0, -1, 0, 1, 0, 0, 0, 0, 0], [0, 0, 0, 1, 0, 0, 0, 0, 0], [0, 0, 0, 0, 0, 0, -1, 0, 0], [-1, -1, 0, 0, 0, 0, -1, 0, 0], [0, 0, -1, 0, 0, 0, -1, 0, 0], [0, 0, 0, 0, 0, -1, -1, 0, 1], [1, 0, -1, 1, 0, 0, 0, 0, 0]])
Sa = dict(m=4, k=3, n=3,
    a_prog=[(1, 1, 3, -1), (2, 1, 6, -1), (9, -1, 3, 1), (7, -1, 5, 1), (3, 1, 10, 1), (0, 1, 14, 1), (17, 1, 2, -1), (9, 1, 18, 1), (4, 1, 1, 1), (20, 1, 5, 1), (10, -1, 20, 1), (21, 1, 10, -1), (7, 1, 22, 1), (5, 1, 8, 1), (6, -1, 25, 1), (11, -1, 25, 1), (6, -1, 27, 1), (3, 1, 7, 1), (29, 1, 4, 1), (0, 1, 1, 1), (6, -1, 31, 1), (2, 1, 7, -1), (8, -1, 33, 1), (16, 1, 28, 1), (35, 1, 14, -1), (11, -1, 23, 1), (18, 1, 37, -1)],
    a_use=[14, 16, 1, 23, 11, 10, 3, 36, 17, 5, 22, 18, 38, 2, 28, 26, 21, 19, 12, 1, 30, 27, 15, 7, 32, 6, 24, 13, 34],
    c_prog=[(8, 1, 0, 1), (9, 1, 7, 1), (4, 1, 7, -1), (4, 1, 10, 1), (2, 1, 5, -1), (11, 1, 5, 1), (6, -1, 3, 1), (4, -1, 1, 1), (11, -1, 1, 1), (14, 1, 11, -1), (18, 1, 8, 1), (16, -1, 0, 1), (15, 1, 9, -1), (24, 1, 19, 1), (23, 1, 17, -1), (15, 1, 21, -1), (3, -1, 23, 1), (24, 1, 28, 1), (9, 1, 3, 1), (30, 1, 22, -1), (0, 1, 7, -1), (32, 1, 6, 1), (8, 1, 2, 1), (1, 1, 34, 1), (21, 1, 17, 1), (22, 1, 36, -1)],
    c_use=[(25, 1), (24, -1), (19, -1), (21, -1), (27, 1), (15, -1), (29, 1), (9, -1), (1, -1), (37, -1), (14, -1), (20, -1), (11, -1), (35, 1), (13, 1), (31, -1), (17, 1), (26, -1), (23, 1), (16, 1), (3, -1), (7, -1), (22, -1), (18, -1), (0, 1), (33, 1), (7, -1), (12, -1), (8, -1)],
    w=[[0, -1, 0, 0, 0, 0, 0, 0, 0], [-1, -1, 0, 1, 0, 0, 0, 0, 0], [0, 0, 0, 0, -1, 0, 0, 0, 0], [0, 0, 0, 0, 0, -1, 0, -1, 1], [0, 0, 0, 0, 0, 0, 0, 1, 0], [1, 1, 0, -1, -1, 0, 0, 0, 0], [-1, 0, 0, 1, 0, 0, 0, 0, 0], [-1, -1, 0, 0, 0, 0, 0, 0, 0], [0, -1, 1, 0, 0, 0, 0, -1, 1], [0, 0, 0, 0, 0, -1, 0, 0, 1], [0, 0, 0, 0, -1, 1, 0, 1, -1], [0, 0, -1, 0, 0, 0, 0, 1, -1], [0, 0, 0, 0, 0, 0, 0, 1, -1], [0, 0, 1, 0, 0, 0, 0, 0, 1], [-1, -1, 0, 0, 0, 0, -1, 0, 0], [0, 0, 0, 0, 0, 0, -1, 0, 0], [0, 0, 0, 0, 0, 1, 0, 0, 0], [0, 0, 1, 0, 0, 0, 0, 0, 0], [-1, 0, -1, 1, 0, 0, 0, 0, 0], [-1, 0, -1, 1, 0, 1, 0, 0, 0], [0, 0, 0, -1, 0, 0, 0, 0, 0], [-1, -1, 0, 0, 0, 0, -1, -1, 0], [0, 0, 0, 0, 0, 1, -1, 0, -1], [0, 0, 0, 1, 0, 1, -1, 0, -1], [1, 0, 1, 0, 0, 0, 0, 0, 0], [1, 0, 0, 0, 0, 0, 1, 0, 0], [0, 0, 0, 0, -1, 0, 0, 0, 0], [0, 0, 1, 0, 0, 0, -1, 0, 0], [0, 0, 0, 0, 0, 0, 1, 0, 1]])
Sb = dict(m=4, k=3, n=3,
    a_prog=[(3, -1, 1, 1), (2, 1, 6, -1), (9, -1, 3, 1), (5, 1, 7, -1), (10, 1, 3, 1), (0, 1, 14, 1), (17, 1, 2, -1), (18, 1, 9, 1), (5, 1, 8, 1), (6, -1, 20, 1), (11, -1, 20, 1), (6, -1, 22, 1), (4, 1, 1, 1), (5, 1, 24, 1), (24, 1, 10, -1), (5, 1, 26, 1), (7, 1, 26, 1), (27, 1, 11, -1), (29, -1, 18, 1), (1, 1, 6, -1), (0, 1, 31, 1), (9, 1, 23, 1), (33, 1, 10, 1), (12, 1, 10, -1), (35, -1, 28, 1), (2, 1, 15, 1), (37, 1, 20, -1)],
    a_use=[7, 3, 36, 15, 5, 6, 21, 38, 13, 32, 2, 19, 12, 16, 1, 23, 25, 34, 14, 11, 10, 1, 27, 26, 22, 28, 18, 17, 30],
    c_prog=[(8, 1, 0, 1), (9, 1, 7, 1), (4, 1, 7, -1), (4, 1, 10, 1), (2, 1, 5, -1), (11, 1, 5, 1), (6, -1, 3, 1), (1, 1, 4, -1), (1, 1, 11, -1), (14, 1, 11, -1), (18, 1, 8, 1), (16, -1, 0, 1), (9, -1, 15, 1), (19, 1, 24, 1), (17, -1, 23, 1), (15, 1, 21, -1), (9, -1, 8, 1), (6, 1, 28, -1), (17, -1, 22, 1), (21, -1, 30, 1), (24, 1, 23, 1), (32, 1, 3, -1), (8, 1, 1, 1), (2, 1, 34, 1), (13, -1, 12, 1), (36, 1, 29, 1)],
    c_use=[(18, -1), (33, -1), (3, -1), (22, 1), (31, 1), (37, -1), (29, 1), (8, -1), (12, 1), (0, -1), (35, 1), (26, -1), (23, 1), (24, 1), (16, 1), (13, -1), (17, 1), (9, 1), (25, 1), (27, -1), (15, -1), (19, -1), (21, 1), (14, 1), (7, 1), (7, -1), (20, 1), (1, 1), (11, 1)],
    w=[[0, 0, 0, 1, 0, 1, -1, 0, -1], [1, 0, 0, -1, 0, 0, 0, 0, 0], [0, 0, 0, -1, 0, 0, 0, 0, 0], [0, 0, 0, 0, 0, -1, 1, 0, 1], [0, 0, 0, 0, 0, 1, 0, 0, -1], [-1, 0, 0, 0, 0, 0, -1, 0, 0], [0, 0, 0, 0, 0, 0, 1, 0, 0], [0, 0, 0, 0, 0, 0, 1, 0, 1], [0, 0, -1, 0, 0, 0, 1, 0, 0], [-1, 0, -1, 0, 0, 0, 0, 0, 0], [0, 0, 1, 0, 0, 0, 0, 0, 1], [0, 0, 1, 0, 0, 0, 0, 0, 0], [-1, 0, -1, 1, 0, 0, 0, 0, 0], [1, 1, 0, -1, 0, 0, 0, 0, 0], [-1, 0, -1, 1, 0, 1, 0, 0, 0], [1, 1, 0, 0, 0, 0, 1, 0, 0], [0, 0, 0, 0, 0, 1, 0, 0, 0], [1, 1, 0, 0, 0, 0, 0, 0, 0], [0, -1, 0, 0, 0, 0, 0, 0, 0], [0, 0, 0, 0, 0, 0, 0, -1, 0], [1, 1, 0, -1, -1, 0, 0, 0, 0], [0, 0, 0, 0, -1, 0, 0, 0, 0], [0, 0, 0, 0, 0, 1, 0, 1, -1], [0, 0, 0, 0, 1, -1, 0, -1, 1], [1, 1, 0, 0, 0, 0, 1, 1, 0], [0, 0, 0, 0, -1, 0, 0, 0, 0], [0, 0, 1, 0, 0, 0, 0, -1, 1], [0, 1, -1, 0, 0, 0, 0, 1, -1], [0, 0, 0, 0, 0, 0, 0, -1, 1]])
Sc = dict(m=4, k=3, n=3,
    a_prog=[(1, 1, 3, -1), (10, -1, 3, 1), (2, 1, 6, 1), (5, 1, 7, 1), (9, 1, 3, 1), (16, 1, 0, 1), (2, -1, 17, 1), (9, -1, 18, 1), (4, 1, 1, 1), (20, 1, 10, 1), (20, 1, 5, 1), (7, -1, 21, 1), (22, 1, 10, 1), (8, -1, 5, 1), (11, 1, 25, 1), (6, 1, 25, 1), (11, 1, 27, 1), (28, 1, 10, -1), (29, 1, 9, -1), (2, 1, 7, 1), (8, 1, 31, 1), (23, 1, 12, -1), (10, -1, 33, 1), (6, 1, 0, 1), (1, 1, 35, 1), (24, -1, 18, 1), (37, 1, 11, -1)],
    a_use=[15, 30, 27, 34, 5, 7, 6, 32, 3, 2, 14, 12, 19, 36, 28, 1, 13, 16, 10, 11, 18, 22, 38, 1, 17, 23, 24, 26, 21],
    c_prog=[(4, 1, 7, 1), (7, 1, 9, -1), (11, -1, 5, 1), (5, -1, 2, 1), (6, 1, 3, 1), (4, 1, 10, -1), (4, -1, 1, 1), (8, -1, 0, 1), (11, 1, 1, 1), (9, -1, 17, 1), (8, -1, 16, 1), (15, -1, 0, 1), (11, 1, 12, 1), (23, 1, 14, -1), (17, -1, 24, 1), (18, 1, 21, 1), (9, 1, 22, 1), (3, -1, 28, 1), (6, 1, 7, 1), (30, -1, 0, 1), (22, 1, 24, -1), (14, -1, 32, 1), (23, 1, 3, -1), (21, -1, 34, 1), (20, 1, 19, 1), (36, 1, 25, -1)],
    c_use=[(22, 1), (9, -1), (29, -1), (3, 1), (33, -1), (16, -1), (31, -1), (8, 1), (35, 1), (37, 1), (19, -1), (23, -1), (25, -1), (0, 1), (13, 1), (15, 1), (21, -1), (27, -1), (17, -1), (26, 1), (20, -1), (14, 1), (11, 1), (18, 1), (1, -1), (7, -1), (24, -1), (7, 1), (12, -1)],
    w=[[0, 0, 0, 0, 0, -1, 1, 0, 1], [1, -1, 0, 0, 0, 0, 0, 0, 0], [0, 0, 0, 0, 0, 0, 1, 0, 0], [0, 0, 0, 1, 0, 0, 0, 0, 0], [0, 0, 0, 0, 0, -1, 0, 0, 1], [0, 0, 0, -1, 0, -1, 1, 0, 1], [1, 0, 0, 0, 0, 0, 1, 0, 0], [0, 0, 0, 0, 0, 0, 1, 0, 1], [-1, 0, 0, 1, 0, 0, 0, 0, 0], [0, 0, 1, 0, 0, 0, 0, 0, 1], [0, 0, 1, 0, 0, 0, -1, 0, 0], [1, 0, 1, -1, 0, 0, 0, 0, 0], [0, 0, 1, 0, 0, 0, 0, 0, 0], [1, 0, 1, 0, 0, 0, 0, 0, 0], [-1, 1, 0, 0, 0, 0, -1, 0, 0], [-1, 0, -1, 1, 0, 1, 0, 0, 0], [1, -1, 0, -1, 0, 0, 0, 0, 0], [0, 1, 0, 0, 0, 0, 0, 0, 0], [1, -1, 0, -1, 1, 0, 0, 0, 0], [0, 0, 0, 0, 0, 0, 0, 1, 0], [0, 0, -1, 0, 0, 0, 0, 1, -1], [0, 0, 0, 0, 0, 1, 0, 0, 0], [0, 0, 0, 0, 0, 0, 0, 1, -1], [0, 0, 0, 0, 1, 0, 0, 0, 0], [0, -1, 1, 0, 0, 0, 0, -1, 1], [0, 0, 0, 0, 1, 0, 0, 0, 0], [0, 0, 0, 0, 0, -1, 0, -1, 1], [1, -1, 0, 0, 0, 0, 1, -1, 0], [0, 0, 0, 0, -1, 1, 0, 1, -1]])
Sd = dict(m=4, k=3, n=3,
    a_prog=[(10, -1, 3, 1), (6, -1, 3, 1), (3, 1, 7, -1), (5, -1, 1, 1), (11, -1, 0, 1), (9, -1, 13, 1), (11, -1, 17, 1), (6, 1, 18, 1), (10, -1, 4, 1), (5, 1, 20, 1), (7, -1, 20, 1), (21, 1, 7, -1), (22, 1, 1, 1), (2, 1, 5, 1), (8, -1, 25, 1), (0, 1, 25, 1), (8, -1, 27, 1), (1, 1, 12, -1), (29, 1, 20, 1), (2, 1, 11, 1), (1, 1, 31, 1), (8, -1, 23, 1), (33, 1, 18, 1), (28, 1, 13, 1), (14, -1, 35, 1), (12, 1, 19, -1), (16, 1, 37, 1)],
    a_use=[1, 5, 32, 15, 27, 0, 30, 3, 11, 16, 12, 19, 38, 23, 10, 14, 21, 13, 8, 7, 10, 22, 24, 18, 34, 36, 17, 26, 28],
    c_prog=[(4, 1, 7, 1), (0, 1, 3, -1), (4, 1, 10, 1), (2, 1, 9, 1), (10, 1, 8, 1), (5, 1, 8, 1), (5, 1, 11, 1), (4, -1, 1, 1), (6, -1, 1, 1), (18, 1, 9, 1), (2, 1, 13, 1), (6, 1, 12, 1), (8, 1, 19, 1), (23, 1, 14, -1), (24, 1, 12, 1), (17, 1, 21, -1), (2, 1, 10, -1), (28, 1, 11, -1), (22, 1, 24, 1), (30, 1, 17, -1), (23, 1, 21, 1), (32, 1, 3, 1), (2, 1, 0, 1), (34, 1, 6, 1), (0, 1, 1, 1), (36, 1, 9, -1)],
    c_use=[(13, -1), (31, -1), (2, -1), (22, -1), (35, 1), (37, 1), (3, 1), (33, 1), (29, 1), (15, 1), (21, 1), (27, 1), (9, -1), (24, -1), (18, 1), (23, -1), (17, -1), (25, 1), (26, -1), (12, -1), (14, 1), (19, -1), (1, -1), (16, 1), (8, 1), (6, -1), (10, 1), (1, 1), (20, -1)],
    w=[[0, 0, 0, -1, 0, 1, 1, 0, -1], [0, 0, 0, 0, 0, -1, 0, 0, 1], [0, 0, 0, 0, 0, 0, 1, 0, -1], [0, 0, 0, 0, 0, -1, -1, 0, 1], [0, 0, 0, 0, 0, 0, 1, 0, 0], [1, 0, 0, 0, 0, 0, -1, 0, 0], [0, 0, 0, 1, 0, 0, 0, 0, 0], [1, 0, 0, 1, 0, 0, 0, 0, 0], [0, 0, 1, 0, 0, 0, 0, 0, -1], [0, 0, 1, 0, 0, 0, -1, 0, 0], [-1, 0, 1, -1, 0, 0, 0, 0, 0], [0, 0, 1, 0, 0, 0, 0, 0, 0], [-1, 0, 1, 0, 0, 0, 0, 0, 0], [0, 0, 0, 0, 0, 1, 0, 1, -1], [-1, 0, 1, -1, 0, 1, 0, 0, 0], [1, -1, 0, 1, 0, 0, 0, 0, 0], [0, 0, 0, 0, 0, -1, 0, 0, 0], [0, -1, 0, 0, 0, 0, 0, 0, 0], [0, 0, 0, 0, 0, 0, 0, -1, 0], [1, -1, 0, 1, -1, 0, 0, 0, 0], [0, 0, 0, 0, 1, 0, 0, 0, 0], [0, 0, 0, 0, 1, -1, 0, -1, 1], [0, 0, 0, 0, -1, 0, 0, 0, 0], [0, 0, -1, 0, 0, 0, 0, -1, 1], [0, 0, 0, 0, 0, 0, 0, 1, -1], [1, -1, 0, 0, 0, 0, 0, 0, 0], [0, -1, 1, 0, 0, 0, 0, 1, -1], [1, -1, 0, 0, 0, 0, -1, 1, 0], [1, -1, 0, 0, 0, 0, -1, 0, 0]])
H2 = dict(m=2, k=3, n=3,
    a_prog=[(5, 1, 4, 1), (5, -1, 3, 1), (2, -1, 0, 1), (3, -1, 0, 1), (3, -1, 2, 1), (5, -1, 2, 1), (1, -1, 0, 1), (9, 1, 1, -1), (11, 1, 4, -1), (14, 1, 1, 1), (4, 1, 13, 1)],
    a_use=[3, 13, 16, 12, 7, 4, 6, 14, 15, 1, 2, 8, 9, 10, 11],
    c_prog=[(0, 1, 5, -1), (5, 1, 3, 1), (0, 1, 3, 1), (1, 1, 2, -1), (4, -1, 3, 1), (0, 1, 2, 1), (5, 1, 2, 1), (5, -1, 9, 1), (8, 1, 4, -1), (14, 1, 1, -1), (4, 1, 13, 1)],
    c_use=[(8, 1), (14, -1), (10, -1), (15, 1), (7, 1), (4, -1), (16, -1), (13, 1), (9, 1), (1, 1), (12, 1), (11, 1), (0, -1), (6, 1), (5, 1)],
    w=[[1, 1, 0, 0, 0, 0, 1, 0, 0], [0, -1, 0, 1, 0, 0, 0, 0, 0], [0, 0, 0, -1, 0, 0, 0, 0, 0], [0, -1, 0, 0, 0, 0, 0, 0, 0], [0, 0, 0, 0, 0, 0, -1, 0, 0], [0, 0, 0, -1, -1, 0, 0, 1, 0], [0, 0, 0, 0, 0, 0, 0, -1, 0], [0, 0, 0, 0, 0, 1, 0, 1, 0], [0, 0, 0, 0, 0, -1, 0, 0, 0], [0, 1, 0, 0, 1, 1, 0, 0, 0], [0, 0, 1, 0, 0, 0, 0, 1, 1], [0, 0, 1, 0, 0, 0, 0, 0, 0], [-1, 0, 1, -1, 0, 0, 0, 0, 0], [0, 0, 1, 0, 0, 0, 1, 0, 0], [0, 0, 0, 0, 0, 1, 1, 0, -1]])
H3 = dict(m=2, k=3, n=3,
    a_prog=[(5, 1, 4, 1), (5, -1, 3, 1), (0, 1, 2, -1), (0, 1, 3, -1), (2, 1, 3, -1), (5, -1, 2, 1), (0, 1, 1, -1), (9, 1, 1, -1), (4, -1, 11, 1), (1, 1, 14, 1), (4, 1, 13, 1)],
    a_use=[1, 12, 13, 16, 4, 6, 3, 7, 14, 15, 2, 8, 9, 10, 11],
    c_prog=[(5, -1, 0, 1), (3, 1, 5, 1), (3, 1, 0, 1), (2, -1, 1, 1), (3, 1, 4, -1), (2, 1, 0, 1), (2, 1, 5, 1), (5, -1, 9, 1), (10, 1, 0, 1), (1, -1, 14, 1), (13, 1, 4, 1)],
    c_use=[(1, -1), (15, 1), (14, -1), (10, 1), (4, -1), (16, 1), (8, -1), (7, 1), (13, -1), (9, -1), (12, 1), (11, 1), (0, 1), (6, -1), (5, 1)],
    w=[[0, -1, 0, 0, -1, -1, 0, 0, 0], [0, -1, 0, 0, 0, 0, 0, 0, 0], [0, -1, 0, 1, 0, 0, 0, 0, 0], [0, 0, 0, 1, 0, 0, 0, 0, 0], [0, 0, 0, -1, -1, 0, 0, 1, 0], [0, 0, 0, 0, 0, 0, 0, 1, 0], [-1, -1, 0, 0, 0, 0, -1, 0, 0], [0, 0, 0, 0, 0, 0, -1, 0, 0], [0, 0, 0, 0, 0, -1, 0, -1, 0], [0, 0, 0, 0, 0, 1, 0, 0, 0], [0, 0, 1, 0, 0, 0, 0, 1, 1], [0, 0, 1, 0, 0, 0, 0, 0, 0], [1, 0, -1, 1, 0, 0, 0, 0, 0], [0, 0, -1, 0, 0, 0, -1, 0, 0], [0, 0, 0, 0, 0, 1, 1, 0, -1]])

Se = {'m': 4, 'k': 3, 'n': 3, 'a_prog': [(10, -1, 3, 1), (6, -1, 3, 1), (3, 1, 7, -1), (5, -1, 1, 1), (11, -1, 0, 1), (9, -1, 13, 1), (11, -1, 17, 1), (6, 1, 18, 1), (10, -1, 4, 1), (5, 1, 20, 1), (7, -1, 20, 1), (21, 1, 7, -1), (22, 1, 1, 1), (2, 1, 5, 1), (8, -1, 25, 1), (0, 1, 25, 1), (8, -1, 27, 1), (1, 1, 12, -1), (29, 1, 20, 1), (2, 1, 11, 1), (1, 1, 31, 1), (8, -1, 23, 1), (33, 1, 18, 1), (28, 1, 13, 1), (14, -1, 35, 1), (12, 1, 19, -1), (16, 1, 37, 1)], 'a_use': [5, 27, 32, 15, 0, 1, 30, 3, 16, 11, 12, 19, 38, 10, 14, 21, 13, 23, 8, 7, 10, 22, 18, 34, 24, 17, 26, 28, 36], 'c_prog': [(4, 1, 7, 1), (0, 1, 3, -1), (4, 1, 10, 1), (2, 1, 9, 1), (10, 1, 8, 1), (5, 1, 8, 1), (5, 1, 11, 1), (4, -1, 1, 1), (6, -1, 1, 1), (18, 1, 9, 1), (2, 1, 13, 1), (6, 1, 12, 1), (8, 1, 19, 1), (23, 1, 14, -1), (24, 1, 12, 1), (17, 1, 21, -1), (2, 1, 10, -1), (28, 1, 11, -1), (22, 1, 24, 1), (30, 1, 17, -1), (23, 1, 21, 1), (32, 1, 3, 1), (2, 1, 0, 1), (34, 1, 6, 1), (0, 1, 1, 1), (36, 1, 9, -1)], 'c_use': [(31, 1), (35, 1), (2, 1), (22, -1), (37, 1), (13, -1), (3, -1), (33, 1), (15, -1), (29, 1), (21, 1), (27, 1), (9, 1), (18, 1), (23, -1), (17, 1), (25, 1), (24, -1), (26, -1), (12, 1), (14, -1), (19, -1), (16, 1), (8, -1), (1, 1), (10, -1), (1, -1), (20, 1), (6, -1)], 'w': [[0, 0, 0, 0, 0, 1, 0, 0, -1], [0, 0, 0, 0, 0, 0, 1, 0, 0], [0, 0, 0, 0, 0, 0, -1, 0, 1], [0, 0, 0, 0, 0, -1, -1, 0, 1], [1, 0, 0, 0, 0, 0, -1, 0, 0], [0, 0, 0, -1, 0, 1, 1, 0, -1], [0, 0, 0, -1, 0, 0, 0, 0, 0], [1, 0, 0, 1, 0, 0, 0, 0, 0], [0, 0, -1, 0, 0, 0, 1, 0, 0], [0, 0, 1, 0, 0, 0, 0, 0, -1], [-1, 0, 1, -1, 0, 0, 0, 0, 0], [0, 0, 1, 0, 0, 0, 0, 0, 0], [1, 0, -1, 0, 0, 0, 0, 0, 0], [-1, 0, 1, -1, 0, 1, 0, 0, 0], [1, -1, 0, 1, 0, 0, 0, 0, 0], [0, 0, 0, 0, 0, 1, 0, 0, 0], [0, -1, 0, 0, 0, 0, 0, 0, 0], [0, 0, 0, 0, 0, 1, 0, 1, -1], [0, 0, 0, 0, 0, 0, 0, -1, 0], [-1, 1, 0, -1, 1, 0, 0, 0, 0], [0, 0, 0, 0, -1, 0, 0, 0, 0], [0, 0, 0, 0, 1, -1, 0, -1, 1], [0, 0, -1, 0, 0, 0, 0, -1, 1], [0, 0, 0, 0, 0, 0, 0, -1, 1], [0, 0, 0, 0, 1, 0, 0, 0, 0], [0, 1, -1, 0, 0, 0, 0, -1, 1], [-1, 1, 0, 0, 0, 0, 1, -1, 0], [-1, 1, 0, 0, 0, 0, 1, 0, 0], [1, -1, 0, 0, 0, 0, 0, 0, 0]]}

Sf = {'m': 4, 'k': 3, 'n': 3, 'a_prog': [(10, -1, 3, 1), (6, -1, 3, 1), (3, 1, 7, -1), (5, -1, 1, 1), (11, -1, 0, 1), (9, -1, 13, 1), (11, -1, 17, 1), (6, 1, 18, 1), (10, -1, 4, 1), (5, 1, 20, 1), (7, -1, 20, 1), (21, 1, 7, -1), (22, 1, 1, 1), (2, 1, 5, 1), (8, -1, 25, 1), (0, 1, 25, 1), (8, -1, 27, 1), (1, 1, 12, -1), (29, 1, 20, 1), (2, 1, 11, 1), (1, 1, 31, 1), (8, -1, 23, 1), (33, 1, 18, 1), (28, 1, 13, 1), (14, -1, 35, 1), (12, 1, 19, -1), (16, 1, 37, 1)], 'a_use': [5, 0, 27, 32, 1, 3, 30, 11, 15, 16, 10, 14, 12, 19, 38, 21, 13, 8, 7, 10, 23, 18, 22, 34, 24, 26, 28, 17, 36], 'c_prog': [(4, 1, 7, 1), (0, 1, 3, -1), (4, 1, 10, 1), (2, 1, 9, 1), (10, 1, 8, 1), (5, 1, 8, 1), (5, 1, 11, 1), (4, -1, 1, 1), (6, -1, 1, 1), (18, 1, 9, 1), (2, 1, 13, 1), (6, 1, 12, 1), (8, 1, 19, 1), (23, 1, 14, -1), (24, 1, 12, 1), (17, 1, 21, -1), (2, 1, 10, -1), (28, 1, 11, -1), (22, 1, 24, 1), (30, 1, 17, -1), (23, 1, 21, 1), (32, 1, 3, 1), (2, 1, 0, 1), (34, 1, 6, 1), (0, 1, 1, 1), (36, 1, 9, -1)], 'c_use': [(31, -1), (37, -1), (35, 1), (2, -1), (13, -1), (33, -1), (3, -1), (29, -1), (22, -1), (15, 1), (18, 1), (23, -1), (21, 1), (27, 1), (9, -1), (17, 1), (25, -1), (26, 1), (12, 1), (14, -1), (24, -1), (16, 1), (19, -1), (8, -1), (1, -1), (1, 1), (20, -1), (10, -1), (6, -1)], 'w': [[0, 0, 0, 0, 0, -1, 0, 0, 1], [-1, 0, 0, 0, 0, 0, 1, 0, 0], [0, 0, 0, 0, 0, 0, 1, 0, 0], [0, 0, 0, 0, 0, 0, 1, 0, -1], [0, 0, 0, -1, 0, 1, 1, 0, -1], [-1, 0, 0, -1, 0, 0, 0, 0, 0], [0, 0, 0, -1, 0, 0, 0, 0, 0], [0, 0, -1, 0, 0, 0, 0, 0, 1], [0, 0, 0, 0, 0, -1, -1, 0, 1], [0, 0, 1, 0, 0, 0, -1, 0, 0], [-1, 0, 1, -1, 0, 1, 0, 0, 0], [1, -1, 0, 1, 0, 0, 0, 0, 0], [-1, 0, 1, -1, 0, 0, 0, 0, 0], [0, 0, 1, 0, 0, 0, 0, 0, 0], [-1, 0, 1, 0, 0, 0, 0, 0, 0], [0, 0, 0, 0, 0, 1, 0, 0, 0], [0, 1, 0, 0, 0, 0, 0, 0, 0], [0, 0, 0, 0, 0, 0, 0, 1, 0], [-1, 1, 0, -1, 1, 0, 0, 0, 0], [0, 0, 0, 0, -1, 0, 0, 0, 0], [0, 0, 0, 0, 0, 1, 0, 1, -1], [0, 0, -1, 0, 0, 0, 0, -1, 1], [0, 0, 0, 0, 1, -1, 0, -1, 1], [0, 0, 0, 0, 0, 0, 0, -1, 1], [0, 0, 0, 0, -1, 0, 0, 0, 0], [1, -1, 0, 0, 0, 0, -1, 1, 0], [1, -1, 0, 0, 0, 0, -1, 0, 0], [0, 1, -1, 0, 0, 0, 0, -1, 1], [1, -1, 0, 0, 0, 0, 0, 0, 0]]}

Sg = {'m': 4, 'k': 3, 'n': 3, 'a_prog': [(10, -1, 3, 1), (6, -1, 3, 1), (3, 1, 7, -1), (5, -1, 1, 1), (11, -1, 0, 1), (9, -1, 13, 1), (11, -1, 17, 1), (6, 1, 18, 1), (10, -1, 4, 1), (5, 1, 20, 1), (7, -1, 20, 1), (21, 1, 7, -1), (22, 1, 1, 1), (2, 1, 5, 1), (8, -1, 25, 1), (0, 1, 25, 1), (8, -1, 27, 1), (1, 1, 12, -1), (29, 1, 20, 1), (2, 1, 11, 1), (1, 1, 31, 1), (8, -1, 23, 1), (33, 1, 18, 1), (28, 1, 13, 1), (14, -1, 35, 1), (12, 1, 19, -1), (16, 1, 37, 1)], 'a_use': [5, 0, 27, 1, 32, 15, 30, 3, 11, 16, 10, 14, 12, 19, 21, 38, 13, 7, 8, 10, 23, 18, 22, 34, 24, 28, 26, 17, 36], 'c_prog': [(4, 1, 7, 1), (0, 1, 3, -1), (4, 1, 10, 1), (2, 1, 9, 1), (10, 1, 8, 1), (5, 1, 8, 1), (5, 1, 11, 1), (4, -1, 1, 1), (6, -1, 1, 1), (18, 1, 9, 1), (2, 1, 13, 1), (6, 1, 12, 1), (8, 1, 19, 1), (23, 1, 14, -1), (24, 1, 12, 1), (17, 1, 21, -1), (2, 1, 10, -1), (28, 1, 11, -1), (22, 1, 24, 1), (30, 1, 17, -1), (23, 1, 21, 1), (32, 1, 3, 1), (2, 1, 0, 1), (34, 1, 6, 1), (0, 1, 1, 1), (36, 1, 9, -1)], 'c_use': [(31, -1), (37, -1), (35, 1), (13, -1), (2, -1), (22, -1), (3, -1), (33, -1), (29, -1), (15, 1), (18, 1), (23, -1), (21, 1), (27, 1), (17, -1), (9, 1), (25, -1), (12, 1), (26, 1), (14, -1), (24, -1), (16, 1), (19, -1), (8, -1), (1, -1), (20, 1), (1, -1), (10, -1), (6, -1)], 'w': [[0, 0, 0, 0, 0, -1, 0, 0, 1], [-1, 0, 0, 0, 0, 0, 1, 0, 0], [0, 0, 0, 0, 0, 0, 1, 0, 0], [0, 0, 0, -1, 0, 1, 1, 0, -1], [0, 0, 0, 0, 0, 0, 1, 0, -1], [0, 0, 0, 0, 0, -1, -1, 0, 1], [0, 0, 0, -1, 0, 0, 0, 0, 0], [-1, 0, 0, -1, 0, 0, 0, 0, 0], [0, 0, -1, 0, 0, 0, 0, 0, 1], [0, 0, 1, 0, 0, 0, -1, 0, 0], [-1, 0, 1, -1, 0, 1, 0, 0, 0], [1, -1, 0, 1, 0, 0, 0, 0, 0], [-1, 0, 1, -1, 0, 0, 0, 0, 0], [0, 0, 1, 0, 0, 0, 0, 0, 0], [0, 0, 0, 0, 0, -1, 0, 0, 0], [1, 0, -1, 0, 0, 0, 0, 0, 0], [0, 1, 0, 0, 0, 0, 0, 0, 0], [-1, 1, 0, -1, 1, 0, 0, 0, 0], [0, 0, 0, 0, 0, 0, 0, 1, 0], [0, 0, 0, 0, -1, 0, 0, 0, 0], [0, 0, 0, 0, 0, 1, 0, 1, -1], [0, 0, -1, 0, 0, 0, 0, -1, 1], [0, 0, 0, 0, 1, -1, 0, -1, 1], [0, 0, 0, 0, 0, 0, 0, -1, 1], [0, 0, 0, 0, -1, 0, 0, 0, 0], [-1, 1, 0, 0, 0, 0, 1, 0, 0], [-1, 1, 0, 0, 0, 0, 1, -1, 0], [0, 1, -1, 0, 0, 0, 0, -1, 1], [1, -1, 0, 0, 0, 0, 0, 0, 0]]}


SCHEMES = dict(S433=S433, S343=S343, HK=HK, Se=Se, Sf=Sf, Sg=Sg)


def gelu(y):
    return y * jnp.tanh(y * (y * y + C0)) + y


def lhs_operands(sc, block):
    m, k = sc["m"], sc["k"]
    memo, packed = {}, {}

    def node(v):
        if v not in memo:
            if v < m * k:
                memo[v] = (1, block(v // k, v % k))
            else:
                a, sa, b, sb = sc["a_prog"][v - m * k]
                (ta, xa), (tb, xb) = node(a), node(b)
                ta, tb = ta * sa, tb * sb
                memo[v] = (ta, xa + xb) if ta == tb else (1, xa - xb if ta > 0 else xb - xa)
        return memo[v]

    def op(p):
        v = sc["a_use"][p]
        if v not in packed:
            packed[v] = node(v)[1].astype(BF16)
        return packed[v]
    return op


def combine(sc, product, emit):
    m, n = sc["m"], sc["n"]
    fan = [0] * (m * n + len(sc["c_prog"]))
    for v, _ in sc["c_use"]:
        fan[v] += 1
    for a, _, b, _ in sc["c_prog"]:
        fan[a] += 1
        fan[b] += 1
    val = {}

    def push(v, t, x):
        if v in val:
            u, y = val[v]
            t, x = (t, y + x) if t == u else (1, x - y if t > 0 else y - x)
        val[v] = (t, x)
        fan[v] -= 1
        if fan[v] == 0:
            del val[v]
            if v >= m * n:
                a, sa, b, sb = sc["c_prog"][v - m * n]
                push(a, t * sa, x)
                push(b, t * sb, x)
            else:
                assert t == 1
                emit(v // n, v % n, x)

    for p, (v, t) in enumerate(sc["c_use"]):
        push(v, t, product(p))


def weight_form(sc, p, tile):
    n, acc = sc["n"], None
    for q in sorted(range(len(sc["w"][p])), key=lambda q: -sc["w"][p][q]):
        c = sc["w"][p][q]
        if c:
            v = tile(q // n, q % n)
            acc = (v if c > 0 else -v) if acc is None else (acc + v if c > 0 else acc - v)
    return acc


def make(CH=768, G1=4, G2=2, S=52, XC=8, XR2=4, MC1=48, MC2=48, mode2="k", vmem_mb=128, flags=None, E1=2, E2=2,
         run1=True, run2=True, dma=True, comp=True, pipe=True, PT=0, OFF=0, MCR=48, NR=99, PADV=0, XW=C, RX=2, RB=2, OR=1, HL=False, RCH=384, nobc=False, TD=3, MID=True, LEAD=1, YB=0, YD=0, LNR=16, F0=0.0, F1=0.65, F2=0.68, F3=0.97, sc1='S433', sc2='HK', rs=1, PX=0, PH=0, PO=0, A1=1, B1=1, A2=1, B2=1):
    sc1, sc2 = (SCHEMES[z] if isinstance(z, str) else z for z in (sc1, sc2))
    NP1, NP2 = len(sc1["w"]), len(sc2["w"])
    PR = sc1["m"] * MC1
    KG2 = 12 // sc2["k"]
    TM1, TM2 = CH * G1, CH * G2
    XT = max(2 * TM1, XR2 * TM2)
    W1ROW = TM1

    @jax.jit
    def fn(x, dw, w1, w2, grn_g, grn_b):
        B, H, W, _ = x.shape
        N = B * H * W
        NT1, NT2 = N // TM1, N // TM2
        NCH = N // CH
        NHC = NCH - S
        R1 = -(-NHC * 65536 // (NT1 - E1))
        R2 = -(-NHC * 65536 * 2 // int(2 * NT2 - 2 * E2))
        PER, RF = PT * G2, OFF * G2
        NREC = min(NR, len(range(RF, NHC, PER))) if PT else 0
        assert R1 <= G1 * 65536 and R2 <= G2 * 65536 and S >= 2 * max(G1, G2) and TM1 >= HID and E1 >= 2 and E2 >= (1.5 if MID and G2 == 2 else 2) and TD < XR2
        W2ROW = (NT1 % 2) * TM1
        assert TM1 >= 2 * HID or not PT

        def kernel(x_hbm, dw_ref, w1_hbm, w2_hbm, g_ref, b_ref, out_hbm, h_hbm,
                   xbuf, hbuf, ws, ssq, vec, abuf, ybuf, xsem, osem, hsem, wsem):
            class _Nop:
                def start(self, priority=0): pass
                def wait(self): pass
            mk = pltpu.make_async_copy if dma else (lambda *a: _Nop())

            def xrows(slot, tm):
                return xbuf.at[pl.ds(pl.multiple_of(slot * tm, tm), tm), pl.ds(0, C)]

            def x_copy(i, slot, tm):
                return mk(x_hbm.at[pl.ds(i * tm, tm)], xrows(slot, tm), xsem.at[slot])

            def o_copy(i, slot):
                return mk(xrows(slot, TM2), out_hbm.at[pl.ds(i * TM2, TM2)], osem.at[slot])

            def stored(c):
                return jnp.logical_or((c + (PER - RF)) % PER != 0, c >= RF + NREC * PER) if PT else True

            def h_index(c):
                return c - jnp.minimum((c + (PER - 1 - RF)) // PER, NREC) if PT else c

            def h_out(c, slot):
                return mk(hbuf.at[slot], h_hbm.at[h_index(c)], hsem.at[slot])

            def h_in(c, slot):
                return mk(h_hbm.at[h_index(c)], hbuf.at[slot], hsem.at[slot])

            def w1_copy(q, row=W1ROW):
                return pltpu.make_async_copy(w1_hbm.at[:, pl.ds(q * C, C)], xbuf.at[pl.ds(row + q * C, C), pl.ds(0, C)], wsem.at[q])

            def w2_copy():
                return pltpu.make_async_copy(w2_hbm, xbuf.at[pl.ds(W2ROW, HID), pl.ds(0, C)], wsem.at[4])

            def restage():
                w2_copy().start()
                for q in range(4 if PT else 0):
                    w1_copy(q, W2ROW + HID).start()

            def wrap(v, n):
                return jnp.where(v >= n, v - n, v)

            def wrapn(v, n):
                return jnp.where(v < 0, v + n, v)

            def x0_copy():
                return pltpu.make_async_copy(x_hbm.at[pl.ds(0, PR)], xbuf.at[pl.ds(W1ROW + HID, PR), pl.ds(0, C)], osem.at[0])

            for q in range(4):
                w1_copy(q).start()
            x0_copy().start()
            ssq[...] = jnp.zeros_like(ssq)
            vec[0:8, :] = jnp.broadcast_to(dw_ref[...].astype(F32), (8, C))
            mk(x_hbm.at[pl.ds(PR, TM1)], xbuf.at[pl.ds(0, TM1), pl.ds(0, C)], xsem.at[0]).start()
            for q in range(4):
                w1_copy(q).wait()

            def w1_tile(k, n, row=W1ROW):
                r = row + (n // 3) * C + k * L
                return xbuf[r:r + L, (n % 3) * L:(n % 3 + 1) * L].astype(F32)

            for c in range(4):
                for p in range(NP1):
                    ws[p * 4 + c] = pk(weight_form(sc1, p, lambda k, j: w1_tile(k, 4 * j + c)))

            def layernorm(row, n=LNR):
                y = xbuf[pl.ds(pl.multiple_of(row, 16), n), :C].astype(F32) * jnp.concatenate([vec[0:8, :]] * (n // 8), axis=0)
                mu = jnp.sum(y, axis=-1, keepdims=True) * (1.0 / C)
                d = y - mu
                ss = jnp.sum(d * d, axis=-1, keepdims=True)
                v = ss * (1.0 / (C * ALPHA * ALPHA)) + 1e-5 / (ALPHA * ALPHA)
                if rs == 0:
                    return d * lax.rsqrt(v)
                return d * jnp.exp2(-0.5 * jnp.log2(v))

            def act(y, hs, r0, c):
                h = gelu(y)
                ssq[:, c * L:(c + 1) * L] += jnp.sum((h * h).reshape(MC1 // 8, 8, L), axis=0)
                if HL:
                    hbuf[hs, c, pl.ds(r0 // 2, MC1 // 2), :] = pack16(h)
                else:
                    hbuf[hs, pl.ds(r0 // 2, MC1 // 2), c * L:(c + 1) * L] = pack16(h)

            def operands(row):
                nl = MC1 // LNR
                a = {}
                def ln(t, q):
                    a[t, q] = layernorm(row + t * MC1 + q * LNR)
                op = lhs_operands(sc1, lambda t, k: jnp.concatenate([a[t, q][:, k * L:(k + 1) * L] for q in range(nl)], axis=0))
                lns = [functools.partial(ln, t, q) for t in range(sc1["m"]) for q in range(nl)]
                forms = [functools.partial(op, p) for p in range(NP1)]
                return op, lns, forms

            NB1 = TM1 // (PR)

            PPC = CH // PR

            def x1_copy(i, slot):
                row = pl.multiple_of(jnp.minimum(i * TM1 + PR, N - TM1), 16)
                return mk(x_hbm.at[pl.ds(row, TM1)], xrows(slot, TM1), xsem.at[slot])

            def stage(row):
                for t in range(sc1["m"]):
                    abuf[t * MC1:(t + 1) * MC1, :] = layernorm(row + t * MC1, MC1)

            def phase1(i, carry):
                xb, hb, q, qs, busy = carry
                slots = [wrap(hb + u, S) for u in range(G1)]
                qn = jnp.minimum((i * R1) >> 16, NHC)
                x1_copy(i, xb).wait()
                for u in range(G1):
                    @pl.when(busy[u] != 0)
                    def _():
                        h_out(0, slots[u]).wait()
                for u in range(G1):
                    @pl.when(jnp.logical_and(q + u < qn, stored(q + u)))
                    def _():
                        h_out(q + u, wrap(qs + u, S)).start()
                shift = jnp.where(i == NT1 - 1, PR, 0)

                nxt = None
                parked = []
                park_product = lambda f: f
                def flush():
                    b, t, j, hs, r0, col = parked.pop(0)
                    act(ybuf[b, t * 3 + j], hs, r0, col)
                for m in range(NB1 if comp else 0):
                    u, r = divmod(m * PR, CH)
                    op = lhs_operands(sc1, lambda t, k: abuf[t * MC1:(t + 1) * MC1, k * L:(k + 1) * L]) if m == 0 else nxt
                    nxt, lns, forms = operands(xb * TM1 + shift + m * PR)
                    if m == NB1 - 1:
                        def put(t):
                            abuf[t * MC1:(t + 1) * MC1, :] = layernorm(xb * TM1 + m * PR + t * MC1, MC1)
                        lns, forms = [functools.partial(put, t) for t in range(sc1["m"])], []
                    ns = 4 * NP1
                    todo = {}
                    for e, f in enumerate(lns):
                        todo.setdefault(int(ns * (F0 + (F1 - F0) * e / len(lns))), []).append(f)
                    for e, f in enumerate(forms):
                        todo.setdefault(int(ns * (F2 + (F3 - F2) * e / len(forms))), []).append(f)
                    for c in range(4):
                        def product(p):
                            for f in todo.pop(c * NP1 + p, []):
                                f()
                            return jnp.dot(op(p), upk(ws[p * 4 + c]), preferred_element_type=F32)
                        if YB == 0:
                            combine(sc1, product, lambda t, j, y: act(y, slots[u], r + t * MC1, 4 * j + c))
                        else:
                            def park(t, j, y):
                                ybuf[c % YB, t * 3 + j] = y
                                parked.append((c % YB, t, j, slots[u], r + t * MC1, 4 * j + c))
                                while len(parked) > YD:
                                    flush()
                            combine(sc1, park_product(product), park)
                    assert not todo
                    if m == A1:
                        @pl.when(i + 1 < NT1)
                        def _():
                            x1_copy(i + 1, 1 - xb).start()
                        @pl.when(i == NT1 - 1)
                        def _():
                            restage()
                while parked:
                    flush()
                prev = [(i + 1) * G1 + u - S for u in range(G1)]
                busy = tuple(jnp.logical_and(c >= 0, stored(jnp.maximum(c, 0))).astype(jnp.int32) for c in prev)
                return 1 - xb, wrap(hb + G1, S), qn, wrap(qs + (qn - q), S), busy

            z = jnp.int32(0)
            x0_copy().wait()
            stage(W1ROW + HID)
            if run1:
                lax.fori_loop(0, NT1, phase1, (z, z, z, z, (z,) * G1))
            else:
                x1_copy(0, 0).wait()
                restage()

            free2 = [s for s in range(XR2) if (s + 1) * TM2 <= W2ROW or s * TM2 >= W2ROW + HID]
            first2 = [(j, (NT2 - 1 - j) % XR2) for j in range(XR2 - 1)]
            if run2:
                for j, s in first2:
                    if s in free2:
                        x_copy(NT2 - 1 - j, s, TM2).start()
            gx = jnp.sqrt(jnp.sum(ssq[...], axis=0, keepdims=True) * (HS * HS) + 1e-6)
            nx = gx / (jnp.mean(gx, axis=-1, keepdims=True) + 1e-6)
            sc = (g_ref[...].astype(F32) * nx + 1.0) * HS
            w2_copy().wait()
            for r in range(KG2):
                cols = [jnp.broadcast_to(sc[:, (KG2 * k + r) * L:(KG2 * k + r + 1) * L], (L, L)).T for k in range(sc2["k"])]
                tile = lambda k, j: xbuf[W2ROW + (KG2 * k + r) * L:W2ROW + (KG2 * k + r + 1) * L, j * L:(j + 1) * L].astype(F32) * cols[k]
                for p in range(NP2):
                    ws[p * KG2 + r] = pk(weight_form(sc2, p, tile))
            WR = NP2 * KG2
            if PT:
                for q in range(4):
                    w1_copy(q, W2ROW + HID).wait()
                for c in range(4):
                    for p in range(len(HK["w"])):
                        ws[WR + p * 4 + c] = pk(weight_form(HK, p, lambda k, j: w1_tile(k, 4 * j + c, W2ROW + HID)))
            bv = b_ref[...].astype(F32)
            bias = jnp.zeros((8, C), F32)
            for k in range(HID // L):
                col = jnp.broadcast_to(bv[:, k * L:(k + 1) * L], (L, L)).T
                prod = xbuf[W2ROW + k * L:W2ROW + (k + 1) * L, :C].astype(F32) * jnp.concatenate([col] * 3, axis=1)
                bias = bias + jnp.sum(prod.reshape(L // 8, 8, C), axis=0)
            bias = jnp.broadcast_to(jnp.sum(bias, axis=0, keepdims=True), (8, C))
            vec[8:16, :] = bias
            if run2:
                for j, s in first2:
                    if s not in free2:
                        x_copy(NT2 - 1 - j, s, TM2).start()

            def phase2(j, carry):
                xs, hb, q, qs, fetched, redo = carry
                i = NT2 - 1 - j
                slots = [wrap(hb + u, S) for u in range(G2)]
                nxs, nhb = wrapn(xs - 1, XR2), wrapn(hb - G2, S)

                s2 = wrap(xs + 2, XR2)
                x_copy(i, xs, TM2).wait()
                for u in range(G2):
                    @pl.when(fetched[u] != 0)
                    def _():
                        h_in(0, slots[u]).wait()
                @pl.when(jnp.logical_and(j >= 2, i + 2 > TD))
                def _():
                    o_copy(i + 2, s2).wait()
                def start_io():
                    @pl.when(jnp.logical_and(j >= 1, i + 1 > TD))
                    def _():
                        o_copy(i + 1, wrap(xs + 1, XR2)).start(priority=PO)
                    if TD:
                        @pl.when(i == 0)
                        def _():
                            for t in range(TD, 0, -1):
                                o_copy(t, t % XR2).start(priority=PO)
                    @pl.when(jnp.logical_and(j >= 1, i + 2 - XR2 >= 0))
                    def _():
                        x_copy(i + 2 - XR2, s2, TM2).start(priority=PX)

                if PT and comp:
                    @pl.when(redo != 0)
                    def _():
                        start_io()
                        def rows(g, carry):
                            for r in range(0, RCH, 2 * MCR):
                                r = g * RCH + r
                                a = [layernorm(xs * TM2 + r + t * MCR, MCR) for t in range(2)]
                                op = lhs_operands(HK, lambda t, k: a[t][:, k * L:(k + 1) * L])
                                for c in range(4):
                                    def keep(t, jj, y):
                                        rr = pl.ds(pl.multiple_of((r + t * MCR) // 2, 8), MCR // 2)
                                        hbuf[slots[0], rr, (4 * jj + c) * L:(4 * jj + c + 1) * L] = pack16(gelu(y))
                                    combine(HK, lambda p: jnp.dot(op(p), upk(ws[WR + p * 4 + c]), preferred_element_type=F32), keep)
                            return carry
                        lax.fori_loop(0, CH // RCH, rows, 0)

                    pl.when(redo == 0)(start_io)
                else:
                    start_io()

                NB2 = TM2 // (sc2['m'] * MC2)
                for mi, m in enumerate(reversed(range(NB2))):
                    if mi % (NB2 // G2) == A2 and (MID or mi == A2):
                        e = mi // (NB2 // G2)
                        qn = jnp.minimum(jnp.minimum((((j * G2 + e) * R2) >> 16) // G2 + LEAD, j * G2 + e), NHC)
                        for u in range(G2):
                            @pl.when(jnp.logical_and(q + u < qn, stored(jnp.maximum(NHC - 1 - q - u, 0))))
                            def _():
                                h_in(NHC - 1 - q - u, wrapn(qs - u, S)).start(priority=PH)
                        qn = jnp.clip(qn, q, q + G2)
                        q, qs = qn, wrapn(qs - (qn - q), S)
                    if not comp:
                        continue
                    r0 = [(sc2['m'] * m + t) * MC2 for t in range(sc2['m'])]
                    orow = lambda t: pl.ds(pl.multiple_of(xs * TM2 + r0[t], 16), MC2)
                    hload = (lambda t, c0, n: unpack16(hbuf[slots[r0[t] // CH], c0 // L, pl.ds(r0[t] % CH // 2, MC2 // 2), :])) if HL else (lambda t, c0, n: unpack16(hbuf[slots[r0[t] // CH], pl.ds(r0[t] % CH // 2, MC2 // 2), c0:c0 + n]))
                    acc = {}
                    for r in range(KG2):
                        op = lhs_operands(sc2, lambda t, k: hload(t, (KG2 * k + r) * L, L))
                        def accum(t, jj, o):
                            cs = slice(jj * L, (jj + 1) * L)
                            terms = [o] if r == 0 else ([acc[t, jj], o] if OR & 1 else [o, acc[t, jj]])
                            extra = ([xbuf[orow(t), cs].astype(F32)] if r == RX else []) + ([jnp.concatenate([vec[8:16, cs]] * (MC2 // 8), axis=0)] if r == RB else [])
                            if OR & 2:
                                extra = extra[::-1]
                            terms = extra + terms if OR & 4 else terms + extra
                            acc[t, jj] = functools.reduce(lambda a, b: a + b, terms)
                            if r == KG2 - 1:
                                xbuf[orow(t), cs] = acc[t, jj].astype(BF16)
                        combine(sc2, lambda p: jnp.dot(op(p), upk(ws[p * KG2 + r]), preferred_element_type=F32), accum)
                nxt = [jnp.maximum(i - 1, 0) * G2 + u for u in range(G2)]
                fetched = tuple(jnp.logical_and(c < NHC, stored(c)).astype(jnp.int32) for c in nxt)
                redo = jnp.logical_and(nxt[0] < NHC, jnp.logical_not(stored(nxt[0]))).astype(jnp.int32)
                return nxs, nhb, q, qs, fetched, redo

            if run2:
                lax.fori_loop(0, NT2, phase2, (z + (NT2 - 1) % XR2, z + (NCH - G2) % S, z, z + (NHC - 1) % S, (z,) * G2, z))
                o_copy(0, 0).start()
                for t in range(max(TD, 1), -1, -1):
                    o_copy(t, t % XR2).wait()

        out, _ = pl.pallas_call(
            kernel,
            in_specs=[pl.BlockSpec(memory_space=pl.ANY), pl.BlockSpec(memory_space=pltpu.VMEM),
                      pl.BlockSpec(memory_space=pl.ANY), pl.BlockSpec(memory_space=pl.ANY),
                      pl.BlockSpec(memory_space=pltpu.VMEM), pl.BlockSpec(memory_space=pltpu.VMEM)],
            out_specs=[pl.BlockSpec(memory_space=pl.ANY)] * 2,
            out_shape=[jax.ShapeDtypeStruct((N, C), BF16), jax.ShapeDtypeStruct((NHC - NREC,) + ((HID // L, CH // 2, L) if HL else (CH // 2, HID)), U32)],
            scratch_shapes=[
                pltpu.VMEM((XT, XW), BF16),
                pltpu.VMEM((S,) + ((HID // L, CH // 2, L) if HL else (CH // 2, HID)), U32),
                pltpu.VMEM((max(NP1 * 4, NP2 * KG2 + (60 if PT else 0)), L // 2, L), U32),
                pltpu.VMEM((8, HID), F32),
                pltpu.VMEM((16, C), F32),
                pltpu.VMEM((PR, C), F32),
                pltpu.VMEM((max(YB, 1), 3 * sc1['m'], MC1 if YB else 8, L), F32),
                pltpu.SemaphoreType.DMA((max(XC, XR2),)),
                pltpu.SemaphoreType.DMA((XR2,)),
                pltpu.SemaphoreType.DMA((S,)),
                pltpu.SemaphoreType.DMA((5,)),
            ],
            compiler_params=pltpu.CompilerParams(vmem_limit_bytes=vmem_mb * 1024 * 1024, flags=flags, disable_bounds_checks=nobc),
        )(x.reshape(N, C), dw.reshape(1, C), w1, w2, grn_g.reshape(1, HID), grn_b.reshape(1, HID))
        return out.reshape(x.shape)
    return fn


pallas_standalone__modern_conv_block_slak__vision_kernel = make(E1=3,E2=1.5,MC1=48,LNR=48,sc1='Sg',nobc=True,sc2='S343',MC2=32,S=52,PT=16,OFF=8,LEAD=1,A1=0)
```

```python
import functools

import jax
import jax.experimental.pallas as pl
import jax.experimental.pallas.tpu as pltpu
import jax.numpy as jnp
import numpy as np
from jax import lax

F32, BF16, U32 = jnp.float32, jnp.bfloat16, jnp.uint32
L = 128
C, HID = 384, 1536

_K0 = float(np.sqrt(2.0 / np.pi))
ALPHA = float((_K0 * 0.044715) ** (1.0 / 3.0))
C0 = _K0 / ALPHA
HS = 0.5 / ALPHA

CH = 768
SLOTS = 52
G1, G2 = 4, 2
XR = 4
HOLD = 3
MC1, MC2, MCR = 48, 32, 48
REDO_EVERY, REDO_FIRST = 32, 16

UP = dict(
    m=4, k=3, n=3,
    a_prog=[(10,-1,3,1), (6,-1,3,1), (3,1,7,-1), (5,-1,1,1), (11,-1,0,1), (9,-1,13,1), (11,-1,17,1), (6,1,18,1),
            (10,-1,4,1), (5,1,20,1), (7,-1,20,1), (21,1,7,-1), (22,1,1,1), (2,1,5,1), (8,-1,25,1), (0,1,25,1),
            (8,-1,27,1), (1,1,12,-1), (29,1,20,1), (2,1,11,1), (1,1,31,1), (8,-1,23,1), (33,1,18,1), (28,1,13,1),
            (14,-1,35,1), (12,1,19,-1), (16,1,37,1)],
    a_use=[5, 0, 27, 1, 32, 15, 30, 3, 11, 16, 10, 14, 12, 19, 21, 38, 13, 7, 8, 10, 23, 18, 22, 34, 24, 28, 26, 17,
           36],
    c_prog=[(4,1,7,1), (0,1,3,-1), (4,1,10,1), (2,1,9,1), (10,1,8,1), (5,1,8,1), (5,1,11,1), (4,-1,1,1), (6,-1,1,1),
            (18,1,9,1), (2,1,13,1), (6,1,12,1), (8,1,19,1), (23,1,14,-1), (24,1,12,1), (17,1,21,-1), (2,1,10,-1),
            (28,1,11,-1), (22,1,24,1), (30,1,17,-1), (23,1,21,1), (32,1,3,1), (2,1,0,1), (34,1,6,1), (0,1,1,1),
            (36,1,9,-1)],
    c_use=[(31,-1), (37,-1), (35,1), (13,-1), (2,-1), (22,-1), (3,-1), (33,-1), (29,-1), (15,1), (18,1), (23,-1),
           (21,1), (27,1), (17,-1), (9,1), (25,-1), (12,1), (26,1), (14,-1), (24,-1), (16,1), (19,-1), (8,-1), (1,-1),
           (20,1), (1,-1), (10,-1), (6,-1)],
    w=[(0,0,0,0,0,-1,0,0,1), (-1,0,0,0,0,0,1,0,0), (0,0,0,0,0,0,1,0,0), (0,0,0,-1,0,1,1,0,-1),
       (0,0,0,0,0,0,1,0,-1), (0,0,0,0,0,-1,-1,0,1), (0,0,0,-1,0,0,0,0,0), (-1,0,0,-1,0,0,0,0,0),
       (0,0,-1,0,0,0,0,0,1), (0,0,1,0,0,0,-1,0,0), (-1,0,1,-1,0,1,0,0,0), (1,-1,0,1,0,0,0,0,0),
       (-1,0,1,-1,0,0,0,0,0), (0,0,1,0,0,0,0,0,0), (0,0,0,0,0,-1,0,0,0), (1,0,-1,0,0,0,0,0,0), (0,1,0,0,0,0,0,0,0),
       (-1,1,0,-1,1,0,0,0,0), (0,0,0,0,0,0,0,1,0), (0,0,0,0,-1,0,0,0,0), (0,0,0,0,0,1,0,1,-1),
       (0,0,-1,0,0,0,0,-1,1), (0,0,0,0,1,-1,0,-1,1), (0,0,0,0,0,0,0,-1,1), (0,0,0,0,-1,0,0,0,0),
       (-1,1,0,0,0,0,1,0,0), (-1,1,0,0,0,0,1,-1,0), (0,1,-1,0,0,0,0,-1,1), (1,-1,0,0,0,0,0,0,0)],
)

DOWN = dict(
    m=3, k=4, n=3,
    a_prog=[(0,1,10,-1), (4,1,5,1), (6,1,5,1), (7,1,5,1), (11,1,4,1), (3,1,6,1), (9,1,8,1), (11,1,9,1), (2,1,1,1),
            (0,1,18,-1), (3,1,15,1), (20,1,10,-1), (14,1,11,-1), (22,1,13,-1), (21,1,19,1), (24,1,15,-1), (23,1,24,-1),
            (28,1,19,-1), (12,1,26,-1), (30,1,16,1), (1,1,3,1), (32,-1,23,1), (33,-1,12,1), (34,1,17,-1), (32,1,21,1),
            (15,1,36,1)],
    a_use=[6, 13, 15, 14, 24, 20, 3, 23, 27, 17, 25, 6, 22, 4, 16, 29, 10, 37, 11, 35, 33, 19, 31, 18, 12, 0, 21, 26,
           1],
    c_prog=[(0,1,2,-1), (5,1,8,-1), (0,1,6,1), (6,1,8,-1), (2,1,6,1), (2,1,8,1), (3,-1,0,1), (7,1,8,-1), (0,1,1,-1),
            (1,-1,15,1), (2,1,16,-1), (15,1,2,-1), (5,1,16,1), (6,1,17,1), (6,1,10,1), (19,-1,1,1), (3,1,23,-1),
            (18,1,4,1), (22,1,7,-1), (4,1,21,-1), (20,1,5,1)],
    c_use=[(4,1), (4,1), (26,1), (28,-1), (21,1), (24,-1), (15,-1), (19,1), (5,-1), (20,1), (3,1), (29,1), (18,1),
           (25,1), (23,-1), (16,1), (14,1), (17,-1), (10,-1), (9,1), (2,-1), (7,-1), (12,1), (27,-1), (13,1), (11,-1),
           (22,-1), (6,1), (1,-1)],
    w=[(0,1,0,0,-1,0,0,1,0,0,1,0), (0,1,0,0,0,0,0,0,0,0,0,0), (0,0,0,0,0,0,0,0,0,0,1,0),
       (0,1,0,0,-1,0,0,0,0,0,1,0), (0,-1,0,0,1,1,0,0,0,0,-1,0), (0,0,0,0,0,0,0,-1,0,0,0,0),
       (0,0,0,0,0,1,-1,0,-1,-1,-1,-1), (0,0,0,0,0,1,0,1,0,0,0,0), (0,0,0,0,0,0,0,0,0,0,0,1),
       (0,0,0,0,0,1,-1,0,-1,0,0,-1), (0,0,0,-1,0,0,0,0,0,1,0,0), (0,0,0,0,0,-1,0,0,1,0,0,1),
       (0,0,0,-1,0,0,0,0,0,0,-1,0), (1,0,0,-1,0,0,0,0,0,1,0,0), (-1,0,-1,1,0,0,0,0,0,-1,0,0),
       (0,0,0,0,0,1,0,0,0,0,0,0), (0,0,1,0,0,0,0,1,1,0,0,0), (0,0,0,-1,0,0,0,0,0,0,0,0),
       (1,1,1,-1,-1,-1,0,0,0,1,1,1), (0,0,0,0,0,0,-1,0,0,0,0,0), (0,0,0,0,0,1,-1,0,-1,0,0,0),
       (0,1,0,0,-1,-1,0,0,0,0,0,0), (0,0,-1,0,0,0,0,0,0,0,0,0), (0,1,0,0,0,0,0,0,0,0,0,0),
       (0,0,1,0,0,0,-1,0,0,0,0,0), (-1,-1,0,0,0,0,-1,0,0,0,0,0), (0,1,0,1,0,0,0,0,0,0,0,0),
       (-1,0,-1,1,0,0,0,0,0,0,0,0), (0,0,0,-1,-1,0,0,1,0,0,0,0)],
)

UP15 = dict(
    m=2, k=3, n=3,
    a_prog=[(5,1,4,1), (5,-1,3,1), (0,1,2,-1), (0,1,3,-1), (2,1,3,-1), (5,-1,2,1), (0,1,1,-1), (12,1,3,-1), (6,-1,2,1),
            (1,1,14,1), (13,1,4,1)],
    a_use=[4, 14, 6, 1, 2, 12, 15, 8, 13, 16, 7, 3, 10, 11, 9],
    c_prog=[(5,-1,0,1), (5,1,3,1), (3,1,0,1), (1,1,2,-1), (4,-1,3,1), (0,1,2,1), (5,1,2,1), (12,-1,1,1), (0,1,10,1),
            (1,-1,14,1), (4,1,13,1)],
    c_use=[(4,1), (13,-1), (16,1), (1,1), (12,1), (15,1), (9,-1), (11,-1), (14,-1), (10,1), (7,1), (8,-1), (6,-1),
           (5,-1), (0,1)],
    w=[(0,0,0,1,1,0,0,-1,0), (0,0,0,0,0,-1,0,-1,0), (0,0,0,0,0,0,0,1,0), (0,1,0,0,1,1,0,0,0), (0,0,1,0,0,0,0,1,1),
       (0,-1,0,0,0,0,0,0,0), (0,0,0,0,0,1,0,0,0), (0,0,-1,0,0,0,0,0,0), (0,-1,0,1,0,0,0,0,0), (0,0,0,1,0,0,0,0,0),
       (0,0,0,0,0,0,-1,0,0), (-1,-1,0,0,0,0,-1,0,0), (0,0,-1,0,0,0,-1,0,0), (0,0,0,0,0,-1,-1,0,1),
       (1,0,-1,1,0,0,0,0,0)],
)


def _lhs_operands(sc, block):
    m, k = sc["m"], sc["k"]
    memo, packed = {}, {}

    def node(v):
        if v not in memo:
            if v < m * k:
                memo[v] = (1, block(v // k, v % k))
            else:
                a, sa, b, sb = sc["a_prog"][v - m * k]
                (ta, xa), (tb, xb) = node(a), node(b)
                ta, tb = ta * sa, tb * sb
                memo[v] = (ta, xa + xb) if ta == tb else (1, xa - xb if ta > 0 else xb - xa)
        return memo[v]

    def operand(p):
        v = sc["a_use"][p]
        if v not in packed:
            packed[v] = node(v)[1].astype(BF16)
        return packed[v]

    return operand


def _combine(sc, product, emit):
    m, n = sc["m"], sc["n"]
    pending = [0] * (m * n + len(sc["c_prog"]))
    for v, _ in sc["c_use"]:
        pending[v] += 1
    for a, _, b, _ in sc["c_prog"]:
        pending[a] += 1
        pending[b] += 1
    partial = {}

    def push(v, t, x):
        if v in partial:
            u, y = partial[v]
            t, x = (t, y + x) if t == u else (1, x - y if t > 0 else y - x)
        partial[v] = (t, x)
        pending[v] -= 1
        if pending[v] == 0:
            if v >= m * n:
                a, sa, b, sb = sc["c_prog"][v - m * n]
                push(a, t * sa, x)
                push(b, t * sb, x)
            else:
                assert t == 1
                emit(v // n, v % n, x)

    for p, (v, t) in enumerate(sc["c_use"]):
        push(v, t, product(p))


def _rhs_operand(sc, p, block):
    coef, acc = sc["w"][p], None
    for q in sorted(range(len(coef)), key=lambda q: -coef[q]):
        if coef[q]:
            v = block(q // sc["n"], q % sc["n"])
            if acc is None:
                acc = v if coef[q] > 0 else -v
            else:
                acc = acc + v if coef[q] > 0 else acc - v
    return pltpu.bitcast(acc.astype(BF16), U32)


def _dot(a, words):
    return jnp.dot(a, pltpu.bitcast(words, BF16), preferred_element_type=F32)


def _pack(v):
    t = v.shape[0] // 16
    lo = jnp.concatenate([v[16 * g:16 * g + 8] for g in range(t)], axis=0)
    hi = jnp.concatenate([v[16 * g + 8:16 * g + 16] for g in range(t)], axis=0)
    return pltpu.pack_elementwise([lo, hi], packed_dtype=BF16)


def _unpack(w):
    lo, hi = (pltpu.unpack_elementwise(w, index=i, packed_dtype=BF16, unpacked_dtype=F32) for i in range(2))
    parts = []
    for g in range(w.shape[0] // 8):
        parts += [lo[8 * g:8 * g + 8], hi[8 * g:8 * g + 8]]
    return jnp.concatenate(parts, axis=0)


def _gelu(y):
    return y * jnp.tanh(y * (y * y + C0)) + y


def _column(row, k):
    return jnp.broadcast_to(row[:, k * L:(k + 1) * L], (L, L)).T


def _wrap_up(v, n):
    return jnp.where(v >= n, v - n, v)


def _wrap_down(v, n):
    return jnp.where(v < 0, v + n, v)


def _kernel(x_hbm, dw_ref, w1_hbm, w2_hbm, g_ref, b_ref, out_hbm, h_hbm,
            xbuf, hbuf, wbuf, abuf, ssq, vec, xsem, osem, hsem, wsem):
    n_pix = x_hbm.shape[0]
    tm1, tm2 = G1 * CH, G2 * CH
    nt1, nt2, nch = n_pix // tm1, n_pix // tm2, n_pix // CH
    nhc = nch - SLOTS
    n_redo = nhc - h_hbm.shape[0]
    pace1 = -(-nhc * 65536 // (nt1 - 3))
    pace2 = -(-nhc * 65536 * 2 // (2 * nt2 - 3))
    pr = UP["m"] * MC1
    stage2 = (nt1 % 2) * tm1

    def stored(c):
        return jnp.logical_or((c + (REDO_EVERY - REDO_FIRST)) % REDO_EVERY != 0,
                              c >= REDO_FIRST + n_redo * REDO_EVERY)

    def h_index(c):
        return c - jnp.minimum((c + (REDO_EVERY - 1 - REDO_FIRST)) // REDO_EVERY, n_redo)

    def h_out(c, slot):
        return pltpu.make_async_copy(hbuf.at[slot], h_hbm.at[h_index(c)], hsem.at[slot])

    def h_in(c, slot):
        return pltpu.make_async_copy(h_hbm.at[h_index(c)], hbuf.at[slot], hsem.at[slot])

    def x_rows(slot, tm):
        return xbuf.at[pl.ds(pl.multiple_of(slot * tm, tm), tm)]

    def x1_in(i, slot):
        row = pl.multiple_of(jnp.minimum(i * tm1 + pr, n_pix - tm1), 16)
        return pltpu.make_async_copy(x_hbm.at[pl.ds(row, tm1)], x_rows(slot, tm1), xsem.at[slot])

    def x2_in(i, slot):
        return pltpu.make_async_copy(x_hbm.at[pl.ds(i * tm2, tm2)], x_rows(slot, tm2), xsem.at[slot])

    def o_out(i, slot):
        return pltpu.make_async_copy(x_rows(slot, tm2), out_hbm.at[pl.ds(i * tm2, tm2)], osem.at[slot])

    def w1_in(q, row):
        return pltpu.make_async_copy(w1_hbm.at[:, pl.ds(q * C, C)], xbuf.at[pl.ds(row + q * C, C)], wsem.at[q])

    def w2_in():
        return pltpu.make_async_copy(w2_hbm, xbuf.at[pl.ds(stage2, HID)], wsem.at[4])

    def w1_forms(sc, row, first):
        def tile(k, n):
            r = row + (n // 3) * C + k * L
            return xbuf[r:r + L, (n % 3) * L:(n % 3 + 1) * L].astype(F32)

        for q in range(4):
            w1_in(q, row).wait()
        for c in range(4):
            for p in range(len(sc["w"])):
                wbuf[first + p * 4 + c] = _rhs_operand(sc, p, lambda k, j: tile(k, 4 * j + c))

    def layernorm(row, n):
        y = xbuf[pl.ds(pl.multiple_of(row, 16), n), :].astype(F32) * jnp.concatenate([vec[0:8, :]] * (n // 8), axis=0)
        d = y - jnp.sum(y, axis=-1, keepdims=True) * (1.0 / C)
        v = jnp.sum(d * d, axis=-1, keepdims=True) * (1.0 / (C * ALPHA * ALPHA)) + 1e-5 / (ALPHA * ALPHA)
        return d * jnp.exp2(-0.5 * jnp.log2(v))

    x0_in = pltpu.make_async_copy(x_hbm.at[pl.ds(0, pr)], xbuf.at[pl.ds(tm1 + HID, pr)], osem.at[0])
    for q in range(4):
        w1_in(q, tm1).start()
    x0_in.start()
    x1_in(0, 0).start()
    ssq[...] = jnp.zeros_like(ssq)
    vec[0:8, :] = jnp.broadcast_to(dw_ref[...].astype(F32), (8, C))
    w1_forms(UP, tm1, 0)
    x0_in.wait()
    for t in range(UP["m"]):
        abuf[t * MC1:(t + 1) * MC1, :] = layernorm(tm1 + HID + t * MC1, MC1)

    def pass1(i, carry):
        xs, hs, q, qs, busy = carry
        slots = [_wrap_up(hs + u, SLOTS) for u in range(G1)]
        qn = jnp.minimum((i * pace1) >> 16, nhc)
        x1_in(i, xs).wait()
        for u in range(G1):
            pl.when(busy[u] != 0)(lambda: h_out(0, slots[u]).wait())
        for u in range(G1):
            pl.when(jnp.logical_and(q + u < qn, stored(q + u)))(
                lambda: h_out(q + u, _wrap_up(qs + u, SLOTS)).start())
        ahead = xs * tm1 + jnp.where(i == nt1 - 1, pr, 0)

        groups, n_prod = tm1 // pr, len(UP["w"])
        nxt = _lhs_operands(UP, lambda t, k: abuf[t * MC1:(t + 1) * MC1, k * L:(k + 1) * L])
        for m in range(groups):
            u, r = divmod(m * pr, CH)
            op, normed = nxt, {}

            def norm(t, m=m, normed=normed):
                if m < groups - 1:
                    normed[t] = layernorm(ahead + m * pr + t * MC1, MC1)
                else:
                    abuf[t * MC1:(t + 1) * MC1, :] = layernorm(xs * tm1 + m * pr + t * MC1, MC1)

            nxt = _lhs_operands(UP, lambda t, k, normed=normed: normed[t][:, k * L:(k + 1) * L])
            todo = {}
            for t in range(UP["m"]):
                todo.setdefault(int(4 * n_prod * 0.65 * t / UP["m"]), []).append(functools.partial(norm, t))
            for p in range(n_prod if m < groups - 1 else 0):
                todo.setdefault(int(4 * n_prod * (0.68 + 0.29 * p / n_prod)), []).append(functools.partial(nxt, p))

            for c in range(4):
                def product(p):
                    for step in todo.pop(c * n_prod + p, []):
                        step()
                    return _dot(op(p), wbuf[p * 4 + c])

                def activate(t, j, y):
                    cols = slice((4 * j + c) * L, (4 * j + c + 1) * L)
                    h = _gelu(y)
                    ssq[:, cols] += jnp.sum((h * h).reshape(MC1 // 8, 8, L), axis=0)
                    hbuf[slots[u], pl.ds((r + t * MC1) // 2, MC1 // 2), cols] = _pack(h)

                _combine(UP, product, activate)
            if m == 0:
                pl.when(i + 1 < nt1)(lambda: x1_in(i + 1, 1 - xs).start())

                @pl.when(i == nt1 - 1)
                def _():
                    w2_in().start()
                    for e in range(4):
                        w1_in(e, stage2 + HID).start()

        prev = [(i + 1) * G1 + u - SLOTS for u in range(G1)]
        busy = tuple(jnp.logical_and(c >= 0, stored(jnp.maximum(c, 0))).astype(jnp.int32) for c in prev)
        return 1 - xs, _wrap_up(hs + G1, SLOTS), qn, _wrap_up(qs + (qn - q), SLOTS), busy

    zero = jnp.int32(0)
    lax.fori_loop(0, nt1, pass1, (zero, zero, zero, zero, (zero,) * G1))

    first = [(nt2 - 1 - j, (nt2 - 1 - j) % XR) for j in range(XR - 1)]
    early = [(i, s) for i, s in first if (s + 1) * tm2 <= stage2 or s * tm2 >= stage2 + 2 * HID]
    for i, s in early:
        x2_in(i, s).start()
    gx = jnp.sqrt(jnp.sum(ssq[...], axis=0, keepdims=True) * (HS * HS) + 1e-6)
    nx = gx / (jnp.mean(gx, axis=-1, keepdims=True) + 1e-6)
    scale = (g_ref[...].astype(F32).reshape(1, HID) * nx + 1.0) * HS
    kg = HID // L // DOWN["k"]
    w2_in().wait()
    for r in range(kg):
        cols = [_column(scale, kg * k + r) for k in range(DOWN["k"])]

        def w2_tile(k, j):
            row = stage2 + (kg * k + r) * L
            return xbuf[row:row + L, j * L:(j + 1) * L].astype(F32) * cols[k]

        for p in range(len(DOWN["w"])):
            wbuf[p * kg + r] = _rhs_operand(DOWN, p, w2_tile)
    up15 = len(DOWN["w"]) * kg
    w1_forms(UP15, stage2 + HID, up15)
    b_row = b_ref[...].astype(F32).reshape(1, HID)
    bias = jnp.zeros((8, C), F32)
    for k in range(HID // L):
        prod = xbuf[stage2 + k * L:stage2 + (k + 1) * L, :].astype(F32) * jnp.concatenate([_column(b_row, k)] * 3, axis=1)
        bias = bias + jnp.sum(prod.reshape(L // 8, 8, C), axis=0)
    vec[8:16, :] = jnp.broadcast_to(jnp.sum(bias, axis=0, keepdims=True), (8, C))
    for i, s in first:
        if (i, s) not in early:
            x2_in(i, s).start()

    def pass2(j, carry):
        xs, hs, q, qs, fetched, redo = carry
        i = nt2 - 1 - j
        slots = [_wrap_up(hs + u, SLOTS) for u in range(G2)]
        s2 = _wrap_up(xs + 2, XR)
        x2_in(i, xs).wait()
        for u in range(G2):
            pl.when(fetched[u] != 0)(lambda: h_in(0, slots[u]).wait())
        pl.when(jnp.logical_and(j >= 2, i + 2 > HOLD))(lambda: o_out(i + 2, s2).wait())

        def start_io():
            pl.when(jnp.logical_and(j >= 1, i + 1 > HOLD))(lambda: o_out(i + 1, _wrap_up(xs + 1, XR)).start())

            @pl.when(i == 0)
            def _():
                for t in range(HOLD, 0, -1):
                    o_out(t, t % XR).start()

            pl.when(jnp.logical_and(j >= 1, i + 2 - XR >= 0))(lambda: x2_in(i + 2 - XR, s2).start())

        @pl.when(redo != 0)
        def _():
            start_io()

            def recompute(half, _):
                for r in range(0, CH // 2, 2 * MCR):
                    r = half * (CH // 2) + r
                    a = [layernorm(xs * tm2 + r + t * MCR, MCR) for t in range(2)]
                    op = _lhs_operands(UP15, lambda t, k: a[t][:, k * L:(k + 1) * L])
                    for c in range(4):
                        def keep(t, jj, y):
                            rows = pl.ds(pl.multiple_of((r + t * MCR) // 2, 8), MCR // 2)
                            hbuf[slots[0], rows, (4 * jj + c) * L:(4 * jj + c + 1) * L] = _pack(_gelu(y))

                        _combine(UP15, lambda p: _dot(op(p), wbuf[up15 + p * 4 + c]), keep)
                return _

            lax.fori_loop(0, 2, recompute, 0)

        pl.when(redo == 0)(start_io)

        rows_per_group = DOWN["m"] * MC2
        groups = tm2 // rows_per_group
        for step, m in enumerate(reversed(range(groups))):
            if step % (groups // G2) == 1:
                done = j * G2 + step // (groups // G2)
                qn = jnp.minimum(jnp.minimum(((done * pace2) >> 16) // G2 + 1, done), nhc)
                for u in range(G2):
                    pl.when(jnp.logical_and(q + u < qn, stored(jnp.maximum(nhc - 1 - q - u, 0))))(
                        lambda: h_in(nhc - 1 - q - u, _wrap_down(qs - u, SLOTS)).start())
                qn = jnp.clip(qn, q, q + G2)
                q, qs = qn, _wrap_down(qs - (qn - q), SLOTS)

            u, r0 = divmod(m * rows_per_group, CH)
            acc = {}
            for r in range(kg):
                op = _lhs_operands(DOWN, lambda t, k: _unpack(
                    hbuf[slots[u], pl.ds((r0 + t * MC2) // 2, MC2 // 2), (kg * k + r) * L:(kg * k + r + 1) * L]))

                def accumulate(t, jj, o):
                    acc[t, jj] = o if r == 0 else acc[t, jj] + o
                    if r == kg - 1:
                        rows = pl.ds(pl.multiple_of(xs * tm2 + u * CH + r0 + t * MC2, 16), MC2)
                        cols = slice(jj * L, (jj + 1) * L)
                        res = acc[t, jj] + xbuf[rows, cols].astype(F32)
                        res = res + jnp.concatenate([vec[8:16, cols]] * (MC2 // 8), axis=0)
                        xbuf[rows, cols] = res.astype(BF16)

                _combine(DOWN, lambda p: _dot(op(p), wbuf[p * kg + r]), accumulate)

        nxt = [jnp.maximum(i - 1, 0) * G2 + u for u in range(G2)]
        fetched = tuple(jnp.logical_and(c < nhc, stored(c)).astype(jnp.int32) for c in nxt)
        redo = jnp.logical_and(nxt[0] < nhc, jnp.logical_not(stored(nxt[0]))).astype(jnp.int32)
        return _wrap_down(xs - 1, XR), _wrap_down(hs - G2, SLOTS), q, qs, fetched, redo

    lax.fori_loop(0, nt2, pass2, (zero + (nt2 - 1) % XR, zero + (nch - G2) % SLOTS, zero,
                                  zero + (nhc - 1) % SLOTS, (zero,) * G2, zero))
    o_out(0, 0).start()
    for t in range(HOLD, -1, -1):
        o_out(t, t % XR).wait()


@jax.jit
def pallas_standalone__modern_conv_block_slak__vision_kernel(x, dw, w1, w2, grn_g, grn_b):
    n_pix = x.shape[1] * x.shape[2]
    assert x.shape[0] == 1 and x.shape[3] == C and dw.shape == (1, 1, C) and w1.shape == (C, HID)
    assert n_pix % (G1 * CH) == 0 and n_pix // CH > SLOTS + 4 * G1
    nhc = n_pix // CH - SLOTS
    n_stored = nhc - len(range(REDO_FIRST, nhc, REDO_EVERY))
    n_tiles = max(4 * len(UP["w"]), (HID // L // DOWN["k"]) * len(DOWN["w"]) + 4 * len(UP15["w"]))
    hbm = pl.BlockSpec(memory_space=pl.ANY)
    vmem = pl.BlockSpec(memory_space=pltpu.VMEM)
    out, _ = pl.pallas_call(
        _kernel,
        in_specs=[hbm, vmem, hbm, hbm, vmem, vmem],
        out_specs=[hbm, hbm],
        out_shape=[jax.ShapeDtypeStruct((n_pix, C), BF16), jax.ShapeDtypeStruct((n_stored, CH // 2, HID), U32)],
        scratch_shapes=[
            pltpu.VMEM((max(2 * G1, XR * G2) * CH, C), BF16),
            pltpu.VMEM((SLOTS, CH // 2, HID), U32),
            pltpu.VMEM((n_tiles, L // 2, L), U32),
            pltpu.VMEM((UP["m"] * MC1, C), F32),
            pltpu.VMEM((8, HID), F32),
            pltpu.VMEM((16, C), F32),
            pltpu.SemaphoreType.DMA((XR,)),
            pltpu.SemaphoreType.DMA((XR,)),
            pltpu.SemaphoreType.DMA((SLOTS,)),
            pltpu.SemaphoreType.DMA((5,)),
        ],
        compiler_params=pltpu.CompilerParams(vmem_limit_bytes=128 * 1024 * 1024, disable_bounds_checks=True),
    )(x.reshape(n_pix, C), dw.reshape(1, C), w1, w2, grn_g, grn_b)
    return out.reshape(x.shape)
```

```python
import functools

import jax
import jax.experimental.pallas as pl
import jax.experimental.pallas.tpu as pltpu
import jax.numpy as jnp
import numpy as np
from jax import lax

F32, BF16, U32 = jnp.float32, jnp.bfloat16, jnp.uint32
L = 128
C, HID = 384, 1536

_K0 = float(np.sqrt(2.0 / np.pi))
ALPHA = float((_K0 * 0.044715) ** (1.0 / 3.0))
C0 = _K0 / ALPHA
HS = 0.5 / ALPHA

CH = 768
SLOTS = 52
G1, G2 = 4, 2
XR = 4
HOLD = 3
MC1, MC2, MCR = 48, 32, 48
REDO_EVERY, REDO_FIRST = 32, 16

UP = dict(
    m=4, k=3, n=3,
    a_prog=[(10,-1,3,1), (6,-1,3,1), (3,1,7,-1), (5,-1,1,1), (11,-1,0,1), (9,-1,13,1), (11,-1,17,1), (6,1,18,1),
            (10,-1,4,1), (5,1,20,1), (7,-1,20,1), (21,1,7,-1), (22,1,1,1), (2,1,5,1), (8,-1,25,1), (0,1,25,1),
            (8,-1,27,1), (1,1,12,-1), (29,1,20,1), (2,1,11,1), (1,1,31,1), (8,-1,23,1), (33,1,18,1), (28,1,13,1),
            (14,-1,35,1), (12,1,19,-1), (16,1,37,1)],
    a_use=[5, 0, 27, 1, 32, 15, 30, 3, 11, 16, 10, 14, 12, 19, 21, 38, 13, 7, 8, 10, 23, 18, 22, 34, 24, 28, 26, 17,
           36],
    c_prog=[(4,1,7,1), (0,1,3,-1), (4,1,10,1), (2,1,9,1), (10,1,8,1), (5,1,8,1), (5,1,11,1), (4,-1,1,1), (6,-1,1,1),
            (18,1,9,1), (2,1,13,1), (6,1,12,1), (8,1,19,1), (23,1,14,-1), (24,1,12,1), (17,1,21,-1), (2,1,10,-1),
            (28,1,11,-1), (22,1,24,1), (30,1,17,-1), (23,1,21,1), (32,1,3,1), (2,1,0,1), (34,1,6,1), (0,1,1,1),
            (36,1,9,-1)],
    c_use=[(31,-1), (37,-1), (35,1), (13,-1), (2,-1), (22,-1), (3,-1), (33,-1), (29,-1), (15,1), (18,1), (23,-1),
           (21,1), (27,1), (17,-1), (9,1), (25,-1), (12,1), (26,1), (14,-1), (24,-1), (16,1), (19,-1), (8,-1), (1,-1),
           (20,1), (1,-1), (10,-1), (6,-1)],
    w=[(0,0,0,0,0,-1,0,0,1), (-1,0,0,0,0,0,1,0,0), (0,0,0,0,0,0,1,0,0), (0,0,0,-1,0,1,1,0,-1),
       (0,0,0,0,0,0,1,0,-1), (0,0,0,0,0,-1,-1,0,1), (0,0,0,-1,0,0,0,0,0), (-1,0,0,-1,0,0,0,0,0),
       (0,0,-1,0,0,0,0,0,1), (0,0,1,0,0,0,-1,0,0), (-1,0,1,-1,0,1,0,0,0), (1,-1,0,1,0,0,0,0,0),
       (-1,0,1,-1,0,0,0,0,0), (0,0,1,0,0,0,0,0,0), (0,0,0,0,0,-1,0,0,0), (1,0,-1,0,0,0,0,0,0), (0,1,0,0,0,0,0,0,0),
       (-1,1,0,-1,1,0,0,0,0), (0,0,0,0,0,0,0,1,0), (0,0,0,0,-1,0,0,0,0), (0,0,0,0,0,1,0,1,-1),
       (0,0,-1,0,0,0,0,-1,1), (0,0,0,0,1,-1,0,-1,1), (0,0,0,0,0,0,0,-1,1), (0,0,0,0,-1,0,0,0,0),
       (-1,1,0,0,0,0,1,0,0), (-1,1,0,0,0,0,1,-1,0), (0,1,-1,0,0,0,0,-1,1), (1,-1,0,0,0,0,0,0,0)],
)

DOWN = dict(
    m=3, k=4, n=3,
    a_prog=[(0,1,10,-1), (4,1,5,1), (6,1,5,1), (7,1,5,1), (11,1,4,1), (3,1,6,1), (9,1,8,1), (11,1,9,1), (2,1,1,1),
            (0,1,18,-1), (3,1,15,1), (20,1,10,-1), (14,1,11,-1), (22,1,13,-1), (21,1,19,1), (24,1,15,-1), (23,1,24,-1),
            (28,1,19,-1), (12,1,26,-1), (30,1,16,1), (1,1,3,1), (32,-1,23,1), (33,-1,12,1), (34,1,17,-1), (32,1,21,1),
            (15,1,36,1)],
    a_use=[6, 13, 15, 14, 24, 20, 3, 23, 27, 17, 25, 6, 22, 4, 16, 29, 10, 37, 11, 35, 33, 19, 31, 18, 12, 0, 21, 26,
           1],
    c_prog=[(0,1,2,-1), (5,1,8,-1), (0,1,6,1), (6,1,8,-1), (2,1,6,1), (2,1,8,1), (3,-1,0,1), (7,1,8,-1), (0,1,1,-1),
            (1,-1,15,1), (2,1,16,-1), (15,1,2,-1), (5,1,16,1), (6,1,17,1), (6,1,10,1), (19,-1,1,1), (3,1,23,-1),
            (18,1,4,1), (22,1,7,-1), (4,1,21,-1), (20,1,5,1)],
    c_use=[(4,1), (4,1), (26,1), (28,-1), (21,1), (24,-1), (15,-1), (19,1), (5,-1), (20,1), (3,1), (29,1), (18,1),
           (25,1), (23,-1), (16,1), (14,1), (17,-1), (10,-1), (9,1), (2,-1), (7,-1), (12,1), (27,-1), (13,1), (11,-1),
           (22,-1), (6,1), (1,-1)],
    w=[(0,1,0,0,-1,0,0,1,0,0,1,0), (0,1,0,0,0,0,0,0,0,0,0,0), (0,0,0,0,0,0,0,0,0,0,1,0),
       (0,1,0,0,-1,0,0,0,0,0,1,0), (0,-1,0,0,1,1,0,0,0,0,-1,0), (0,0,0,0,0,0,0,-1,0,0,0,0),
       (0,0,0,0,0,1,-1,0,-1,-1,-1,-1), (0,0,0,0,0,1,0,1,0,0,0,0), (0,0,0,0,0,0,0,0,0,0,0,1),
       (0,0,0,0,0,1,-1,0,-1,0,0,-1), (0,0,0,-1,0,0,0,0,0,1,0,0), (0,0,0,0,0,-1,0,0,1,0,0,1),
       (0,0,0,-1,0,0,0,0,0,0,-1,0), (1,0,0,-1,0,0,0,0,0,1,0,0), (-1,0,-1,1,0,0,0,0,0,-1,0,0),
       (0,0,0,0,0,1,0,0,0,0,0,0), (0,0,1,0,0,0,0,1,1,0,0,0), (0,0,0,-1,0,0,0,0,0,0,0,0),
       (1,1,1,-1,-1,-1,0,0,0,1,1,1), (0,0,0,0,0,0,-1,0,0,0,0,0), (0,0,0,0,0,1,-1,0,-1,0,0,0),
       (0,1,0,0,-1,-1,0,0,0,0,0,0), (0,0,-1,0,0,0,0,0,0,0,0,0), (0,1,0,0,0,0,0,0,0,0,0,0),
       (0,0,1,0,0,0,-1,0,0,0,0,0), (-1,-1,0,0,0,0,-1,0,0,0,0,0), (0,1,0,1,0,0,0,0,0,0,0,0),
       (-1,0,-1,1,0,0,0,0,0,0,0,0), (0,0,0,-1,-1,0,0,1,0,0,0,0)],
)

UP15 = dict(
    m=2, k=3, n=3,
    a_prog=[(5,1,4,1), (5,-1,3,1), (0,1,2,-1), (0,1,3,-1), (2,1,3,-1), (5,-1,2,1), (0,1,1,-1), (12,1,3,-1), (6,-1,2,1),
            (1,1,14,1), (13,1,4,1)],
    a_use=[4, 14, 6, 1, 2, 12, 15, 8, 13, 16, 7, 3, 10, 11, 9],
    c_prog=[(5,-1,0,1), (5,1,3,1), (3,1,0,1), (1,1,2,-1), (4,-1,3,1), (0,1,2,1), (5,1,2,1), (12,-1,1,1), (0,1,10,1),
            (1,-1,14,1), (4,1,13,1)],
    c_use=[(4,1), (13,-1), (16,1), (1,1), (12,1), (15,1), (9,-1), (11,-1), (14,-1), (10,1), (7,1), (8,-1), (6,-1),
           (5,-1), (0,1)],
    w=[(0,0,0,1,1,0,0,-1,0), (0,0,0,0,0,-1,0,-1,0), (0,0,0,0,0,0,0,1,0), (0,1,0,0,1,1,0,0,0), (0,0,1,0,0,0,0,1,1),
       (0,-1,0,0,0,0,0,0,0), (0,0,0,0,0,1,0,0,0), (0,0,-1,0,0,0,0,0,0), (0,-1,0,1,0,0,0,0,0), (0,0,0,1,0,0,0,0,0),
       (0,0,0,0,0,0,-1,0,0), (-1,-1,0,0,0,0,-1,0,0), (0,0,-1,0,0,0,-1,0,0), (0,0,0,0,0,-1,-1,0,1),
       (1,0,-1,1,0,0,0,0,0)],
)


def _lhs_operands(sc, block):
    m, k = sc["m"], sc["k"]
    memo, packed = {}, {}

    def node(v):
        if v not in memo:
            if v < m * k:
                memo[v] = (1, block(v // k, v % k))
            else:
                a, sa, b, sb = sc["a_prog"][v - m * k]
                (ta, xa), (tb, xb) = node(a), node(b)
                ta, tb = ta * sa, tb * sb
                memo[v] = (ta, xa + xb) if ta == tb else (1, xa - xb if ta > 0 else xb - xa)
        return memo[v]

    def operand(p):
        v = sc["a_use"][p]
        if v not in packed:
            packed[v] = node(v)[1].astype(BF16)
        return packed[v]

    return operand


def _combine(sc, product, emit):
    m, n = sc["m"], sc["n"]
    pending = [0] * (m * n + len(sc["c_prog"]))
    for v, _ in sc["c_use"]:
        pending[v] += 1
    for a, _, b, _ in sc["c_prog"]:
        pending[a] += 1
        pending[b] += 1
    partial = {}

    def push(v, t, x):
        if v in partial:
            u, y = partial[v]
            t, x = (t, y + x) if t == u else (1, x - y if t > 0 else y - x)
        partial[v] = (t, x)
        pending[v] -= 1
        if pending[v] == 0:
            if v >= m * n:
                a, sa, b, sb = sc["c_prog"][v - m * n]
                push(a, t * sa, x)
                push(b, t * sb, x)
            else:
                assert t == 1
                emit(v // n, v % n, x)

    for p, (v, t) in enumerate(sc["c_use"]):
        push(v, t, product(p))


def _rhs_operand(sc, p, block):
    coef, acc = sc["w"][p], None
    for q in sorted(range(len(coef)), key=lambda q: -coef[q]):
        if coef[q]:
            v = block(q // sc["n"], q % sc["n"])
            if acc is None:
                acc = v if coef[q] > 0 else -v
            else:
                acc = acc + v if coef[q] > 0 else acc - v
    return pltpu.bitcast(acc.astype(BF16), U32)


def _dot(a, words):
    return jnp.dot(a, pltpu.bitcast(words, BF16), preferred_element_type=F32)


def _pack(v):
    t = v.shape[0] // 16
    lo = jnp.concatenate([v[16 * g:16 * g + 8] for g in range(t)], axis=0)
    hi = jnp.concatenate([v[16 * g + 8:16 * g + 16] for g in range(t)], axis=0)
    return pltpu.pack_elementwise([lo, hi], packed_dtype=BF16)


def _unpack(w):
    lo, hi = (pltpu.unpack_elementwise(w, index=i, packed_dtype=BF16, unpacked_dtype=F32) for i in range(2))
    parts = []
    for g in range(w.shape[0] // 8):
        parts += [lo[8 * g:8 * g + 8], hi[8 * g:8 * g + 8]]
    return jnp.concatenate(parts, axis=0)


def _gelu(y):
    return y * jnp.tanh(y * (y * y + C0)) + y


def _column(row, k):
    return jnp.broadcast_to(row[:, k * L:(k + 1) * L], (L, L)).T


def _wrap_up(v, n):
    return jnp.where(v >= n, v - n, v)


def _wrap_down(v, n):
    return jnp.where(v < 0, v + n, v)


def _kernel(x_hbm, dw_ref, w1_hbm, w2_hbm, g_ref, b_ref, out_hbm, h_hbm,
            xbuf, hbuf, wbuf, abuf, ssq, vec, xsem, osem, hsem, wsem):
    n_pix = x_hbm.shape[0]
    tm1, tm2 = G1 * CH, G2 * CH
    nt1, nt2, nch = n_pix // tm1, n_pix // tm2, n_pix // CH
    nhc = nch - SLOTS
    n_redo = nhc - h_hbm.shape[0]
    pace1 = -(-nhc * 65536 // (nt1 - 3))
    pace2 = -(-nhc * 65536 * 2 // (2 * nt2 - 3))
    pr = UP["m"] * MC1
    stage2 = (nt1 % 2) * tm1

    def stored(c):
        return jnp.logical_or((c + (REDO_EVERY - REDO_FIRST)) % REDO_EVERY != 0,
                              c >= REDO_FIRST + n_redo * REDO_EVERY)

    def h_index(c):
        return c - jnp.minimum((c + (REDO_EVERY - 1 - REDO_FIRST)) // REDO_EVERY, n_redo)

    def h_out(c, slot):
        return pltpu.make_async_copy(hbuf.at[slot], h_hbm.at[h_index(c)], hsem.at[slot])

    def h_in(c, slot):
        return pltpu.make_async_copy(h_hbm.at[h_index(c)], hbuf.at[slot], hsem.at[slot])

    def x_rows(slot, tm):
        return xbuf.at[pl.ds(pl.multiple_of(slot * tm, tm), tm)]

    def x1_in(i, slot):
        row = pl.multiple_of(jnp.minimum(i * tm1 + pr, n_pix - tm1), 16)
        return pltpu.make_async_copy(x_hbm.at[pl.ds(row, tm1)], x_rows(slot, tm1), xsem.at[slot])

    def x2_in(i, slot):
        return pltpu.make_async_copy(x_hbm.at[pl.ds(i * tm2, tm2)], x_rows(slot, tm2), xsem.at[slot])

    def o_out(i, slot):
        return pltpu.make_async_copy(x_rows(slot, tm2), out_hbm.at[pl.ds(i * tm2, tm2)], osem.at[slot])

    def w1_in(q, row):
        return pltpu.make_async_copy(w1_hbm.at[:, pl.ds(q * C, C)], xbuf.at[pl.ds(row + q * C, C)], wsem.at[q])

    def w2_in():
        return pltpu.make_async_copy(w2_hbm, xbuf.at[pl.ds(stage2, HID)], wsem.at[4])

    def w1_forms(sc, row, first):
        def tile(k, n):
            r = row + (n // 3) * C + k * L
            return xbuf[r:r + L, (n % 3) * L:(n % 3 + 1) * L].astype(F32)

        for q in range(4):
            w1_in(q, row).wait()
        for c in range(4):
            for p in range(len(sc["w"])):
                wbuf[first + p * 4 + c] = _rhs_operand(sc, p, lambda k, j: tile(k, 4 * j + c))

    def layernorm(row, n):
        y = xbuf[pl.ds(pl.multiple_of(row, 16), n), :].astype(F32) * jnp.concatenate([vec[0:8, :]] * (n // 8), axis=0)
        d = y - jnp.sum(y, axis=-1, keepdims=True) * (1.0 / C)
        v = jnp.sum(d * d, axis=-1, keepdims=True) * (1.0 / (C * ALPHA * ALPHA)) + 1e-5 / (ALPHA * ALPHA)
        return d * jnp.exp2(-0.5 * jnp.log2(v))

    x0_in = pltpu.make_async_copy(x_hbm.at[pl.ds(0, pr)], xbuf.at[pl.ds(tm1 + HID, pr)], osem.at[0])
    for q in range(4):
        w1_in(q, tm1).start()
    x0_in.start()
    x1_in(0, 0).start()
    ssq[...] = jnp.zeros_like(ssq)
    vec[0:8, :] = jnp.broadcast_to(dw_ref[...].astype(F32), (8, C))
    w1_forms(UP, tm1, 0)
    x0_in.wait()
    for t in range(UP["m"]):
        abuf[t * MC1:(t + 1) * MC1, :] = layernorm(tm1 + HID + t * MC1, MC1)

    def pass1(i, carry):
        xs, hs, q, qs, busy = carry
        slots = [_wrap_up(hs + u, SLOTS) for u in range(G1)]
        qn = jnp.minimum((i * pace1) >> 16, nhc)
        x1_in(i, xs).wait()
        for u in range(G1):
            pl.when(busy[u] != 0)(lambda: h_out(0, slots[u]).wait())
        for u in range(G1):
            pl.when(jnp.logical_and(q + u < qn, stored(q + u)))(
                lambda: h_out(q + u, _wrap_up(qs + u, SLOTS)).start())
        ahead = xs * tm1 + jnp.where(i == nt1 - 1, pr, 0)

        groups, n_prod = tm1 // pr, len(UP["w"])
        nxt = _lhs_operands(UP, lambda t, k: abuf[t * MC1:(t + 1) * MC1, k * L:(k + 1) * L])
        for m in range(groups):
            u, r = divmod(m * pr, CH)
            op, normed = nxt, {}

            def norm(t, m=m, normed=normed):
                if m < groups - 1:
                    normed[t] = layernorm(ahead + m * pr + t * MC1, MC1)
                else:
                    abuf[t * MC1:(t + 1) * MC1, :] = layernorm(xs * tm1 + m * pr + t * MC1, MC1)

            nxt = _lhs_operands(UP, lambda t, k, normed=normed: normed[t][:, k * L:(k + 1) * L])
            todo = {}
            for t in range(UP["m"]):
                todo.setdefault(int(4 * n_prod * 0.65 * t / UP["m"]), []).append(functools.partial(norm, t))
            for p in range(n_prod if m < groups - 1 else 0):
                todo.setdefault(int(4 * n_prod * (0.68 + 0.29 * p / n_prod)), []).append(functools.partial(nxt, p))

            for c in range(4):
                def product(p):
                    for step in todo.pop(c * n_prod + p, []):
                        step()
                    return _dot(op(p), wbuf[p * 4 + c])

                def activate(t, j, y):
                    cols = slice((4 * j + c) * L, (4 * j + c + 1) * L)
                    h = _gelu(y)
                    ssq[:, cols] += jnp.sum((h * h).reshape(MC1 // 8, 8, L), axis=0)
                    hbuf[slots[u], pl.ds((r + t * MC1) // 2, MC1 // 2), cols] = _pack(h)

                _combine(UP, product, activate)
            if m == 0:
                pl.when(i + 1 < nt1)(lambda: x1_in(i + 1, 1 - xs).start())

                @pl.when(i == nt1 - 1)
                def _():
                    w2_in().start()
                    for e in range(4):
                        w1_in(e, stage2 + HID).start()

        prev = [(i + 1) * G1 + u - SLOTS for u in range(G1)]
        busy = tuple(jnp.logical_and(c >= 0, stored(jnp.maximum(c, 0))).astype(jnp.int32) for c in prev)
        return 1 - xs, _wrap_up(hs + G1, SLOTS), qn, _wrap_up(qs + (qn - q), SLOTS), busy

    zero = jnp.int32(0)
    lax.fori_loop(0, nt1, pass1, (zero, zero, zero, zero, (zero,) * G1))

    first = [(nt2 - 1 - j, (nt2 - 1 - j) % XR) for j in range(XR - 1)]
    early = [(i, s) for i, s in first if (s + 1) * tm2 <= stage2 or s * tm2 >= stage2 + 2 * HID]
    for i, s in early:
        x2_in(i, s).start()
    gx = jnp.sqrt(jnp.sum(ssq[...], axis=0, keepdims=True) * (HS * HS) + 1e-6)
    nx = gx / (jnp.mean(gx, axis=-1, keepdims=True) + 1e-6)
    scale = (g_ref[...].astype(F32).reshape(1, HID) * nx + 1.0) * HS
    kg = HID // L // DOWN["k"]
    w2_in().wait()
    for r in range(kg):
        cols = [_column(scale, kg * k + r) for k in range(DOWN["k"])]

        def w2_tile(k, j):
            row = stage2 + (kg * k + r) * L
            return xbuf[row:row + L, j * L:(j + 1) * L].astype(F32) * cols[k]

        for p in range(len(DOWN["w"])):
            wbuf[p * kg + r] = _rhs_operand(DOWN, p, w2_tile)
    up15 = len(DOWN["w"]) * kg
    w1_forms(UP15, stage2 + HID, up15)
    b_row = b_ref[...].astype(F32).reshape(1, HID)
    bias = jnp.zeros((8, C), F32)
    for k in range(HID // L):
        prod = xbuf[stage2 + k * L:stage2 + (k + 1) * L, :].astype(F32) * jnp.concatenate([_column(b_row, k)] * 3, axis=1)
        bias = bias + jnp.sum(prod.reshape(L // 8, 8, C), axis=0)
    vec[8:16, :] = jnp.broadcast_to(jnp.sum(bias, axis=0, keepdims=True), (8, C))
    for i, s in first:
        if (i, s) not in early:
            x2_in(i, s).start()

    def pass2(j, carry):
        xs, hs, q, qs, fetched, x_ready = carry
        i = nt2 - 1 - j
        slots = [_wrap_up(hs + u, SLOTS) for u in range(G2)]
        s2 = _wrap_up(xs + 2, XR)
        pl.when(x_ready == 0)(lambda: x2_in(i, xs).wait())
        for u in range(G2):
            pl.when(fetched[u] != 0)(lambda: h_in(0, slots[u]).wait())
        pl.when(jnp.logical_and(j >= 2, i + 2 > HOLD))(lambda: o_out(i + 2, s2).wait())

        pl.when(jnp.logical_and(j >= 1, i + 1 > HOLD))(lambda: o_out(i + 1, _wrap_up(xs + 1, XR)).start())

        @pl.when(i == 0)
        def _():
            for t in range(HOLD, 0, -1):
                o_out(t, t % XR).start()

        pl.when(jnp.logical_and(j >= 1, i + 2 - XR >= 0))(lambda: x2_in(i + 2 - XR, s2).start())

        rows_per_group = DOWN["m"] * MC2
        groups = tm2 // rows_per_group
        for step, m in enumerate(reversed(range(groups))):
            if step % (groups // G2) == 1:
                done = j * G2 + step // (groups // G2)
                qn = jnp.minimum(jnp.minimum(((done * pace2) >> 16) // G2 + 1, done), nhc)
                for u in range(G2):
                    pl.when(jnp.logical_and(q + u < qn, stored(jnp.maximum(nhc - 1 - q - u, 0))))(
                        lambda: h_in(nhc - 1 - q - u, _wrap_down(qs - u, SLOTS)).start())
                qn = jnp.clip(qn, q, q + G2)
                q, qs = qn, _wrap_down(qs - (qn - q), SLOTS)

            u, r0 = divmod(m * rows_per_group, CH)
            acc = {}
            for r in range(kg):
                op = _lhs_operands(DOWN, lambda t, k: _unpack(
                    hbuf[slots[u], pl.ds((r0 + t * MC2) // 2, MC2 // 2), (kg * k + r) * L:(kg * k + r + 1) * L]))

                def accumulate(t, jj, o):
                    acc[t, jj] = o if r == 0 else acc[t, jj] + o
                    if r == kg - 1:
                        rows = pl.ds(pl.multiple_of(xs * tm2 + u * CH + r0 + t * MC2, 16), MC2)
                        cols = slice(jj * L, (jj + 1) * L)
                        res = acc[t, jj] + xbuf[rows, cols].astype(F32)
                        res = res + jnp.concatenate([vec[8:16, cols]] * (MC2 // 8), axis=0)
                        xbuf[rows, cols] = res.astype(BF16)

                _combine(DOWN, lambda p: _dot(op(p), wbuf[p * kg + r]), accumulate)

        nxt = [jnp.maximum(i - 1, 0) * G2 + u for u in range(G2)]
        fetched = tuple(jnp.logical_and(c < nhc, stored(c)).astype(jnp.int32) for c in nxt)
        return _wrap_down(xs - 1, XR), _wrap_down(hs - G2, SLOTS), q, qs, fetched, zero

    def recompute(xs, slot):
        def half(e, _):
            for r in range(0, CH // 2, 2 * MCR):
                r = e * (CH // 2) + r
                a = [layernorm(xs * tm2 + r + t * MCR, MCR) for t in range(2)]
                op = _lhs_operands(UP15, lambda t, k: a[t][:, k * L:(k + 1) * L])
                for c in range(4):
                    def keep(t, jj, y):
                        rows = pl.ds(pl.multiple_of((r + t * MCR) // 2, 8), MCR // 2)
                        hbuf[slot, rows, (4 * jj + c) * L:(4 * jj + c + 1) * L] = _pack(_gelu(y))

                    _combine(UP15, lambda p: _dot(op(p), wbuf[up15 + p * 4 + c]), keep)
            return _

        lax.fori_loop(0, 2, half, 0)

    def segment(e, carry):
        every = REDO_EVERY // G2
        top = nt2 - 1 - REDO_FIRST // G2 - (n_redo - 1) * every
        lo = jnp.where(e == 0, 0, top + (e - 1) * every)
        hi = jnp.where(e == n_redo, nt2, top + e * every)

        @pl.when(e > 0)
        def _():
            x2_in(nt2 - 1 - lo, carry[0]).wait()
            recompute(carry[0], carry[1])

        return lax.fori_loop(lo, hi, pass2, carry[:5] + (jnp.minimum(e, 1),))

    lax.fori_loop(0, n_redo + 1, segment, (zero + (nt2 - 1) % XR, zero + (nch - G2) % SLOTS, zero,
                                           zero + (nhc - 1) % SLOTS, (zero,) * G2, zero))
    o_out(0, 0).start()
    for t in range(HOLD, -1, -1):
        o_out(t, t % XR).wait()


@jax.jit
def pallas_standalone__modern_conv_block_slak__vision_kernel(x, dw, w1, w2, grn_g, grn_b):
    n_pix = x.shape[1] * x.shape[2]
    assert x.shape[0] == 1 and x.shape[3] == C and dw.shape == (1, 1, C) and w1.shape == (C, HID)
    assert n_pix % (G1 * CH) == 0 and n_pix // CH > SLOTS + 4 * G1
    nhc = n_pix // CH - SLOTS
    n_stored = nhc - len(range(REDO_FIRST, nhc, REDO_EVERY))
    n_tiles = max(4 * len(UP["w"]), (HID // L // DOWN["k"]) * len(DOWN["w"]) + 4 * len(UP15["w"]))
    hbm = pl.BlockSpec(memory_space=pl.ANY)
    vmem = pl.BlockSpec(memory_space=pltpu.VMEM)
    out, _ = pl.pallas_call(
        _kernel,
        in_specs=[hbm, vmem, hbm, hbm, vmem, vmem],
        out_specs=[hbm, hbm],
        out_shape=[jax.ShapeDtypeStruct((n_pix, C), BF16), jax.ShapeDtypeStruct((n_stored, CH // 2, HID), U32)],
        scratch_shapes=[
            pltpu.VMEM((max(2 * G1, XR * G2) * CH, C), BF16),
            pltpu.VMEM((SLOTS, CH // 2, HID), U32),
            pltpu.VMEM((n_tiles, L // 2, L), U32),
            pltpu.VMEM((UP["m"] * MC1, C), F32),
            pltpu.VMEM((8, HID), F32),
            pltpu.VMEM((16, C), F32),
            pltpu.SemaphoreType.DMA((XR,)),
            pltpu.SemaphoreType.DMA((XR,)),
            pltpu.SemaphoreType.DMA((SLOTS,)),
            pltpu.SemaphoreType.DMA((5,)),
        ],
        compiler_params=pltpu.CompilerParams(vmem_limit_bytes=128 * 1024 * 1024, disable_bounds_checks=True),
    )(x.reshape(n_pix, C), dw.reshape(1, C), w1, w2, grn_g, grn_b)
    return out.reshape(x.shape)
```

```python
import functools

import jax
import jax.experimental.pallas as pl
import jax.experimental.pallas.tpu as pltpu
import jax.numpy as jnp
import numpy as np
from jax import lax

F32, BF16, U32 = jnp.float32, jnp.bfloat16, jnp.uint32
L = 128
C, HID = 384, 1536

_K0 = float(np.sqrt(2.0 / np.pi))
ALPHA = float((_K0 * 0.044715) ** (1.0 / 3.0))
C0 = _K0 / ALPHA
HS = 0.5 / ALPHA

CH = 768
SLOTS = 52
G1, G2 = 4, 2
XR = 4
HOLD = 3
MC1, MC2, MCR = 48, 32, 48
REDO_EVERY, REDO_FIRST = 32, 16

UP = dict(
    m=4, k=3, n=3,
    a_prog=[(10,-1,3,1), (6,-1,3,1), (3,1,7,-1), (5,-1,1,1), (11,-1,0,1), (9,-1,13,1), (11,-1,17,1), (6,1,18,1),
            (10,-1,4,1), (5,1,20,1), (7,-1,20,1), (21,1,7,-1), (22,1,1,1), (2,1,5,1), (8,-1,25,1), (0,1,25,1),
            (8,-1,27,1), (1,1,12,-1), (29,1,20,1), (2,1,11,1), (1,1,31,1), (8,-1,23,1), (33,1,18,1), (28,1,13,1),
            (14,-1,35,1), (12,1,19,-1), (16,1,37,1)],
    a_use=[5, 0, 27, 1, 32, 15, 30, 3, 11, 16, 10, 14, 12, 19, 21, 38, 13, 7, 8, 10, 23, 18, 22, 34, 24, 28, 26, 17,
           36],
    c_prog=[(4,1,7,1), (0,1,3,-1), (4,1,10,1), (2,1,9,1), (10,1,8,1), (5,1,8,1), (5,1,11,1), (4,-1,1,1), (6,-1,1,1),
            (18,1,9,1), (2,1,13,1), (6,1,12,1), (8,1,19,1), (23,1,14,-1), (24,1,12,1), (17,1,21,-1), (2,1,10,-1),
            (28,1,11,-1), (22,1,24,1), (30,1,17,-1), (23,1,21,1), (32,1,3,1), (2,1,0,1), (34,1,6,1), (0,1,1,1),
            (36,1,9,-1)],
    c_use=[(31,-1), (37,-1), (35,1), (13,-1), (2,-1), (22,-1), (3,-1), (33,-1), (29,-1), (15,1), (18,1), (23,-1),
           (21,1), (27,1), (17,-1), (9,1), (25,-1), (12,1), (26,1), (14,-1), (24,-1), (16,1), (19,-1), (8,-1), (1,-1),
           (20,1), (1,-1), (10,-1), (6,-1)],
    w=[(0,0,0,0,0,-1,0,0,1), (-1,0,0,0,0,0,1,0,0), (0,0,0,0,0,0,1,0,0), (0,0,0,-1,0,1,1,0,-1),
       (0,0,0,0,0,0,1,0,-1), (0,0,0,0,0,-1,-1,0,1), (0,0,0,-1,0,0,0,0,0), (-1,0,0,-1,0,0,0,0,0),
       (0,0,-1,0,0,0,0,0,1), (0,0,1,0,0,0,-1,0,0), (-1,0,1,-1,0,1,0,0,0), (1,-1,0,1,0,0,0,0,0),
       (-1,0,1,-1,0,0,0,0,0), (0,0,1,0,0,0,0,0,0), (0,0,0,0,0,-1,0,0,0), (1,0,-1,0,0,0,0,0,0), (0,1,0,0,0,0,0,0,0),
       (-1,1,0,-1,1,0,0,0,0), (0,0,0,0,0,0,0,1,0), (0,0,0,0,-1,0,0,0,0), (0,0,0,0,0,1,0,1,-1),
       (0,0,-1,0,0,0,0,-1,1), (0,0,0,0,1,-1,0,-1,1), (0,0,0,0,0,0,0,-1,1), (0,0,0,0,-1,0,0,0,0),
       (-1,1,0,0,0,0,1,0,0), (-1,1,0,0,0,0,1,-1,0), (0,1,-1,0,0,0,0,-1,1), (1,-1,0,0,0,0,0,0,0)],
)

DOWN = dict(
    m=3, k=4, n=3,
    a_prog=[(0,1,10,-1), (4,1,5,1), (6,1,5,1), (7,1,5,1), (11,1,4,1), (3,1,6,1), (9,1,8,1), (11,1,9,1), (2,1,1,1),
            (0,1,18,-1), (3,1,15,1), (20,1,10,-1), (14,1,11,-1), (22,1,13,-1), (21,1,19,1), (24,1,15,-1), (23,1,24,-1),
            (28,1,19,-1), (12,1,26,-1), (30,1,16,1), (1,1,3,1), (32,-1,23,1), (33,-1,12,1), (34,1,17,-1), (32,1,21,1),
            (15,1,36,1)],
    a_use=[6, 13, 15, 14, 24, 20, 3, 23, 27, 17, 25, 6, 22, 4, 16, 29, 10, 37, 11, 35, 33, 19, 31, 18, 12, 0, 21, 26,
           1],
    c_prog=[(0,1,2,-1), (5,1,8,-1), (0,1,6,1), (6,1,8,-1), (2,1,6,1), (2,1,8,1), (3,-1,0,1), (7,1,8,-1), (0,1,1,-1),
            (1,-1,15,1), (2,1,16,-1), (15,1,2,-1), (5,1,16,1), (6,1,17,1), (6,1,10,1), (19,-1,1,1), (3,1,23,-1),
            (18,1,4,1), (22,1,7,-1), (4,1,21,-1), (20,1,5,1)],
    c_use=[(4,1), (4,1), (26,1), (28,-1), (21,1), (24,-1), (15,-1), (19,1), (5,-1), (20,1), (3,1), (29,1), (18,1),
           (25,1), (23,-1), (16,1), (14,1), (17,-1), (10,-1), (9,1), (2,-1), (7,-1), (12,1), (27,-1), (13,1), (11,-1),
           (22,-1), (6,1), (1,-1)],
    w=[(0,1,0,0,-1,0,0,1,0,0,1,0), (0,1,0,0,0,0,0,0,0,0,0,0), (0,0,0,0,0,0,0,0,0,0,1,0),
       (0,1,0,0,-1,0,0,0,0,0,1,0), (0,-1,0,0,1,1,0,0,0,0,-1,0), (0,0,0,0,0,0,0,-1,0,0,0,0),
       (0,0,0,0,0,1,-1,0,-1,-1,-1,-1), (0,0,0,0,0,1,0,1,0,0,0,0), (0,0,0,0,0,0,0,0,0,0,0,1),
       (0,0,0,0,0,1,-1,0,-1,0,0,-1), (0,0,0,-1,0,0,0,0,0,1,0,0), (0,0,0,0,0,-1,0,0,1,0,0,1),
       (0,0,0,-1,0,0,0,0,0,0,-1,0), (1,0,0,-1,0,0,0,0,0,1,0,0), (-1,0,-1,1,0,0,0,0,0,-1,0,0),
       (0,0,0,0,0,1,0,0,0,0,0,0), (0,0,1,0,0,0,0,1,1,0,0,0), (0,0,0,-1,0,0,0,0,0,0,0,0),
       (1,1,1,-1,-1,-1,0,0,0,1,1,1), (0,0,0,0,0,0,-1,0,0,0,0,0), (0,0,0,0,0,1,-1,0,-1,0,0,0),
       (0,1,0,0,-1,-1,0,0,0,0,0,0), (0,0,-1,0,0,0,0,0,0,0,0,0), (0,1,0,0,0,0,0,0,0,0,0,0),
       (0,0,1,0,0,0,-1,0,0,0,0,0), (-1,-1,0,0,0,0,-1,0,0,0,0,0), (0,1,0,1,0,0,0,0,0,0,0,0),
       (-1,0,-1,1,0,0,0,0,0,0,0,0), (0,0,0,-1,-1,0,0,1,0,0,0,0)],
)

UP15 = dict(
    m=2, k=3, n=3,
    a_prog=[(5,1,4,1), (5,-1,3,1), (0,1,2,-1), (0,1,3,-1), (2,1,3,-1), (5,-1,2,1), (0,1,1,-1), (12,1,3,-1), (6,-1,2,1),
            (1,1,14,1), (13,1,4,1)],
    a_use=[4, 14, 6, 1, 2, 12, 15, 8, 13, 16, 7, 3, 10, 11, 9],
    c_prog=[(5,-1,0,1), (5,1,3,1), (3,1,0,1), (1,1,2,-1), (4,-1,3,1), (0,1,2,1), (5,1,2,1), (12,-1,1,1), (0,1,10,1),
            (1,-1,14,1), (4,1,13,1)],
    c_use=[(4,1), (13,-1), (16,1), (1,1), (12,1), (15,1), (9,-1), (11,-1), (14,-1), (10,1), (7,1), (8,-1), (6,-1),
           (5,-1), (0,1)],
    w=[(0,0,0,1,1,0,0,-1,0), (0,0,0,0,0,-1,0,-1,0), (0,0,0,0,0,0,0,1,0), (0,1,0,0,1,1,0,0,0), (0,0,1,0,0,0,0,1,1),
       (0,-1,0,0,0,0,0,0,0), (0,0,0,0,0,1,0,0,0), (0,0,-1,0,0,0,0,0,0), (0,-1,0,1,0,0,0,0,0), (0,0,0,1,0,0,0,0,0),
       (0,0,0,0,0,0,-1,0,0), (-1,-1,0,0,0,0,-1,0,0), (0,0,-1,0,0,0,-1,0,0), (0,0,0,0,0,-1,-1,0,1),
       (1,0,-1,1,0,0,0,0,0)],
)


def _lhs_operands(sc, block):
    m, k = sc["m"], sc["k"]
    memo, packed = {}, {}

    def node(v):
        if v not in memo:
            if v < m * k:
                memo[v] = (1, block(v // k, v % k))
            else:
                a, sa, b, sb = sc["a_prog"][v - m * k]
                (ta, xa), (tb, xb) = node(a), node(b)
                ta, tb = ta * sa, tb * sb
                memo[v] = (ta, xa + xb) if ta == tb else (1, xa - xb if ta > 0 else xb - xa)
        return memo[v]

    def operand(p):
        v = sc["a_use"][p]
        if v not in packed:
            packed[v] = node(v)[1].astype(BF16)
        return packed[v]

    return operand


def _combine(sc, product, emit):
    m, n = sc["m"], sc["n"]
    pending = [0] * (m * n + len(sc["c_prog"]))
    for v, _ in sc["c_use"]:
        pending[v] += 1
    for a, _, b, _ in sc["c_prog"]:
        pending[a] += 1
        pending[b] += 1
    partial = {}

    def push(v, t, x):
        if v in partial:
            u, y = partial[v]
            t, x = (t, y + x) if t == u else (1, x - y if t > 0 else y - x)
        partial[v] = (t, x)
        pending[v] -= 1
        if pending[v] == 0:
            if v >= m * n:
                a, sa, b, sb = sc["c_prog"][v - m * n]
                push(a, t * sa, x)
                push(b, t * sb, x)
            else:
                assert t == 1
                emit(v // n, v % n, x)

    for p, (v, t) in enumerate(sc["c_use"]):
        push(v, t, product(p))


def _rhs_operand(sc, p, block):
    coef, acc = sc["w"][p], None
    for q in sorted(range(len(coef)), key=lambda q: -coef[q]):
        if coef[q]:
            v = block(q // sc["n"], q % sc["n"])
            if acc is None:
                acc = v if coef[q] > 0 else -v
            else:
                acc = acc + v if coef[q] > 0 else acc - v
    return pltpu.bitcast(acc.astype(BF16), U32)


def _dot(a, words):
    return jnp.dot(a, pltpu.bitcast(words, BF16), preferred_element_type=F32)


def _pack(v):
    t = v.shape[0] // 16
    lo = jnp.concatenate([v[16 * g:16 * g + 8] for g in range(t)], axis=0)
    hi = jnp.concatenate([v[16 * g + 8:16 * g + 16] for g in range(t)], axis=0)
    return jnp.concatenate([lo, hi], axis=1).astype(BF16)


def _unpack(w):
    w = w.astype(F32)
    parts = []
    for g in range(w.shape[0] // 8):
        parts += [w[8 * g:8 * g + 8, :L], w[8 * g:8 * g + 8, L:]]
    return jnp.concatenate(parts, axis=0)


def _gelu(y):
    return y * jnp.tanh(y * (y * y + C0)) + y


def _column(row, k):
    return jnp.broadcast_to(row[:, k * L:(k + 1) * L], (L, L)).T


def _wrap_up(v, n):
    return jnp.where(v >= n, v - n, v)


def _wrap_down(v, n):
    return jnp.where(v < 0, v + n, v)


def _kernel(x_hbm, dw_ref, w1_hbm, w2_hbm, g_ref, b_ref, out_hbm, h_hbm,
            xbuf, hbuf, wbuf, abuf, ssq, vec, xsem, osem, hsem, wsem):
    n_pix = x_hbm.shape[0]
    tm1, tm2 = G1 * CH, G2 * CH
    nt1, nt2, nch = n_pix // tm1, n_pix // tm2, n_pix // CH
    nhc = nch - SLOTS
    n_redo = nhc - h_hbm.shape[0]
    pace1 = -(-nhc * 65536 // (nt1 - 3))
    pace2 = -(-nhc * 65536 * 2 // (2 * nt2 - 3))
    pr = UP["m"] * MC1
    stage2 = (nt1 % 2) * tm1

    def stored(c):
        return jnp.logical_or((c + (REDO_EVERY - REDO_FIRST)) % REDO_EVERY != 0,
                              c >= REDO_FIRST + n_redo * REDO_EVERY)

    def h_index(c):
        return c - jnp.minimum((c + (REDO_EVERY - 1 - REDO_FIRST)) // REDO_EVERY, n_redo)

    def h_out(c, slot):
        return pltpu.make_async_copy(hbuf.at[slot], h_hbm.at[h_index(c)], hsem.at[slot])

    def h_in(c, slot):
        return pltpu.make_async_copy(h_hbm.at[h_index(c)], hbuf.at[slot], hsem.at[slot])

    def x_rows(slot, tm):
        return xbuf.at[pl.ds(pl.multiple_of(slot * tm, tm), tm)]

    def x1_in(i, slot):
        row = pl.multiple_of(jnp.minimum(i * tm1 + pr, n_pix - tm1), 16)
        return pltpu.make_async_copy(x_hbm.at[pl.ds(row, tm1)], x_rows(slot, tm1), xsem.at[slot])

    def x2_in(i, slot):
        return pltpu.make_async_copy(x_hbm.at[pl.ds(i * tm2, tm2)], x_rows(slot, tm2), xsem.at[slot])

    def o_out(i, slot):
        return pltpu.make_async_copy(x_rows(slot, tm2), out_hbm.at[pl.ds(i * tm2, tm2)], osem.at[slot])

    def w1_in(q, row):
        return pltpu.make_async_copy(w1_hbm.at[:, pl.ds(q * C, C)], xbuf.at[pl.ds(row + q * C, C)], wsem.at[q])

    def w2_in():
        return pltpu.make_async_copy(w2_hbm, xbuf.at[pl.ds(stage2, HID)], wsem.at[4])

    def w1_forms(sc, row, first):
        def tile(k, n):
            r = row + (n // 3) * C + k * L
            return xbuf[r:r + L, (n % 3) * L:(n % 3 + 1) * L].astype(F32)

        for q in range(4):
            w1_in(q, row).wait()
        for c in range(4):
            for p in range(len(sc["w"])):
                wbuf[first + p * 4 + c] = _rhs_operand(sc, p, lambda k, j: tile(k, 4 * j + c))

    def layernorm(row, n):
        y = xbuf[pl.ds(pl.multiple_of(row, 16), n), :].astype(F32) * jnp.concatenate([vec[0:8, :]] * (n // 8), axis=0)
        d = y - jnp.sum(y, axis=-1, keepdims=True) * (1.0 / C)
        v = jnp.sum(d * d, axis=-1, keepdims=True) * (1.0 / (C * ALPHA * ALPHA)) + 1e-5 / (ALPHA * ALPHA)
        return d * jnp.exp2(-0.5 * jnp.log2(v))

    x0_in = pltpu.make_async_copy(x_hbm.at[pl.ds(0, pr)], xbuf.at[pl.ds(tm1 + HID, pr)], osem.at[0])
    for q in range(4):
        w1_in(q, tm1).start()
    x0_in.start()
    x1_in(0, 0).start()
    ssq[...] = jnp.zeros_like(ssq)
    vec[0:8, :] = jnp.broadcast_to(dw_ref[...].astype(F32), (8, C))
    w1_forms(UP, tm1, 0)
    x0_in.wait()
    for t in range(UP["m"]):
        abuf[t * MC1:(t + 1) * MC1, :] = layernorm(tm1 + HID + t * MC1, MC1)

    def pass1(i, carry):
        xs, hs, q, qs, busy = carry
        slots = [_wrap_up(hs + u, SLOTS) for u in range(G1)]
        qn = jnp.minimum((i * pace1) >> 16, nhc)
        x1_in(i, xs).wait()
        for u in range(G1):
            pl.when(busy[u] != 0)(lambda: h_out(0, slots[u]).wait())
        for u in range(G1):
            pl.when(jnp.logical_and(q + u < qn, stored(q + u)))(
                lambda: h_out(q + u, _wrap_up(qs + u, SLOTS)).start())
        ahead = xs * tm1 + jnp.where(i == nt1 - 1, pr, 0)

        groups, n_prod = tm1 // pr, len(UP["w"])
        nxt = _lhs_operands(UP, lambda t, k: abuf[t * MC1:(t + 1) * MC1, k * L:(k + 1) * L])
        for m in range(groups):
            u, r = divmod(m * pr, CH)
            op, normed = nxt, {}

            def norm(t, m=m, normed=normed):
                if m < groups - 1:
                    normed[t] = layernorm(ahead + m * pr + t * MC1, MC1)
                else:
                    abuf[t * MC1:(t + 1) * MC1, :] = layernorm(xs * tm1 + m * pr + t * MC1, MC1)

            nxt = _lhs_operands(UP, lambda t, k, normed=normed: normed[t][:, k * L:(k + 1) * L])
            todo = {}
            for t in range(UP["m"]):
                todo.setdefault(int(4 * n_prod * 0.65 * t / UP["m"]), []).append(functools.partial(norm, t))
            for p in range(n_prod if m < groups - 1 else 0):
                todo.setdefault(int(4 * n_prod * (0.68 + 0.29 * p / n_prod)), []).append(functools.partial(nxt, p))

            for c in range(4):
                def product(p):
                    for step in todo.pop(c * n_prod + p, []):
                        step()
                    return _dot(op(p), wbuf[p * 4 + c])

                def activate(t, j, y):
                    cols = slice((4 * j + c) * L, (4 * j + c + 1) * L)
                    h = _gelu(y)
                    ssq[:, cols] += jnp.sum((h * h).reshape(MC1 // 8, 8, L), axis=0)
                    hbuf[slots[u], pl.ds((r + t * MC1) // 2, MC1 // 2), pl.ds((4 * j + c) * 2 * L, 2 * L)] = _pack(h)

                _combine(UP, product, activate)
            if m == 0:
                pl.when(i + 1 < nt1)(lambda: x1_in(i + 1, 1 - xs).start())

                @pl.when(i == nt1 - 1)
                def _():
                    w2_in().start()
                    for e in range(4):
                        w1_in(e, stage2 + HID).start()

        prev = [(i + 1) * G1 + u - SLOTS for u in range(G1)]
        busy = tuple(jnp.logical_and(c >= 0, stored(jnp.maximum(c, 0))).astype(jnp.int32) for c in prev)
        return 1 - xs, _wrap_up(hs + G1, SLOTS), qn, _wrap_up(qs + (qn - q), SLOTS), busy

    zero = jnp.int32(0)
    lax.fori_loop(0, nt1, pass1, (zero, zero, zero, zero, (zero,) * G1))

    first = [(nt2 - 1 - j, (nt2 - 1 - j) % XR) for j in range(XR - 1)]
    early = [(i, s) for i, s in first if (s + 1) * tm2 <= stage2 or s * tm2 >= stage2 + 2 * HID]
    for i, s in early:
        x2_in(i, s).start()
    gx = jnp.sqrt(jnp.sum(ssq[...], axis=0, keepdims=True) * (HS * HS) + 1e-6)
    nx = gx / (jnp.mean(gx, axis=-1, keepdims=True) + 1e-6)
    scale = (g_ref[...].astype(F32).reshape(1, HID) * nx + 1.0) * HS
    kg = HID // L // DOWN["k"]
    w2_in().wait()
    for r in range(kg):
        cols = [_column(scale, kg * k + r) for k in range(DOWN["k"])]

        def w2_tile(k, j):
            row = stage2 + (kg * k + r) * L
            return xbuf[row:row + L, j * L:(j + 1) * L].astype(F32) * cols[k]

        for p in range(len(DOWN["w"])):
            wbuf[p * kg + r] = _rhs_operand(DOWN, p, w2_tile)
    up15 = len(DOWN["w"]) * kg
    w1_forms(UP15, stage2 + HID, up15)
    b_row = b_ref[...].astype(F32).reshape(1, HID)
    bias = jnp.zeros((8, C), F32)
    for k in range(HID // L):
        prod = xbuf[stage2 + k * L:stage2 + (k + 1) * L, :].astype(F32) * jnp.concatenate([_column(b_row, k)] * 3, axis=1)
        bias = bias + jnp.sum(prod.reshape(L // 8, 8, C), axis=0)
    vec[8:16, :] = jnp.broadcast_to(jnp.sum(bias, axis=0, keepdims=True), (8, C))
    for i, s in first:
        if (i, s) not in early:
            x2_in(i, s).start()

    def pass2(j, carry):
        xs, hs, q, qs, fetched, x_ready = carry
        i = nt2 - 1 - j
        slots = [_wrap_up(hs + u, SLOTS) for u in range(G2)]
        s2 = _wrap_up(xs + 2, XR)
        pl.when(x_ready == 0)(lambda: x2_in(i, xs).wait())
        for u in range(G2):
            pl.when(fetched[u] != 0)(lambda: h_in(0, slots[u]).wait())
        pl.when(jnp.logical_and(j >= 2, i + 2 > HOLD))(lambda: o_out(i + 2, s2).wait())

        pl.when(jnp.logical_and(j >= 1, i + 1 > HOLD))(lambda: o_out(i + 1, _wrap_up(xs + 1, XR)).start())

        @pl.when(i == 0)
        def _():
            for t in range(HOLD, 0, -1):
                o_out(t, t % XR).start()

        pl.when(jnp.logical_and(j >= 1, i + 2 - XR >= 0))(lambda: x2_in(i + 2 - XR, s2).start())

        rows_per_group = DOWN["m"] * MC2
        groups = tm2 // rows_per_group
        for step, m in enumerate(reversed(range(groups))):
            if step % (groups // G2) == 1:
                done = j * G2 + step // (groups // G2)
                qn = jnp.minimum(jnp.minimum(((done * pace2) >> 16) // G2 + 1, done), nhc)
                for u in range(G2):
                    pl.when(jnp.logical_and(q + u < qn, stored(jnp.maximum(nhc - 1 - q - u, 0))))(
                        lambda: h_in(nhc - 1 - q - u, _wrap_down(qs - u, SLOTS)).start())
                qn = jnp.clip(qn, q, q + G2)
                q, qs = qn, _wrap_down(qs - (qn - q), SLOTS)

            u, r0 = divmod(m * rows_per_group, CH)
            acc = {}
            for r in range(kg):
                op = _lhs_operands(DOWN, lambda t, k: _unpack(
                    hbuf[slots[u], pl.ds((r0 + t * MC2) // 2, MC2 // 2), pl.ds((kg * k + r) * 2 * L, 2 * L)]))

                def accumulate(t, jj, o):
                    acc[t, jj] = o if r == 0 else acc[t, jj] + o
                    if r == kg - 1:
                        rows = pl.ds(pl.multiple_of(xs * tm2 + u * CH + r0 + t * MC2, 16), MC2)
                        cols = slice(jj * L, (jj + 1) * L)
                        res = acc[t, jj] + xbuf[rows, cols].astype(F32)
                        res = res + jnp.concatenate([vec[8:16, cols]] * (MC2 // 8), axis=0)
                        xbuf[rows, cols] = res.astype(BF16)

                _combine(DOWN, lambda p: _dot(op(p), wbuf[p * kg + r]), accumulate)

        nxt = [jnp.maximum(i - 1, 0) * G2 + u for u in range(G2)]
        fetched = tuple(jnp.logical_and(c < nhc, stored(c)).astype(jnp.int32) for c in nxt)
        return _wrap_down(xs - 1, XR), _wrap_down(hs - G2, SLOTS), q, qs, fetched, zero

    def recompute(xs, slot):
        def half(e, _):
            for r in range(0, CH // 2, 2 * MCR):
                r = e * (CH // 2) + r
                a = [layernorm(xs * tm2 + r + t * MCR, MCR) for t in range(2)]
                op = _lhs_operands(UP15, lambda t, k: a[t][:, k * L:(k + 1) * L])
                for c in range(4):
                    def keep(t, jj, y):
                        rows = pl.ds(pl.multiple_of((r + t * MCR) // 2, 8), MCR // 2)
                        hbuf[slot, rows, pl.ds((4 * jj + c) * 2 * L, 2 * L)] = _pack(_gelu(y))

                    _combine(UP15, lambda p: _dot(op(p), wbuf[up15 + p * 4 + c]), keep)
            return _

        lax.fori_loop(0, 2, half, 0)

    def segment(e, carry):
        every = REDO_EVERY // G2
        top = nt2 - 1 - REDO_FIRST // G2 - (n_redo - 1) * every
        lo = jnp.where(e == 0, 0, top + (e - 1) * every)
        hi = jnp.where(e == n_redo, nt2, top + e * every)

        @pl.when(e > 0)
        def _():
            x2_in(nt2 - 1 - lo, carry[0]).wait()
            recompute(carry[0], carry[1])

        return lax.fori_loop(lo, hi, pass2, carry[:5] + (jnp.minimum(e, 1),))

    lax.fori_loop(0, n_redo + 1, segment, (zero + (nt2 - 1) % XR, zero + (nch - G2) % SLOTS, zero,
                                           zero + (nhc - 1) % SLOTS, (zero,) * G2, zero))
    o_out(0, 0).start()
    for t in range(HOLD, -1, -1):
        o_out(t, t % XR).wait()


@jax.jit
def pallas_standalone__modern_conv_block_slak__vision_kernel(x, dw, w1, w2, grn_g, grn_b):
    n_pix = x.shape[1] * x.shape[2]
    assert x.shape[0] == 1 and x.shape[3] == C and dw.shape == (1, 1, C) and w1.shape == (C, HID)
    assert n_pix % (G1 * CH) == 0 and n_pix // CH > SLOTS + 4 * G1
    nhc = n_pix // CH - SLOTS
    n_stored = nhc - len(range(REDO_FIRST, nhc, REDO_EVERY))
    n_tiles = max(4 * len(UP["w"]), (HID // L // DOWN["k"]) * len(DOWN["w"]) + 4 * len(UP15["w"]))
    hbm = pl.BlockSpec(memory_space=pl.ANY)
    vmem = pl.BlockSpec(memory_space=pltpu.VMEM)
    out, _ = pl.pallas_call(
        _kernel,
        in_specs=[hbm, vmem, hbm, hbm, vmem, vmem],
        out_specs=[hbm, hbm],
        out_shape=[jax.ShapeDtypeStruct((n_pix, C), BF16), jax.ShapeDtypeStruct((n_stored, CH // 2, 2 * HID), BF16)],
        scratch_shapes=[
            pltpu.VMEM((max(2 * G1, XR * G2) * CH, C), BF16),
            pltpu.VMEM((SLOTS, CH // 2, 2 * HID), BF16),
            pltpu.VMEM((n_tiles, L // 2, L), U32),
            pltpu.VMEM((UP["m"] * MC1, C), F32),
            pltpu.VMEM((8, HID), F32),
            pltpu.VMEM((16, C), F32),
            pltpu.SemaphoreType.DMA((XR,)),
            pltpu.SemaphoreType.DMA((XR,)),
            pltpu.SemaphoreType.DMA((SLOTS,)),
            pltpu.SemaphoreType.DMA((5,)),
        ],
        compiler_params=pltpu.CompilerParams(vmem_limit_bytes=128 * 1024 * 1024, disable_bounds_checks=True),
    )(x.reshape(n_pix, C), dw.reshape(1, C), w1, w2, grn_g, grn_b)
    return out.reshape(x.shape)
```
